```python
import os as _os
_os.environ.setdefault('JAX_PLATFORMS', 'cpu')
import jax
import jax.numpy as jnp

def _softmax(x, axis=-1):
    return jax.nn.softmax(x, axis=axis)

def _gelu(x):
    return jax.nn.gelu(x, approximate=True)

def _silu(x):
    return jax.nn.silu(x)

def _sigmoid(x):
    return jax.nn.sigmoid(x)

def _layernorm(x, axis=-1, eps=1e-05):
    m = jnp.mean(x, axis=axis, keepdims=True)
    v = jnp.var(x, axis=axis, keepdims=True)
    return (x - m) / jnp.sqrt(v + eps)

def _scatter_add(tgt, idx, src, axis=0):
    return tgt.at[idx].add(src)

def _segment_sum(src, seg, n):
    return jax.ops.segment_sum(src, seg, n)

class _Rng:

    def __init__(self, key):
        self._k = key

    def _next(self):
        self._k, sub = jax.random.split(self._k)
        return sub

    def normal(self, shape):
        return jax.random.normal(self._next(), shape, dtype=jnp.bfloat16)

    def randint(self, lo, hi, shape):
        return jax.random.randint(self._next(), shape, lo, hi, dtype=jnp.int32)

    def uniform(self, shape, lo=0.0, hi=1.0):
        return jax.random.uniform(self._next(), shape, jnp.bfloat16, lo, hi)

    def permutation(self, n):
        return jax.random.permutation(self._next(), n)
kernel_name = 'standalone__neighborhood_nat__vision'

def setup_inputs():
    _rng = _Rng(jax.random.key(int.from_bytes(__import__("os").urandom(4), "little")))
    _w = lambda a: (lambda t: t.astype(jnp.bfloat16) if jnp.issubdtype(t.dtype, jnp.floating) else t)(jnp.asarray(a))
    H = W = 384
    C = 96
    return {'x': _w((lambda *s: _rng.normal(s) * 0.2)(1, H, W, C)), 'wqkv': _w((lambda *s: _rng.normal(s) * 0.2)(C, 3 * C)), 'wo': _w((lambda *s: _rng.normal(s) * 0.05)(C, C))}

def reference(x, wqkv, wo):
    B, H, W, C = x.shape
    ks, dil = (7, 2)
    qkv = x @ wqkv
    q, k, v = (qkv[..., :C].copy(), qkv[..., C:2 * C].copy(), qkv[..., 2 * C:].copy())
    half = (ks - 1) // 2 * dil
    ir = jnp.arange(H)
    ic = jnp.arange(W)
    off = jnp.arange(ks) * dil
    r0 = jnp.clip(ir - half, 0, H - 1 - (ks - 1) * dil)
    c0 = jnp.clip(ic - half, 0, W - 1 - (ks - 1) * dil)
    ri = r0[:, None] + off[None, :]
    ci = c0[:, None] + off[None, :]
    nidx = (ri[:, None, :, None] * W + ci[None, :, None, :]).reshape(1, H * W * ks * ks, 1)
    kf = k.reshape(B, H * W, C)
    vf = v.reshape(B, H * W, C)
    kn = jnp.take_along_axis(kf, nidx, 1).reshape(B, H * W, ks * ks, C)
    vn = jnp.take_along_axis(vf, nidx, 1).reshape(B, H * W, ks * ks, C)
    qf = q.reshape(B, H * W, C)
    scale = C ** (-0.5)
    logits = jnp.einsum('bnc,bnkc->bnk', qf, kn) * scale
    p = _softmax(logits, axis=-1)
    o = jnp.einsum('bnk,bnkc->bnc', p, vn) @ wo
    return o.reshape(B, H, W, C)
```

```python
import math

import jax
import jax.numpy as jnp
from jax import lax
from jax.experimental import pallas as pl
from jax.experimental.pallas import tpu as pltpu

H = 384
W = 384
C = 96
NB = 24
NS = 24
NG = 25
BIG = 2.0 ** 100
ONE2 = 0x3F803F80
RM = 14
CM = 15
L_ROW = 96
L_COL = 110
L_ONE = 125
L_PAD = 126
NBIG_BITS = 0xF180
D = 6
E = 4
NTAIL = 6

bf16 = jnp.bfloat16
f32 = jnp.float32
u32 = jnp.uint32
i32 = jnp.int32


def _iota(shape, dim):
    return lax.broadcasted_iota(i32, shape, dim)


def _nt(a, b):
    return lax.dot_general(a, b, (((1,), (1,)), ((), ())), preferred_element_type=f32)


def _nn(a, b):
    return lax.dot_general(a, b, (((1,), (0,)), ((), ())), preferred_element_type=f32)


def _unpack(u, idx):
    return pltpu.unpack_elementwise(u, index=idx, packed_dtype=bf16, unpacked_dtype=f32)


def _packi(a, b):
    return pltpu.pack_elementwise([a, b], packed_dtype=bf16)


def _b(u):
    return pltpu.bitcast(u, bf16)


def _u(b):
    return pltpu.bitcast(b, u32)


VSTRIPS = [(pc, j, pc) for j in range(NS) for pc in range(2)] + [(1, 0, 0), (0, NS - 1, 1)]


def _kernel(x_ref, wqkv_ref, wo_ref, out_ref,
            a_ref, bt_ref, aug0_ref, aug1_ref, ulast_ref, x2_ref, q2_ref, c_ref, ow_ref):
    s = pl.program_id(0)
    sub8 = _iota((8, 128), 0)
    lane8 = _iota((8, 128), 1)
    pad_word = jnp.where(lane8 == L_PAD, jnp.uint32(ONE2), jnp.uint32(0))
    lo4 = sub8 < 4

    def _setup():
        wq = wqkv_ref[:, 0:C]
        wk = wqkv_ref[:, C:2 * C]
        wv = wqkv_ref[:, 2 * C:3 * C]
        a = _nt(wq, wk) * (C ** -0.5 * math.log2(math.e))
        a = jnp.concatenate([a, jnp.zeros((C, 128 - C), f32)], axis=1)
        a = jnp.concatenate([a, jnp.zeros((128 - C, 128), f32)], axis=0)
        r = _iota((128, 128), 0)
        c = _iota((128, 128), 1)
        rowm = (r >= L_ROW) & (r < L_COL) & (c >= L_ROW) & (c < L_COL) & (((c - r + 3 + RM) % RM) > 6)
        colm = (r >= L_COL) & (r < L_ONE) & (c >= L_COL) & (c < L_ONE) & (((c - r + 3 + CM) % CM) > 6)
        padm = (r == L_ONE) & (c == L_PAD)
        a_ref[...] = _u(jnp.where(rowm | colm | padm, -BIG, a).astype(bf16))
        b = _nn(wv, wo_ref[...])
        bt = jnp.concatenate([b.T, jnp.zeros((C, 128 - C), f32)], axis=1)
        bt = jnp.concatenate([bt, jnp.zeros((112 - C, 128), f32)], axis=0)
        r = _iota((112, 128), 0)
        c = _iota((112, 128), 1)
        bt_ref[...] = _u(jnp.where((r == C) & (c == L_ONE), 1.0, bt).astype(bf16))
        sl = _iota((16, 128), 0)
        ln = _iota((16, 128), 1)
        for m in range(3):
            cres = ((m * 128 + ln) // 2) % CM

            def val(rho):
                return ((rho >= 14) & (rho < 29) & (rho - 14 == cres)) | (rho == 29)
            lo = jnp.where(val(2 * sl), jnp.uint32(0x3F80), jnp.uint32(0))
            hi = jnp.where(val(2 * sl + 1), jnp.uint32(0x3F800000), jnp.uint32(0))
            w = lo | hi
            aug1_ref[m] = w[8:16]
            for rho in range(RM):
                rw = jnp.where(sub8 == rho // 2, jnp.uint32(0x3F80 if rho % 2 == 0 else 0x3F800000), jnp.uint32(0))
                aug0_ref[m, rho] = w[0:8] | rw
        for pr in range(2):
            for u in range(NS):
                ulast_ref[pr, u] = pad_word
            for pc in range(2):
                for p in range(2):
                    for g in range(NG):
                        x2_ref[0, pr, pc, p, g] = pad_word
        q2_ref[NB] = jnp.zeros(q2_ref.shape[1:], u32)

    pl.when(s == 0)(_setup)

    colpatch_lane = (lane8 >= L_COL) & (lane8 < L_ONE)
    m_first = colpatch_lane & (sub8 < 3)
    m_last = colpatch_lane & (sub8 >= 5)
    p_first = jnp.where(lane8 == L_COL + (3 % CM), 1.0, 0.0)
    p_last = jnp.where(lane8 == L_COL + (188 % CM), 1.0, 0.0)

    bnd = {}

    def pre_unit(xw, qw, pr, k, m):
        uss = []
        for il in (2 * k, 2 * k + 1):
            h = 2 * il + pr
            rho = (8 * s + il) % RM
            xt = x_ref[h, :, m * 128:(m + 1) * 128]
            aug = jnp.concatenate([aug0_ref[m, rho], aug1_ref[m]], axis=0)
            full = jnp.concatenate([xt, _b(aug)], axis=0)
            uw = _u(full.T)
            uss.append([uw[8 * v:8 * v + 8] for v in range(8)])
        xs = xw(0, 2 + k) if k < 2 else xw(1, k - 2)
        parts = [[], []]
        for v in range(8):
            u = 8 * m + v
            prev = ulast_ref[pr, u]
            ulast_ref[pr, u] = uss[1][v]
            for pc in range(2):
                ea = _unpack(uss[0][v], pc)
                eb = _unpack(uss[1][v], pc)
                ep = _unpack(prev, pc)
                rolled = pltpu.roll(_packi(ep, ea), 4, 0)
                left = pad_word if u == 0 else bnd[(pr, k, pc)]
                xs(pr, pc, u, jnp.where(lo4, left, rolled))
                bnd[(pr, k, pc)] = rolled
                if u == NS - 1:
                    xs(pr, pc, NS, jnp.where(lo4, rolled, pad_word))
                if u == 0:
                    ea = jnp.where(m_first, p_first, ea)
                    eb = jnp.where(m_first, p_first, eb)
                if u == NS - 1:
                    ea = jnp.where(m_last, p_last, ea)
                    eb = jnp.where(m_last, p_last, eb)
                parts[pc] += [ea, eb]
        for pc in range(2):
            lp = jnp.concatenate(parts[pc], axis=0).astype(bf16)
            q = _nn(lp, _b(a_ref[...]))
            for v in range(8):
                qw(pr, pc, 8 * m + v, k, _packi(q[16 * v:16 * v + 8], q[16 * v + 8:16 * v + 16]))

    PRE_UNITS = [(pr, k, m) for pr in range(2) for k in range(4) for m in range(3)]

    def out_unit(h, m):
        pr = h % 2
        i = h // 2
        w = _b(jnp.concatenate([ow_ref[pr, i // 2, 8 * m + v, pl.ds(i % 2, 8, stride=2), :] for v in range(8)], axis=0))
        r = _nt(_b(bt_ref[...]), w)
        inv = 1.0 / r[C:C + 1]
        out_ref[h, :, m * 128:(m + 1) * 128] = (r[0:C] * inv).astype(bf16)

    OUT_UNITS = [(h, m) for h in range(16) for m in range(3)]

    def colidx(n):
        r = _iota((n, 128), 0)
        return 4 * ((r // 8) % 2) + (r % 8) // 2

    def attn_stage(with_pre, with_out):
        xv = x2_ref.at[pl.ds(s - 2, 4 if with_pre else 2)]
        qv = q2_ref.at[pl.ds(s - 2, 3 if with_pre else 2)]

        def keytile(slot, pr, pck, j):
            return _b(xv[slot, pr, pck, :, j:j + 2].reshape(64, 128))

        def xw(o, p):
            def st(pr, pc, u, val):
                xv[2 + o, pr, pc, p, u] = val
            return st

        def qw(pr, pc, u, k, val):
            qv[2, pr, pc, u, k] = val

        tiles = []
        for pr in range(2):
            order = [2 * NS, 2 * NS + 1] + list(range(2 * NS))
            tiles += [(pr, vi) for vi in order]
        nt = len(tiles)
        col = colidx(64)
        sl = _iota((48, 128), 0)
        ln = _iota((48, 128), 1)
        irow = jnp.maximum(2 * (sl // 16) + sl % 2, jnp.where(s == 2, 3, 0))
        pos = 2 * (ln // 32) + ln % 2
        mnew = pos <= irow
        pvals = {}
        res = {}

        def qk(pr, vi):
            pcq, j, pck = VSTRIPS[vi]
            l = _b(jnp.concatenate([qv[0, pr, pcq, j].reshape(32, 128),
                                    qv[1, pr, pcq, j, 0:3].reshape(24, 128)], axis=0))
            sc = _nt(l, keytile(1, pr, pck, j))
            cp = c_ref[pr, vi]
            comb = jnp.concatenate([jnp.maximum(cp, sc[0:48]), sc[48:64]], axis=0)
            c_ref[pr, vi] = sc[64:112]
            m = jnp.max(comb, axis=1, keepdims=True)
            e = jnp.exp2(comb - m)
            pn = jnp.concatenate([jnp.where(mnew, e[0:48], 0.0), e[48:64]], axis=0).astype(bf16)
            po = jnp.where(mnew, 0.0, e[0:48]).astype(bf16)
            pvals[(pr, vi)] = (pn, po)

        def pv(pr, vi):
            pcq, j, pck = VSTRIPS[vi]
            pn, po = pvals.pop((pr, vi))
            o = _nn(pn, keytile(1, pr, pck, j))
            oa = _nn(po, keytile(0, pr, pck, j))
            res[(pr, vi)] = jnp.concatenate([o[0:48] + oa, o[48:64]], axis=0)
            if vi < 2 * NS and vi % 2 == 1:
                j = vi // 2
                o0 = res.pop((pr, vi - 1))
                o1 = res.pop((pr, vi))
                if j == 0:
                    o1 = jnp.where(col < 3, res.pop((pr, 2 * NS)), o1)
                if j == NS - 1:
                    o0 = jnp.where(col >= 5, res.pop((pr, 2 * NS + 1)), o0)
                ow_ref[pr, :, j] = _packi(o0, o1).reshape(4, 16, 128)

        extra = {}
        if with_out:
            for pr in range(2):
                for m in range(3):
                    ready = pr * 50 + 2 + 16 * (m + 1) - 1 + D
                    for i in range(8):
                        extra.setdefault(ready + E + 2 * i, []).append(('o', 2 * i + pr, m))
        if with_pre:
            npre = len(PRE_UNITS) - NTAIL
            for n, un in enumerate(PRE_UNITS[:npre]):
                extra.setdefault((n * nt) // npre, []).append(('p',) + un)
            last = nt + D
            for n, un in enumerate(PRE_UNITS[npre:]):
                extra.setdefault(last - 1 + 2 * n, []).append(('p',) + un)
        nslot = max([nt + D] + [k + 1 for k in extra])
        for n in range(nslot):
            if n < nt:
                qk(*tiles[n])
            if D <= n < nt + D:
                pv(*tiles[n - D])
            for e in extra.get(n, []):
                if e[0] == 'o':
                    out_unit(e[1], e[2])
                else:
                    pre_unit(xw, qw, *e[1:])

    def patch_rows(slot, qp, halves, center):
        inrow = (lane8 >= L_ROW) & (lane8 < L_COL)
        off = ((lane8 - L_ROW - (center % RM) + 3 + RM) % RM) > 6
        hm = sum(0xFFFF << (16 * hf) for hf in halves)
        keep = jnp.where(inrow, jnp.uint32(0xFFFFFFFF ^ hm), jnp.uint32(0xFFFFFFFF))
        pat = jnp.where(inrow & off, jnp.uint32((NBIG_BITS * 0x10001) & hm), jnp.uint32(0))
        for pr in range(2):
            for pc in range(2):
                for j in range(NS):
                    q2_ref[slot, pr, pc, j, qp] = (q2_ref[slot, pr, pc, j, qp] & keep) | pat

    def fixup(pr_q, qslot, qp0, keyfn, full, part, part_half):
        tiles = [(1, 0, 0), (0, NS - 1, 1)] + [(pc, j, pc) for j in range(NS) for pc in range(2)]
        sv = {}
        res = {}
        col = colidx(32)
        keepnew = (_iota((16, 128), 0) % 2) == part_half

        def qk(n):
            pcq, j, pck = tiles[n]
            l = _b(q2_ref[qslot, pr_q, pcq, j, qp0:qp0 + 2].reshape(16, 128))
            sv[n] = _nt(l, keyfn(pck, j))

        def pv(n):
            pcq, j, pck = tiles[n]
            sc = sv.pop(n)
            m = jnp.max(sc, axis=1, keepdims=True)
            p = jnp.exp2(sc - m).astype(bf16)
            res[n] = _nn(p, keyfn(pck, j))
            if n >= 2 and n % 2 == 1:
                o0 = res.pop(n - 1)
                o1 = res.pop(n)
                if j == 0:
                    o1 = jnp.where(col < 3, res.pop(0), o1)
                if j == NS - 1:
                    o0 = jnp.where(col >= 5, res.pop(1), o0)
                w = _packi(o0, o1)
                ow_ref[pr_q, qp0 + full, j] = w[16 * full:16 * full + 16]
                ow_ref[pr_q, qp0 + part, j] = jnp.where(keepnew, w[16 * part:16 * part + 16],
                                                        ow_ref[pr_q, qp0 + part, j])
        DF = 10
        for n in range(len(tiles) + DF):
            if n < len(tiles):
                qk(n)
            if n >= DF:
                pv(n - DF)

    @pl.when(s <= 2)
    def _():
        xv = x2_ref.at[pl.ds(s, 2)]
        qv = q2_ref.at[pl.ds(s, 1)]

        def xw(o, p):
            def st(pr, pc, u, val):
                xv[o, pr, pc, p, u] = val
            return st

        def qw(pr, pc, u, k, val):
            qv[0, pr, pc, u, k] = val
        for u in PRE_UNITS:
            pre_unit(xw, qw, *u)

    @pl.when(s == 0)
    def _():
        patch_rows(0, 0, (0, 1), 3)
        patch_rows(0, 1, (0,), 3)

    @pl.when(s == 1)
    def _conly():
        for pr in range(2):
            for vi, (pcq, j, pck) in enumerate(VSTRIPS):
                l = _b(q2_ref[0, pr, pcq, j, 0:3].reshape(24, 128))
                c_ref[pr, vi] = _nt(l, _b(x2_ref[0, pr, pck, :, j:j + 2].reshape(64, 128)))

    @pl.when((s >= 3) & (s < NB))
    def _():
        attn_stage(True, True)

    @pl.when(s == NB - 1)
    def _():
        patch_rows(NB - 1, 2, (1,), 188)
        patch_rows(NB - 1, 3, (0, 1), 188)

    @pl.when(s == NB)
    def _tail_pairs():
        for pr in range(2):
            for pc in range(2):
                left = pad_word
                for u in range(NS):
                    ep = _unpack(ulast_ref[pr, u], pc)
                    rolled = pltpu.roll(_packi(ep, _unpack(pad_word, pc)), 4, 0)
                    x2_ref[NB, pr, pc, 2, u] = jnp.where(lo4, left, rolled)
                    left = rolled
                x2_ref[NB, pr, pc, 2, NS] = jnp.where(lo4, left, pad_word)
                for g in range(NG):
                    x2_ref[NB, pr, pc, 3, g] = pad_word

    @pl.when((s == 2) | (s >= NB))
    def _():
        attn_stage(False, False)

    @pl.when(s == 2)
    def _():
        def keyfn(pck, j):
            return _b(jnp.concatenate([x2_ref[0, 0, pck, 2:4, j:j + 2].reshape(32, 128),
                                       x2_ref[1, 0, pck, 0:2, j:j + 2].reshape(32, 128)], axis=0))
        fixup(1, 0, 0, keyfn, 0, 1, 0)

    @pl.when(s == NB + 1)
    def _():
        def keyfn(pck, j):
            return _b(jnp.concatenate([x2_ref[NB - 1, 1, pck, 3:4, j:j + 2].reshape(16, 128),
                                       x2_ref[NB, 1, pck, 0:3, j:j + 2].reshape(48, 128)], axis=0))
        fixup(0, NB - 1, 2, keyfn, 1, 0, 1)
        fixup(1, NB - 1, 2, keyfn, 1, 0, 1)

    @pl.when((s == 2) | (s >= NB))
    def _():
        for h, m in OUT_UNITS:
            out_unit(h, m)


@jax.jit
def pallas_standalone__neighborhood_nat__vision_kernel(x, wqkv, wo):
    xt = jnp.transpose(x.reshape(H, W, C), (0, 2, 1))
    out = pl.pallas_call(
        _kernel,
        grid=(NB + 2,),
        in_specs=[
            pl.BlockSpec((16, C, W), lambda s: (jnp.minimum(s, NB - 1), 0, 0)),
            pl.BlockSpec((C, 3 * C), lambda s: (0, 0)),
            pl.BlockSpec((C, C), lambda s: (0, 0)),
        ],
        out_specs=pl.BlockSpec((16, C, W), lambda s: (jnp.clip(s - 2, 0, NB - 1), 0, 0)),
        out_shape=jax.ShapeDtypeStruct((H, C, W), bf16),
        scratch_shapes=[
            pltpu.VMEM((64, 128), u32),
            pltpu.VMEM((56, 128), u32),
            pltpu.VMEM((3, RM, 8, 128), u32),
            pltpu.VMEM((3, 8, 128), u32),
            pltpu.VMEM((2, NS, 8, 128), u32),
            pltpu.VMEM((NB + 1, 2, 2, 4, NG, 8, 128), u32),
            pltpu.VMEM((NB + 1, 2, 2, NS, 4, 8, 128), u32),
            pltpu.VMEM((2, 2 * NS + 2, 48, 128), f32),
            pltpu.VMEM((2, 4, NS, 16, 128), u32),
        ],
        compiler_params=pltpu.CompilerParams(
            dimension_semantics=("arbitrary",), vmem_limit_bytes=110 * 1024 * 1024),
        name="nat_kernel",
    )(xt, wqkv, wo)
    return jnp.transpose(out, (0, 2, 1)).reshape(1, H, W, C)
```

```python
import math

import jax
import jax.numpy as jnp
from jax import lax
from jax.experimental import pallas as pl
from jax.experimental.pallas import tpu as pltpu

H = 384
W = 384
C = 96
NB = 24
NS = 24
NG = 25
BIG = 2.0 ** 100
ONE2 = 0x3F803F80
RM = 14
CM = 15
L_ROW = 96
L_COL = 110
L_ONE = 125
L_PAD = 126
NBIG_BITS = 0xF180
D = 8
E = 8
NTAIL = 9
POFF = 6

bf16 = jnp.bfloat16
f32 = jnp.float32
u32 = jnp.uint32
i32 = jnp.int32


def _iota(shape, dim):
    return lax.broadcasted_iota(i32, shape, dim)


def _nt(a, b):
    return lax.dot_general(a, b, (((1,), (1,)), ((), ())), preferred_element_type=f32)


def _nn(a, b):
    return lax.dot_general(a, b, (((1,), (0,)), ((), ())), preferred_element_type=f32)


def _unpack(u, idx):
    return pltpu.unpack_elementwise(u, index=idx, packed_dtype=bf16, unpacked_dtype=f32)


def _packi(a, b):
    return pltpu.pack_elementwise([a, b], packed_dtype=bf16)


def _b(u):
    return pltpu.bitcast(u, bf16)


def _u(b):
    return pltpu.bitcast(b, u32)


VSTRIPS = [(pc, j, pc) for j in range(NS) for pc in range(2)] + [(1, 0, 0), (0, NS - 1, 1)]


def _kernel(x_ref, wqkv_ref, wo_ref, out_ref,
            a_ref, bt_ref, aug0_ref, aug1_ref, ulast_ref, x2_ref, q2_ref, c_ref, ow_ref):
    s = pl.program_id(0)
    sub8 = _iota((8, 128), 0)
    lane8 = _iota((8, 128), 1)
    pad_word = jnp.where(lane8 == L_PAD, jnp.uint32(ONE2), jnp.uint32(0))
    lo4 = sub8 < 4

    def _setup():
        wq = wqkv_ref[:, 0:C]
        wk = wqkv_ref[:, C:2 * C]
        wv = wqkv_ref[:, 2 * C:3 * C]
        a = _nt(wq, wk) * (C ** -0.5 * math.log2(math.e))
        a = jnp.concatenate([a, jnp.zeros((C, 128 - C), f32)], axis=1)
        a = jnp.concatenate([a, jnp.zeros((128 - C, 128), f32)], axis=0)
        r = _iota((128, 128), 0)
        c = _iota((128, 128), 1)
        rowm = (r >= L_ROW) & (r < L_COL) & (c >= L_ROW) & (c < L_COL) & (((c - r + 3 + RM) % RM) > 6)
        colm = (r >= L_COL) & (r < L_ONE) & (c >= L_COL) & (c < L_ONE) & (((c - r + 3 + CM) % CM) > 6)
        padm = (r == L_ONE) & (c == L_PAD)
        a_ref[...] = _u(jnp.where(rowm | colm | padm, -BIG, a).astype(bf16))
        b = _nn(wv, wo_ref[...])
        bt = jnp.concatenate([b.T, jnp.zeros((C, 128 - C), f32)], axis=1)
        bt = jnp.concatenate([bt, jnp.zeros((112 - C, 128), f32)], axis=0)
        r = _iota((112, 128), 0)
        c = _iota((112, 128), 1)
        bt_ref[...] = _u(jnp.where((r == C) & (c == L_ONE), 1.0, bt).astype(bf16))
        sl = _iota((16, 128), 0)
        ln = _iota((16, 128), 1)
        for m in range(3):
            cres = ((m * 128 + ln) // 2) % CM

            def val(rho):
                return ((rho >= 14) & (rho < 29) & (rho - 14 == cres)) | (rho == 29)
            lo = jnp.where(val(2 * sl), jnp.uint32(0x3F80), jnp.uint32(0))
            hi = jnp.where(val(2 * sl + 1), jnp.uint32(0x3F800000), jnp.uint32(0))
            w = lo | hi
            aug1_ref[m] = w[8:16]
            for rho in range(RM):
                rw = jnp.where(sub8 == rho // 2, jnp.uint32(0x3F80 if rho % 2 == 0 else 0x3F800000), jnp.uint32(0))
                aug0_ref[m, rho] = w[0:8] | rw
        for pr in range(2):
            for u in range(NS):
                ulast_ref[pr, u] = pad_word
            for pc in range(2):
                for p in range(2):
                    for g in range(NG):
                        x2_ref[0, pr, pc, p, g] = pad_word
        q2_ref[NB] = jnp.zeros(q2_ref.shape[1:], u32)

    pl.when(s == 0)(_setup)

    colpatch_lane = (lane8 >= L_COL) & (lane8 < L_ONE)
    m_first = colpatch_lane & (sub8 < 3)
    m_last = colpatch_lane & (sub8 >= 5)
    p_first = jnp.where(lane8 == L_COL + (3 % CM), 1.0, 0.0)
    p_last = jnp.where(lane8 == L_COL + (188 % CM), 1.0, 0.0)

    bnd = {}

    def pre_unit(xw, qw, pr, k, m):
        uss = []
        for il in (2 * k, 2 * k + 1):
            h = 2 * il + pr
            rho = (8 * s + il) % RM
            xt = x_ref[h, :, m * 128:(m + 1) * 128]
            aug = jnp.concatenate([aug0_ref[m, rho], aug1_ref[m]], axis=0)
            full = jnp.concatenate([xt, _b(aug)], axis=0)
            uw = _u(full.T)
            uss.append([uw[8 * v:8 * v + 8] for v in range(8)])
        xs = xw(0, 2 + k) if k < 2 else xw(1, k - 2)
        parts = [[], []]
        for v in range(8):
            u = 8 * m + v
            prev = ulast_ref[pr, u]
            ulast_ref[pr, u] = uss[1][v]
            for pc in range(2):
                ea = _unpack(uss[0][v], pc)
                eb = _unpack(uss[1][v], pc)
                ep = _unpack(prev, pc)
                rolled = pltpu.roll(_packi(ep, ea), 4, 0)
                left = pad_word if u == 0 else bnd[(pr, k, pc)]
                xs(pr, pc, u, jnp.where(lo4, left, rolled))
                bnd[(pr, k, pc)] = rolled
                if u == NS - 1:
                    xs(pr, pc, NS, jnp.where(lo4, rolled, pad_word))
                if u == 0:
                    ea = jnp.where(m_first, p_first, ea)
                    eb = jnp.where(m_first, p_first, eb)
                if u == NS - 1:
                    ea = jnp.where(m_last, p_last, ea)
                    eb = jnp.where(m_last, p_last, eb)
                parts[pc] += [ea, eb]
        for pc in range(2):
            lp = jnp.concatenate(parts[pc], axis=0).astype(bf16)
            q = _nn(lp, _b(a_ref[...]))
            for v in range(8):
                qw(pr, pc, 8 * m + v, k, _packi(q[16 * v:16 * v + 8], q[16 * v + 8:16 * v + 16]))

    PRE_UNITS = [(pr, k, m) for pr in range(2) for k in range(4) for m in range(3)]

    def out_unit(h, m):
        pr = h % 2
        i = h // 2
        w = _b(jnp.concatenate([ow_ref[pr, i // 2, 8 * m + v, pl.ds(i % 2, 8, stride=2), :] for v in range(8)], axis=0))
        r = _nt(_b(bt_ref[...]), w)
        inv = 1.0 / r[C:C + 1]
        out_ref[h, :, m * 128:(m + 1) * 128] = (r[0:C] * inv).astype(bf16)

    OUT_UNITS = [(h, m) for h in range(16) for m in range(3)]

    def colidx(n):
        r = _iota((n, 128), 0)
        return 4 * ((r // 8) % 2) + (r % 8) // 2

    def attn_stage(with_pre, with_out):
        xv = x2_ref.at[pl.ds(s - 2, 4 if with_pre else 2)]
        qv = q2_ref.at[pl.ds(s - 2, 3 if with_pre else 2)]

        def keytile(slot, pr, pck, j):
            return _b(xv[slot, pr, pck, :, j:j + 2].reshape(64, 128))

        def xw(o, p):
            def st(pr, pc, u, val):
                xv[2 + o, pr, pc, p, u] = val
            return st

        def qw(pr, pc, u, k, val):
            qv[2, pr, pc, u, k] = val

        tiles = []
        for pr in range(2):
            order = [2 * NS, 2 * NS + 1] + list(range(2 * NS))
            tiles += [(pr, vi) for vi in order]
        nt = len(tiles)
        col = colidx(64)
        sl = _iota((48, 128), 0)
        ln = _iota((48, 128), 1)
        irow = jnp.maximum(2 * (sl // 16) + sl % 2, jnp.where(s == 2, 3, 0))
        pos = 2 * (ln // 32) + ln % 2
        mnew = pos <= irow
        pvals = {}
        res = {}

        def qk(pr, vi):
            pcq, j, pck = VSTRIPS[vi]
            l = _b(jnp.concatenate([qv[0, pr, pcq, j].reshape(32, 128),
                                    qv[1, pr, pcq, j, 0:3].reshape(24, 128)], axis=0))
            sc = _nt(l, keytile(1, pr, pck, j))
            cp = c_ref[pr, vi]
            comb = jnp.concatenate([jnp.maximum(cp, sc[0:48]), sc[48:64]], axis=0)
            c_ref[pr, vi] = sc[64:112]
            m = jnp.max(comb, axis=1, keepdims=True)
            e = jnp.exp2(comb - m)
            pn = jnp.concatenate([jnp.where(mnew, e[0:48], 0.0), e[48:64]], axis=0).astype(bf16)
            po = jnp.where(mnew, 0.0, e[0:48]).astype(bf16)
            pvals[(pr, vi)] = (pn, po)

        def pv(pr, vi):
            pcq, j, pck = VSTRIPS[vi]
            pn, po = pvals.pop((pr, vi))
            o = _nn(pn, keytile(1, pr, pck, j))
            oa = _nn(po, keytile(0, pr, pck, j))
            res[(pr, vi)] = jnp.concatenate([o[0:48] + oa, o[48:64]], axis=0)
            if vi < 2 * NS and vi % 2 == 1:
                j = vi // 2
                o0 = res.pop((pr, vi - 1))
                o1 = res.pop((pr, vi))
                if j == 0:
                    o1 = jnp.where(col < 3, res.pop((pr, 2 * NS)), o1)
                if j == NS - 1:
                    o0 = jnp.where(col >= 5, res.pop((pr, 2 * NS + 1)), o0)
                ow_ref[pr, :, j] = _packi(o0, o1).reshape(4, 16, 128)

        extra = {}
        if with_out:
            for pr in range(2):
                for m in range(3):
                    ready = pr * 50 + 2 + 16 * (m + 1) - 1 + D
                    for i in range(8):
                        extra.setdefault(ready + E + 2 * i, []).append(('o', 2 * i + pr, m))
        if with_pre:
            npre = len(PRE_UNITS) - NTAIL
            for n, un in enumerate(PRE_UNITS[:npre]):
                extra.setdefault(POFF + (n * (nt - POFF)) // npre, []).append(('p',) + un)
            last = nt + D
            for n, un in enumerate(PRE_UNITS[npre:]):
                extra.setdefault(last - 1 + 2 * n, []).append(('p',) + un)
        nslot = max([nt + D] + [k + 1 for k in extra])
        for n in range(nslot):
            if n < nt:
                qk(*tiles[n])
            if D <= n < nt + D:
                pv(*tiles[n - D])
            for e in extra.get(n, []):
                if e[0] == 'o':
                    out_unit(e[1], e[2])
                else:
                    pre_unit(xw, qw, *e[1:])

    def patch_rows(slot, qp, halves, center):
        inrow = (lane8 >= L_ROW) & (lane8 < L_COL)
        off = ((lane8 - L_ROW - (center % RM) + 3 + RM) % RM) > 6
        hm = sum(0xFFFF << (16 * hf) for hf in halves)
        keep = jnp.where(inrow, jnp.uint32(0xFFFFFFFF ^ hm), jnp.uint32(0xFFFFFFFF))
        pat = jnp.where(inrow & off, jnp.uint32((NBIG_BITS * 0x10001) & hm), jnp.uint32(0))
        for pr in range(2):
            for pc in range(2):
                for j in range(NS):
                    q2_ref[slot, pr, pc, j, qp] = (q2_ref[slot, pr, pc, j, qp] & keep) | pat

    def fixup(pr_q, qslot, qp0, keyfn, full, part, part_half):
        tiles = [(1, 0, 0), (0, NS - 1, 1)] + [(pc, j, pc) for j in range(NS) for pc in range(2)]
        sv = {}
        res = {}
        col = colidx(32)
        keepnew = (_iota((16, 128), 0) % 2) == part_half

        def qk(n):
            pcq, j, pck = tiles[n]
            l = _b(q2_ref[qslot, pr_q, pcq, j, qp0:qp0 + 2].reshape(16, 128))
            sv[n] = _nt(l, keyfn(pck, j))

        def pv(n):
            pcq, j, pck = tiles[n]
            sc = sv.pop(n)
            m = jnp.max(sc, axis=1, keepdims=True)
            p = jnp.exp2(sc - m).astype(bf16)
            res[n] = _nn(p, keyfn(pck, j))
            if n >= 2 and n % 2 == 1:
                o0 = res.pop(n - 1)
                o1 = res.pop(n)
                if j == 0:
                    o1 = jnp.where(col < 3, res.pop(0), o1)
                if j == NS - 1:
                    o0 = jnp.where(col >= 5, res.pop(1), o0)
                w = _packi(o0, o1)
                ow_ref[pr_q, qp0 + full, j] = w[16 * full:16 * full + 16]
                ow_ref[pr_q, qp0 + part, j] = jnp.where(keepnew, w[16 * part:16 * part + 16],
                                                        ow_ref[pr_q, qp0 + part, j])
        DF = 10
        for n in range(len(tiles) + DF):
            if n < len(tiles):
                qk(n)
            if n >= DF:
                pv(n - DF)

    @pl.when(s <= 2)
    def _():
        xv = x2_ref.at[pl.ds(s, 2)]
        qv = q2_ref.at[pl.ds(s, 1)]

        def xw(o, p):
            def st(pr, pc, u, val):
                xv[o, pr, pc, p, u] = val
            return st

        def qw(pr, pc, u, k, val):
            qv[0, pr, pc, u, k] = val
        for u in PRE_UNITS:
            pre_unit(xw, qw, *u)

    @pl.when(s == 0)
    def _():
        patch_rows(0, 0, (0, 1), 3)
        patch_rows(0, 1, (0,), 3)

    @pl.when(s == 1)
    def _conly():
        for pr in range(2):
            for vi, (pcq, j, pck) in enumerate(VSTRIPS):
                l = _b(q2_ref[0, pr, pcq, j, 0:3].reshape(24, 128))
                c_ref[pr, vi] = _nt(l, _b(x2_ref[0, pr, pck, :, j:j + 2].reshape(64, 128)))

    @pl.when((s >= 3) & (s < NB))
    def _():
        attn_stage(True, True)

    @pl.when(s == NB - 1)
    def _():
        patch_rows(NB - 1, 2, (1,), 188)
        patch_rows(NB - 1, 3, (0, 1), 188)

    @pl.when(s == NB)
    def _tail_pairs():
        for pr in range(2):
            for pc in range(2):
                left = pad_word
                for u in range(NS):
                    ep = _unpack(ulast_ref[pr, u], pc)
                    rolled = pltpu.roll(_packi(ep, _unpack(pad_word, pc)), 4, 0)
                    x2_ref[NB, pr, pc, 2, u] = jnp.where(lo4, left, rolled)
                    left = rolled
                x2_ref[NB, pr, pc, 2, NS] = jnp.where(lo4, left, pad_word)
                for g in range(NG):
                    x2_ref[NB, pr, pc, 3, g] = pad_word

    @pl.when((s == 2) | (s >= NB))
    def _():
        attn_stage(False, False)

    @pl.when(s == 2)
    def _():
        def keyfn(pck, j):
            return _b(jnp.concatenate([x2_ref[0, 0, pck, 2:4, j:j + 2].reshape(32, 128),
                                       x2_ref[1, 0, pck, 0:2, j:j + 2].reshape(32, 128)], axis=0))
        fixup(1, 0, 0, keyfn, 0, 1, 0)

    @pl.when(s == NB + 1)
    def _():
        def keyfn(pck, j):
            return _b(jnp.concatenate([x2_ref[NB - 1, 1, pck, 3:4, j:j + 2].reshape(16, 128),
                                       x2_ref[NB, 1, pck, 0:3, j:j + 2].reshape(48, 128)], axis=0))
        fixup(0, NB - 1, 2, keyfn, 1, 0, 1)
        fixup(1, NB - 1, 2, keyfn, 1, 0, 1)

    @pl.when((s == 2) | (s >= NB))
    def _():
        for h, m in OUT_UNITS:
            out_unit(h, m)


@jax.jit
def pallas_standalone__neighborhood_nat__vision_kernel(x, wqkv, wo):
    xt = jnp.transpose(x.reshape(H, W, C), (0, 2, 1))
    out = pl.pallas_call(
        _kernel,
        grid=(NB + 2,),
        in_specs=[
            pl.BlockSpec((16, C, W), lambda s: (jnp.minimum(s, NB - 1), 0, 0)),
            pl.BlockSpec((C, 3 * C), lambda s: (0, 0)),
            pl.BlockSpec((C, C), lambda s: (0, 0)),
        ],
        out_specs=pl.BlockSpec((16, C, W), lambda s: (jnp.clip(s - 2, 0, NB - 1), 0, 0)),
        out_shape=jax.ShapeDtypeStruct((H, C, W), bf16),
        scratch_shapes=[
            pltpu.VMEM((64, 128), u32),
            pltpu.VMEM((56, 128), u32),
            pltpu.VMEM((3, RM, 8, 128), u32),
            pltpu.VMEM((3, 8, 128), u32),
            pltpu.VMEM((2, NS, 8, 128), u32),
            pltpu.VMEM((NB + 1, 2, 2, 4, NG, 8, 128), u32),
            pltpu.VMEM((NB + 1, 2, 2, NS, 4, 8, 128), u32),
            pltpu.VMEM((2, 2 * NS + 2, 48, 128), f32),
            pltpu.VMEM((2, 4, NS, 16, 128), u32),
        ],
        compiler_params=pltpu.CompilerParams(
            dimension_semantics=("arbitrary",), vmem_limit_bytes=110 * 1024 * 1024),
        name="nat_kernel",
    )(xt, wqkv, wo)
    return jnp.transpose(out, (0, 2, 1)).reshape(1, H, W, C)
```

```python
import math

import jax
import jax.numpy as jnp
from jax import lax
from jax.experimental import pallas as pl
from jax.experimental.pallas import tpu as pltpu

H = 384
W = 384
C = 96
NB = 24
NS = 24
NG = 25
NGX = NG + 2
BIG = 2.0 ** 100
ONE2 = 0x3F803F80
NBIG = 0xF180
RM = 14
CM = 15
L_ROW = 96
L_COL = 110
L_ONE = 125
L_PAD = 126
D = 7
E = 8
NTAIL = 2
POFF = 6
NFILL = 4
PEND = 0
FK = 14

bf16 = jnp.bfloat16
f32 = jnp.float32
u32 = jnp.uint32
i32 = jnp.int32


def _iota(shape, dim):
    return lax.broadcasted_iota(i32, shape, dim)


def _nt(a, b):
    return lax.dot_general(a, b, (((1,), (1,)), ((), ())), preferred_element_type=f32)


def _nn(a, b):
    return lax.dot_general(a, b, (((1,), (0,)), ((), ())), preferred_element_type=f32)


def _unpack(u, idx):
    return pltpu.unpack_elementwise(u, index=idx, packed_dtype=bf16, unpacked_dtype=f32)


def _packi(a, b):
    return pltpu.pack_elementwise([a, b], packed_dtype=bf16)


def _b(u):
    return pltpu.bitcast(u, bf16)


def _u(b):
    return pltpu.bitcast(b, u32)


def _halves(a, b, idx):
    return _packi(_unpack(a, idx), _unpack(b, idx))


VSTRIPS = [(pc, j, pc, j) for j in range(NS) for pc in range(2)] + [(0, NS, 0, NG)]
NV = len(VSTRIPS)


def _kernel(x_ref, wqkv_ref, wo_ref, out_ref,
            at_ref, bt_ref, aug0_ref, aug1_ref, qaug0_ref, qaug1_ref, ulast_ref, x2_ref, q2_ref, c_ref, ow_ref, flag_ref):
    s = pl.program_id(0)
    sub8 = _iota((8, 128), 0)
    lane8 = _iota((8, 128), 1)
    pad_word = jnp.where(lane8 == L_PAD, jnp.uint32(ONE2), jnp.uint32(0))
    lo4 = sub8 < 4

    def _setup():
        wq = wqkv_ref[:, 0:C]
        wk = wqkv_ref[:, C:2 * C]
        wv = wqkv_ref[:, 2 * C:3 * C]
        at = _nt(wk, wq) * (C ** -0.5 * math.log2(math.e))
        at = jnp.concatenate([at, jnp.zeros((C, 128 - C), f32)], axis=1)
        at_ref[...] = _u(at.astype(bf16))
        b = _nn(wv, wo_ref[...])
        bt = jnp.concatenate([b.T, jnp.zeros((C, 128 - C), f32)], axis=1)
        bt = jnp.concatenate([bt, jnp.zeros((112 - C, 128), f32)], axis=0)
        r = _iota((112, 128), 0)
        c = _iota((112, 128), 1)
        bt_ref[...] = _u(jnp.where((r == C) & (c == L_ONE), 1.0, bt).astype(bf16))
        sl = _iota((16, 128), 0)
        ln = _iota((16, 128), 1)

        def words(val, bits):
            lo = jnp.where(val(2 * sl), jnp.uint32(bits), jnp.uint32(0))
            hi = jnp.where(val(2 * sl + 1), jnp.uint32(bits << 16), jnp.uint32(0))
            return lo | hi
        for m in range(3):
            ccol = (m * 128 + ln) // 2
            cres = ccol % CM
            w = words(lambda rho: ((rho >= 14) & (rho < 29) & (rho - 14 == cres)) | (rho == 29), 0x3F80)
            aug1_ref[m] = w[8:16]
            rq = _iota((32, 128), 0)
            lq = _iota((32, 128), 1)
            ccq = jnp.clip((m * 128 + lq) // 2, 3, 188) % CM
            qcol = jnp.where(((rq >= 14) & (rq < 29) & (((rq - 14 - ccq + 3 + CM) % CM) > 6)) | (rq == 30), -BIG, 0.0)
            qaug1_ref[m] = qcol[16:32]
            for rho in range(RM):
                rw = jnp.where(sub8 == rho // 2, jnp.uint32(0x3F80 if rho % 2 == 0 else 0x3F800000), jnp.uint32(0))
                aug0_ref[m, rho] = w[0:8] | rw
                qaug0_ref[m, rho] = jnp.where((rq < 14) & (((rq - rho + 3 + RM) % RM) > 6), -BIG, qcol)[0:16]
        for pr in range(2):
            for u in range(NS):
                ulast_ref[pr, u] = pad_word
            for pc in range(2):
                for p in range(2):
                    for g in range(NGX):
                        x2_ref[0, pr, pc, p, g] = pad_word
        q2_ref[NB] = jnp.zeros(q2_ref.shape[1:], u32)
        flag_ref[0] = 0

    pl.when(s == 0)(_setup)

    colpatch_lane = (lane8 >= L_COL) & (lane8 < L_ONE)
    klabel = jnp.where(lane8 - L_COL == 7 + sub8, jnp.uint32(ONE2), jnp.uint32(0))
    qlabel = jnp.where(lane8 - L_COL < 8, jnp.uint32(NBIG * 0x10001), jnp.uint32(0))

    bnd = {}

    def pre_unit(xw, qw, pr, k, m):
        uss = []
        qss = []
        for il in (2 * k, 2 * k + 1):
            h = 2 * il + pr
            row = 8 * s + il
            rho = row % RM
            rhoq = jnp.clip(row, 3, 188) % RM
            xt = x_ref[h, :, m * 128:(m + 1) * 128]
            aug = jnp.concatenate([aug0_ref[m, rho], aug1_ref[m]], axis=0)
            full = jnp.concatenate([xt, _b(aug)], axis=0)
            uw = _u(full.T)
            uss.append([uw[8 * v:8 * v + 8] for v in range(8)])
            qt = _nn(_b(at_ref[...]), full)
            qfull = jnp.concatenate([qt, qaug0_ref[m, rhoq], qaug1_ref[m]], axis=0)
            qwd = _u(qfull.astype(bf16).T)
            qss.append([qwd[8 * v:8 * v + 8] for v in range(8)])
        xs = xw(0, 2 + k) if k < 2 else xw(1, k - 2)
        for v in range(8):
            u = 8 * m + v
            prev = ulast_ref[pr, u]
            ulast_ref[pr, u] = uss[1][v]
            for pc in range(2):
                w = _halves(prev, uss[0][v], pc)
                rolled = pltpu.roll(w, 4, 0)
                left = pad_word if u == 0 else bnd[(pr, k, pc)]
                xs(pr, pc, u, jnp.where(lo4, left, rolled))
                bnd[(pr, k, pc)] = rolled
                qwrd = _halves(qss[0][v], qss[1][v], pc)
                qw(pr, pc, u, k, qwrd)
                if u == NS - 1:
                    xs(pr, pc, NS, jnp.where(lo4, rolled, pad_word))
                if u == 0 and pc == 0:
                    xs(pr, 0, NG, w)
                if u == NS - 1 and pc == 1:
                    xs(pr, 0, NG + 1, jnp.where(colpatch_lane, klabel, w))
                if u == 0 and pc == 1:
                    bnd[(pr, k, 'q')] = qwrd
                if u == NS - 1 and pc == 0:
                    qw(pr, 0, NS, k, jnp.where(lo4, bnd[(pr, k, 'q')], jnp.where(colpatch_lane, qlabel, qwrd)))

    PRE_UNITS = [(pr, k, m) for pr in range(2) for k in range(4) for m in range(3)]

    def out_unit(h, m):
        pr = h % 2
        i = h // 2
        w = _b(jnp.concatenate([ow_ref[pr, i // 2, 8 * m + v, pl.ds(i % 2, 8, stride=2), :] for v in range(8)], axis=0))
        r = _nt(_b(bt_ref[...]), w)
        inv = 1.0 / r[C:C + 1]
        out_ref[h, :, m * 128:(m + 1) * 128] = (r[0:C] * inv).astype(bf16)

    OUT_UNITS = [(h, m) for h in range(16) for m in range(3)]

    def colidx(n):
        r = _iota((n, 128), 0)
        return 4 * ((r // 8) % 2) + (r % 8) // 2

    def attn_stage(with_pre, with_out):
        xv = x2_ref.at[pl.ds(s - 2, 4 if with_pre else 2)]
        qv = q2_ref.at[pl.ds(s - 2, 3 if with_pre else 2)]

        def keytile(slot, pr, pck, g):
            return _b(xv[slot, pr, pck, :, g:g + 2].reshape(64, 128))

        def xw(o, p):
            def st(pr, pc, u, val):
                xv[2 + o, pr, pc, p, u] = val
            return st

        def qw(pr, pc, u, k, val):
            qv[2, pr, pc, u, k] = val

        tiles = []
        for pr in range(2):
            order = [NV - 1] + list(range(NV - 1))
            tiles += [(pr, vi) for vi in order]
        nt = len(tiles)
        col = colidx(64)
        sl = _iota((48, 128), 0)
        ln = _iota((48, 128), 1)
        irow = 2 * (sl // 16) + sl % 2
        if not (with_pre or with_out):
            irow = jnp.maximum(irow, jnp.where(s == 2, 3, 0))
        pos = 2 * (ln // 32) + ln % 2
        mnew = pos <= irow
        pvals = {}
        res = {}
        fence = {}
        never = flag_ref[0] != 0
        sd = jnp.minimum(s + flag_ref[0], NB - 1)

        def qk(pr, vi):
            pcq, j, pck, g = VSTRIPS[vi]
            l = _b(jnp.concatenate([qv[0, pr, pcq, j].reshape(32, 128),
                                    qv[1, pr, pcq, j, 0:3].reshape(24, 128)], axis=0))
            sc = _nt(l, keytile(1, pr, pck, g))
            cp = c_ref[pr, vi]
            for tok in fence.pop((pr, vi), []):
                cp = jnp.concatenate([jnp.where(never, pltpu.bitcast(tok, f32), cp[0:8]), cp[8:48]], axis=0)
            comb = jnp.concatenate([jnp.maximum(cp, sc[0:48]), sc[48:64]], axis=0)
            c_ref[pr, vi] = sc[64:112]
            m = jnp.max(comb, axis=1, keepdims=True)
            e = jnp.exp2(comb - m)
            if with_pre or with_out:
                pn = jnp.concatenate([jnp.where(mnew[16:48], e[16:48], 0.0), e[48:64]], axis=0).astype(bf16)
                po = jnp.concatenate([e[0:16], jnp.where(mnew[16:48], 0.0, e[16:48])], axis=0).astype(bf16)
            else:
                pn = jnp.concatenate([jnp.where(mnew, e[0:48], 0.0), e[48:64]], axis=0).astype(bf16)
                po = jnp.where(mnew, 0.0, e[0:48]).astype(bf16)
            pvals[(pr, vi)] = (pn, po)

        def pv(pr, vi):
            pcq, j, pck, g = VSTRIPS[vi]
            pn, po = pvals.pop((pr, vi))
            o = _nn(pn, keytile(1, pr, pck, g))
            if with_pre or with_out:
                merged = jnp.concatenate([xv[1, pr, pck, 0:1, g:g + 2], xv[0, pr, pck, 1:4, g:g + 2]], axis=0)
                oa = _nn(po, _b(merged.reshape(64, 128)))
                res[(pr, vi)] = jnp.concatenate([oa[0:16], oa[16:48] + o[0:32], o[32:48]], axis=0)
            else:
                oa = _nn(po, keytile(0, pr, pck, g))
                res[(pr, vi)] = jnp.concatenate([o[0:48] + oa, o[48:64]], axis=0)
            if vi < 2 * NS and vi % 2 == 1:
                o0 = res.pop((pr, vi - 1))
                o1 = res.pop((pr, vi))
                if j == 0:
                    o1 = jnp.where(col < 3, res[(pr, NV - 1)], o1)
                if j == NS - 1:
                    o0 = jnp.where(col >= 5, res.pop((pr, NV - 1)), o0)
                ow_ref[pr, :, j] = _packi(o0, o1).reshape(4, 16, 128)

        extra = {}
        if with_out:
            for pr in range(2):
                for m in range(3):
                    ready = pr * NV + 1 + 16 * (m + 1) - 1 + D
                    for i in range(8):
                        pos_ = ready + E + 2 * i
                        if pr == 1 and m == 1 and i >= 8 - NFILL:
                            pos_ = nt + D - 1
                        if pr == 1 and m == 2:
                            pos_ = nt + D + NTAIL + i
                        extra.setdefault(pos_, []).append(('o', 2 * i + pr, m))
        if with_pre:
            npre = len(PRE_UNITS) - NTAIL
            for n, un in enumerate(PRE_UNITS[:npre]):
                extra.setdefault(POFF + (n * (nt + PEND - POFF)) // npre, []).append(('p',) + un)
            last = nt + D
            for n, un in enumerate(PRE_UNITS[npre:]):
                extra.setdefault(last - 1 + n, []).append(('p',) + un)
        nslot = max([nt + D] + [k + 1 for k in extra])
        for n in range(nslot):
            if n < nt:
                qk(*tiles[n])
            if D <= n < nt + D:
                pv(*tiles[n - D])
            for e in extra.get(n, []):
                if e[0] == 'o':
                    out_unit(e[1], e[2])
                else:
                    pre_unit(xw, qw, *e[1:])
                    if FK and n + FK < nt:
                        fence.setdefault(tiles[n + FK], []).append(x2_ref[sd, 0, 0, 0, 0] | q2_ref[sd, 0, 0, 0, 0])

    def fixup(pr_q, qslot, qp0, keyfn, full, part, part_half):
        tiles = [VSTRIPS[NV - 1]] + VSTRIPS[:NV - 1]
        sv = {}
        res = {}
        col = colidx(32)
        keepnew = (_iota((16, 128), 0) % 2) == part_half

        def qk(n):
            pcq, j, pck, g = tiles[n]
            l = _b(q2_ref[qslot, pr_q, pcq, j, qp0:qp0 + 2].reshape(16, 128))
            sv[n] = _nt(l, keyfn(pck, g))

        def pv(n):
            pcq, j, pck, g = tiles[n]
            sc = sv.pop(n)
            m = jnp.max(sc, axis=1, keepdims=True)
            p = jnp.exp2(sc - m).astype(bf16)
            res[n] = _nn(p, keyfn(pck, g))
            if n >= 1 and n % 2 == 0:
                o0 = res.pop(n - 1)
                o1 = res.pop(n)
                if j == 0:
                    o1 = jnp.where(col < 3, res[0], o1)
                if j == NS - 1:
                    o0 = jnp.where(col >= 5, res.pop(0), o0)
                w = _packi(o0, o1)
                ow_ref[pr_q, qp0 + full, j] = w[16 * full:16 * full + 16]
                ow_ref[pr_q, qp0 + part, j] = jnp.where(keepnew, w[16 * part:16 * part + 16],
                                                        ow_ref[pr_q, qp0 + part, j])
        DF = 10
        for n in range(len(tiles) + DF):
            if n < len(tiles):
                qk(n)
            if n >= DF:
                pv(n - DF)

    @pl.when(s <= 2)
    def _():
        xv = x2_ref.at[pl.ds(s, 2)]
        qv = q2_ref.at[pl.ds(s, 1)]

        def xw(o, p):
            def st(pr, pc, u, val):
                xv[o, pr, pc, p, u] = val
            return st

        def qw(pr, pc, u, k, val):
            qv[0, pr, pc, u, k] = val
        for u in PRE_UNITS:
            pre_unit(xw, qw, *u)

    @pl.when(s == 1)
    def _conly():
        for pr in range(2):
            for vi, (pcq, j, pck, g) in enumerate(VSTRIPS):
                l = _b(q2_ref[0, pr, pcq, j, 0:3].reshape(24, 128))
                c_ref[pr, vi] = _nt(l, _b(x2_ref[0, pr, pck, :, g:g + 2].reshape(64, 128)))

    @pl.when((s >= 3) & (s < NB))
    def _():
        attn_stage(True, True)

    @pl.when(s == NB)
    def _tail_pairs():
        for pr in range(2):
            for pc in range(2):
                left = pad_word
                for u in range(NS):
                    w = _halves(ulast_ref[pr, u], pad_word, pc)
                    rolled = pltpu.roll(w, 4, 0)
                    x2_ref[NB, pr, pc, 2, u] = jnp.where(lo4, left, rolled)
                    left = rolled
                    if u == 0 and pc == 0:
                        x2_ref[NB, pr, 0, 2, NG] = w
                    if u == NS - 1 and pc == 1:
                        x2_ref[NB, pr, 0, 2, NG + 1] = jnp.where(colpatch_lane, klabel, w)
                x2_ref[NB, pr, pc, 2, NS] = jnp.where(lo4, left, pad_word)
                for g in range(NGX):
                    x2_ref[NB, pr, pc, 3, g] = pad_word

    @pl.when((s == 2) | (s >= NB))
    def _():
        attn_stage(False, False)

    @pl.when(s == 2)
    def _():
        def keyfn(pck, g):
            return _b(jnp.concatenate([x2_ref[0, 0, pck, 2:4, g:g + 2].reshape(32, 128),
                                       x2_ref[1, 0, pck, 0:2, g:g + 2].reshape(32, 128)], axis=0))
        fixup(1, 0, 0, keyfn, 0, 1, 0)

    @pl.when(s == NB + 1)
    def _():
        def keyfn(pck, g):
            return _b(jnp.concatenate([x2_ref[NB - 1, 1, pck, 3:4, g:g + 2].reshape(16, 128),
                                       x2_ref[NB, 1, pck, 0:3, g:g + 2].reshape(48, 128)], axis=0))
        fixup(0, NB - 1, 2, keyfn, 1, 0, 1)
        fixup(1, NB - 1, 2, keyfn, 1, 0, 1)

    @pl.when((s == 2) | (s >= NB))
    def _():
        for h, m in OUT_UNITS:
            out_unit(h, m)


@jax.jit
def pallas_standalone__neighborhood_nat__vision_kernel(x, wqkv, wo):
    xt = jnp.transpose(x.reshape(H, W, C), (0, 2, 1))
    out = pl.pallas_call(
        _kernel,
        grid=(NB + 2,),
        in_specs=[
            pl.BlockSpec((16, C, W), lambda s: (jnp.minimum(s, NB - 1), 0, 0)),
            pl.BlockSpec((C, 3 * C), lambda s: (0, 0)),
            pl.BlockSpec((C, C), lambda s: (0, 0)),
        ],
        out_specs=pl.BlockSpec((16, C, W), lambda s: (jnp.clip(s - 2, 0, NB - 1), 0, 0)),
        out_shape=jax.ShapeDtypeStruct((H, C, W), bf16),
        scratch_shapes=[
            pltpu.VMEM((48, 128), u32),
            pltpu.VMEM((56, 128), u32),
            pltpu.VMEM((3, RM, 8, 128), u32),
            pltpu.VMEM((3, 8, 128), u32),
            pltpu.VMEM((3, RM, 16, 128), f32),
            pltpu.VMEM((3, 16, 128), f32),
            pltpu.VMEM((2, NS, 8, 128), u32),
            pltpu.VMEM((NB + 1, 2, 2, 4, NGX, 8, 128), u32),
            pltpu.VMEM((NB + 1, 2, 2, NS + 1, 4, 8, 128), u32),
            pltpu.VMEM((2, NV, 48, 128), f32),
            pltpu.VMEM((2, 4, NS, 16, 128), u32),
            pltpu.SMEM((1,), i32),
        ],
        compiler_params=pltpu.CompilerParams(
            dimension_semantics=("arbitrary",), vmem_limit_bytes=110 * 1024 * 1024),
        name="nat_kernel",
    )(xt, wqkv, wo)
    return jnp.transpose(out, (0, 2, 1)).reshape(1, H, W, C)
```

```python
import math

import jax
import jax.numpy as jnp
from jax import lax
from jax.experimental import pallas as pl
from jax.experimental.pallas import tpu as pltpu

H = 384
W = 384
C = 96
NP = 12
NB = 24
NS = 24
NR = 4
XR = W + 16
BIG = 2.0 ** 100
ONE = 0x3F80
ONE2 = 0x3F803F80
NBIG = 0xF180
RM = 14
CM = 15
L_COL = 110
L_ONE = 125
L_PAD = 126
D = 8
E = 4
POFF = 6
NFILL = 4
PEND = -20
FK1 = 8
FENCE1 = 1
FPOS = -6
FSTEP = 0
LE = 8
LOFF = 0
LSTEP = 1
DF = 6

bf16 = jnp.bfloat16
f32 = jnp.float32
u32 = jnp.uint32
i32 = jnp.int32


def _iota(shape, dim):
    return lax.broadcasted_iota(i32, shape, dim)


def _nt(a, b):
    return lax.dot_general(a, b, (((1,), (1,)), ((), ())), preferred_element_type=f32)


def _nn(a, b):
    return lax.dot_general(a, b, (((1,), (0,)), ((), ())), preferred_element_type=f32)


def _unpack(u, idx):
    return pltpu.unpack_elementwise(u, index=idx, packed_dtype=bf16, unpacked_dtype=f32)


def _packi(a, b):
    return pltpu.pack_elementwise([a, b], packed_dtype=bf16)


def _b(u):
    return pltpu.bitcast(u, bf16)


def _u(b):
    return pltpu.bitcast(b, u32)


def _s2(start):
    return pl.ds(start, 8, stride=2)


VSTRIPS = [(pc, j) for j in range(NS) for pc in range(2)] + [(0, NS)]
NV = len(VSTRIPS)
PRE_UNITS = [(pr, k, m) for pr in range(2) for k in range(4) for m in range(3)]
LATE_UNITS = [(2 * i + 1, 2) for i in range(8)]
EARLY_UNITS = [(h, m) for h in range(16) for m in range(3) if (h, m) not in LATE_UNITS]


def _kernel(x_hbm, wqkv_ref, wo_ref, out_ref,
            at_ref, bt_ref, augx_ref, augq_ref, x2_ref, xs_ref, q2_ref, qs_ref, c_ref, ow_ref,
            xbuf_ref, obuf_ref, owf_ref, flag_ref, sem):
    t = pl.program_id(0)
    sub8 = _iota((8, 128), 0)
    lane8 = _iota((8, 128), 1)
    pad_word = jnp.where(lane8 == L_PAD, jnp.uint32(ONE2), jnp.uint32(0))
    lo4 = sub8 < 4

    def _setup():
        wq = wqkv_ref[:, 0:C]
        wk = wqkv_ref[:, C:2 * C]
        wv = wqkv_ref[:, 2 * C:3 * C]
        pl_ = _iota((C, C), 0)
        pc_ = _iota((C, C), 1)
        perm = jnp.where(pc_ == jnp.where(pl_ < C // 2, 2 * pl_, 2 * (pl_ - C // 2) + 1), 1.0, 0.0).astype(bf16)
        at = (_nt(wk, wq) * (C ** -0.5 * math.log2(math.e))).astype(bf16)
        at_ref[...] = _u(_nn(perm, at).astype(bf16))
        b = _nn(wv, wo_ref[...]).astype(bf16)
        bt = _nn(perm, b).T
        bt = jnp.concatenate([bt, jnp.zeros((C, 128 - C), f32)], axis=1)
        bt = jnp.concatenate([bt, jnp.zeros((112 - C, 128), f32)], axis=0)
        r = _iota((112, 128), 0)
        c = _iota((112, 128), 1)
        bt_ref[...] = _u(jnp.where((r == C) & (c == L_ONE), 1.0, bt).astype(bf16))
        rho = _iota((32, 128), 0)
        for m in range(3):
            ccol = (m * 128 + _iota((32, 128), 1)) // 2
            kcol = ((rho >= 14) & (rho < 29) & (rho - 14 == ccol % CM)) | (rho == 29)
            ccq = jnp.clip(ccol, 3, 188) % CM
            qcol = ((rho >= 14) & (rho < 29) & (((rho - 14 - ccq + 3 + CM) % CM) > 6)) | (rho == 30)

            def kaug(res):
                return rho == 30 if res is None else kcol | (rho == res)

            def qaug(res):
                return qcol | ((rho < 14) & (((rho - res + 3 + RM) % RM) > 6))

            def words(lo, hi, bits):
                return (jnp.where(lo, jnp.uint32(bits), jnp.uint32(0))
                        | jnp.where(hi, jnp.uint32(bits << 16), jnp.uint32(0)))
            kvar = [(2 * v + 1, (2 * v + 2) % RM) for v in range(7)] + [(None, 0), (191 % RM, None)]
            qvar = [(2 * v, 2 * v + 1) for v in range(7)] + [(3, 3), (188 % RM, 188 % RM)]
            for v in range(9):
                augx_ref[m, v] = words(kaug(kvar[v][0]), kaug(kvar[v][1]), ONE)
                augq_ref[m, v] = words(qaug(qvar[v][0]), qaug(qvar[v][1]), NBIG)
        pad_plane = jnp.where(_iota((XR, 128), 1) == L_PAD, jnp.uint32(ONE2), jnp.uint32(0))
        for pr in range(2):
            for sl in range(NR):
                for p in range(4):
                    x2_ref[sl, pr, p, 0:8] = pad_word
                    x2_ref[sl, pr, p, XR - 8:XR] = pad_word
                    if sl == 0 and p < 2:
                        x2_ref[sl, pr, p] = pad_plane
                        xs_ref[sl, pr, p] = pad_word
        xbuf_ref[0, 0:2] = jnp.zeros((2, C, W), bf16)
        flag_ref[0] = 0

    colpatch_lane = (lane8 >= L_COL) & (lane8 < L_ONE)
    klabel = jnp.where(lane8 - L_COL == 7 + sub8, jnp.uint32(ONE2), jnp.uint32(0))
    qlabel = jnp.where(lane8 - L_COL < 8, jnp.uint32(NBIG * 0x10001), jnp.uint32(0))

    def key_words(xa, xb, aug, tile, pr, p, m):
        slot = tile % NR
        w = jnp.concatenate([_packi(_unpack(xa, 0), _unpack(xb, 0)), _packi(_unpack(xa, 1), _unpack(xb, 1)), aug],
                            axis=0)
        x2_ref[slot, pr, p, 8 + 128 * m:8 + 128 * (m + 1)] = w.T
        if m == 2:
            xs_ref[slot, pr, p] = jnp.where(colpatch_lane, klabel, x2_ref[slot, pr, p, _s2(8 + 369)])

    def pre_unit(xsrc, r0, blk, tile, pr, k, m):
        rows = [xsrc[r0 + 2 * il + pr, :, m * 128:(m + 1) * 128] for il in (2 * k - 1, 2 * k, 2 * k + 1)]
        ra = 8 * blk + 2 * k
        vx = jnp.where(ra < 1, 7, ((ra + RM - 1) % RM) // 2)
        vq = jnp.where(ra < 3, 7, jnp.where(ra >= 188, 8, (ra % RM) // 2))
        key_words(_u(rows[0]), _u(rows[1]), augx_ref[m, vx], tile + k // 2, pr, (k + 2) % 4, m)
        at = _b(at_ref[...])
        qw = jnp.concatenate([_packi(_nn(at, rows[1]), _nn(at, rows[2])), augq_ref[m, vq]], axis=0)
        slot = tile % NR
        q2_ref[slot, pr, k, 128 * m:128 * (m + 1)] = qw.T
        if m == 2:
            qs_ref[slot, pr, k] = jnp.where(lo4, q2_ref[slot, pr, k, _s2(1)],
                                            jnp.where(colpatch_lane, qlabel, q2_ref[slot, pr, k, _s2(368)]))

    def keytile(tiles_pairs, pr, vi):
        pc, j = VSTRIPS[vi]
        vs = []
        for tile, p in tiles_pairs:
            if j == NS:
                vs += [x2_ref[tile % NR, pr, p, _s2(8)], xs_ref[tile % NR, pr, p]]
            else:
                vs += [x2_ref[tile % NR, pr, p, _s2(16 * j + pc)], x2_ref[tile % NR, pr, p, _s2(16 * j + 16 + pc)]]
        return _b(jnp.concatenate(vs, axis=0))

    def qrows(tiles_pairs, pr, vi):
        pc, j = VSTRIPS[vi]
        return [qs_ref[tile % NR, pr, k] if j == NS else q2_ref[tile % NR, pr, k, _s2(16 * j + pc)]
                for tile, k in tiles_pairs]

    def out_unit(dst, r0, h, m):
        pr = h % 2
        i = h // 2
        w = _b(jnp.concatenate([ow_ref[pr, i // 2, 8 * m + v, _s2(i % 2), :] for v in range(8)], axis=0))
        r = _nt(_b(bt_ref[...]), w)
        inv = 1.0 / r[C:C + 1]
        dst[r0 + h, :, m * 128:(m + 1) * 128] = (r[0:C] * inv).astype(bf16)

    def in_copy(p):
        return pltpu.make_async_copy(x_hbm.at[pl.ds(32 * p - 2, 34)], xbuf_ref.at[p % 2], sem.at[p % 2])

    def in_copy0(i):
        return pltpu.make_async_copy(x_hbm.at[pl.ds(16 * i, 16)], xbuf_ref.at[0, pl.ds(2 + 16 * i, 16)], sem.at[2 + i])

    def out_copy(p, r0=0, nr=32, si=None):
        return pltpu.make_async_copy(obuf_ref.at[p % 3, pl.ds(r0, nr)], out_ref.at[pl.ds(32 * p + r0, nr)],
                                     sem.at[4 + p % 3 if si is None else si])

    def colidx(n):
        r = _iota((n, 128), 0)
        return 4 * ((r // 8) % 2) + (r % 8) // 2

    def store_pair(res, key0, key1, keysp, j, col):
        o0 = res.pop(key0)
        o1 = res.pop(key1)
        if j == 0:
            o1 = jnp.where(col < 3, res[keysp], o1)
        if j == NS - 1:
            o0 = jnp.where(col >= 5, res.pop(keysp), o0)
        return _packi(o0, o1)

    def attn_stage(base, blk0, nsub, with_pre, xsrc, o_prev, o_cur, o_prev_r0, o_cur_r0, top):
        tiles = []
        for pr in range(2):
            order = [NV - 1] + list(range(NV - 1))
            tiles += [(pr, vi) for vi in order]
        nt = len(tiles)
        gtiles = [(d,) + tl for d in range(nsub) for tl in tiles]
        ntot = len(gtiles)
        col = colidx(64)
        sl = _iota((32, 128), 0)
        ln = _iota((32, 128), 1)
        mnew = (2 * (ln // 32) + ln % 2) <= (2 + 2 * (sl // 16) + sl % 2)
        topmask = None if top is None else (top & ((sl < 16) | (sl % 2 == 0)))
        pvals = {}
        res = {}

        def qk(d, pr, vi):
            g = base + d
            l = _b(jnp.concatenate(qrows([(g, k) for k in range(4)] + [(g + 1, k) for k in range(3)], pr, vi), axis=0))
            sc = _nt(l, keytile([(g + 1, p) for p in range(4)], pr, vi))
            cp = c_ref[pr, vi]
            comb = jnp.concatenate([jnp.maximum(cp, sc[0:48]), sc[48:64]], axis=0)
            c_ref[pr, vi] = sc[64:112]
            m = jnp.max(comb, axis=1, keepdims=True)
            e = jnp.exp2(comb - m)
            pn = jnp.concatenate([jnp.where(mnew, e[16:48], 0.0), e[48:64]], axis=0).astype(bf16)
            po = jnp.concatenate([e[0:16], jnp.where(mnew, 0.0, e[16:48])], axis=0).astype(bf16)
            pvals[(d, pr, vi)] = (pn, po)

        def pv(d, pr, vi):
            pn, po = pvals.pop((d, pr, vi))
            g = base + d
            o = _nn(pn, keytile([(g + 1, p) for p in range(4)], pr, vi))
            oa = _nn(po, keytile([(g + 1, 0), (g, 1), (g, 2), (g, 3)], pr, vi))
            res[(pr, vi)] = jnp.concatenate([oa[0:16], oa[16:48] + o[0:32], o[32:48]], axis=0)
            if vi < 2 * NS and vi % 2 == 1:
                j = vi // 2
                w = store_pair(res, (pr, vi - 1), (pr, vi), (pr, NV - 1), j, col)
                if d == 0 and topmask is not None:
                    w = jnp.concatenate([jnp.where(topmask, owf_ref[pr, :, j].reshape(32, 128), w[0:32]), w[32:64]],
                                        axis=0)
                ow_ref[pr, :, j] = w.reshape(4, 16, 128)

        extra = {}
        for d in range(nsub):
            off = d * nt
            dst_late = (o_prev, o_prev_r0) if d == 0 else (o_cur, o_cur_r0 + 16 * (d - 1))
            dst = (o_cur, o_cur_r0 + 16 * d)
            for n, (h, m) in enumerate(LATE_UNITS):
                pos_ = LOFF + LSTEP * n if d == 0 else off + D + LE + 2 * n
                extra.setdefault(pos_, []).append(('o', dst_late, h, m))
            for h, m in EARLY_UNITS:
                pr, i = h % 2, h // 2
                ready = pr * NV + 1 + 16 * (m + 1) - 1 + D
                pos_ = off + ready + E + 2 * i
                if d == nsub - 1 and pr == 1 and m == 1 and i >= 8 - NFILL:
                    pos_ = ntot + D + FPOS + (FSTEP * (i - 8 + NFILL)) // 2
                extra.setdefault(pos_, []).append(('o', dst, h, m))
            if with_pre:
                span = nt + (PEND if d == nsub - 1 else 0) - (POFF if d == 0 else 0)
                start = off + (POFF if d == 0 else 0)
                for n, un in enumerate(PRE_UNITS):
                    extra.setdefault(start + (n * span) // len(PRE_UNITS), []).append(('p', d) + un)
        nslot = max([ntot + D] + [k + 1 for k in extra])
        for n in range(nslot):
            if n < ntot:
                qk(*gtiles[n])
            if D <= n < ntot + D:
                pv(*gtiles[n - D])
            for e in extra.get(n, []):
                if e[0] == 'o':
                    out_unit(e[1][0], e[1][1], e[2], e[3])
                else:
                    d = e[1]
                    pre_unit(xsrc, 2 + 16 * d, blk0 + 2 + d, base + 2 + d, *e[2:])

    def fixup(qslot, qp0, key_slots_pairs, key_pr, store):
        order = [NV - 1] + list(range(NV - 1))
        sv = {}
        res = {}
        col = colidx(64)

        def qk(n):
            vi = order[n]
            l = _b(jnp.concatenate(qrows([(qslot, qp0), (qslot, qp0 + 1)], 0, vi)
                                   + qrows([(qslot, qp0), (qslot, qp0 + 1)], 1, vi), axis=0))
            sc = _nt(l, keytile(key_slots_pairs, key_pr, vi))
            m = jnp.max(sc, axis=1, keepdims=True)
            sv[n] = jnp.exp2(sc - m).astype(bf16)

        def pv(n):
            vi = order[n]
            res[vi] = _nn(sv.pop(n), keytile(key_slots_pairs, key_pr, vi))
            if vi < 2 * NS and vi % 2 == 1:
                store(vi // 2, store_pair(res, vi - 1, vi, NV - 1, vi // 2, col))
        return qk, pv, NV

    def merge_fixup(pr, j, qp0, full, part, part_half, wfull, wpart):
        keepnew = (_iota((16, 128), 0) % 2) == part_half
        ow_ref[pr, qp0 + full, j] = wfull
        ow_ref[pr, qp0 + part, j] = jnp.where(keepnew, wpart, ow_ref[pr, qp0 + part, j])

    def main_block(par):
        attn_stage(2 * par + 2, 2 * t - 2, 2, True, xbuf_ref.at[par], obuf_ref.at[(t + 1) % 3],
                   obuf_ref.at[(t + 2) % 3], 16, 0, t == 1 if par == 1 else None)

    @pl.when(t == 0)
    def _():
        in_copy0(0).start()
        in_copy0(1).start()
        _setup()
        in_copy0(0).wait()

    @pl.when(t == 0)
    def _():
        for u in PRE_UNITS:
            pre_unit(xbuf_ref.at[0], 2, 0, 0, *u)

    @pl.when(t == 0)
    def _():
        in_copy0(1).wait()
        in_copy(1).start()

    @pl.when(t == 0)
    def _():
        never = flag_ref[0] != 0
        sd = jnp.minimum(t + flag_ref[0], NR - 1)
        fence = {}

        def store(j, w):
            owf_ref[:, :, j] = w.reshape(2, 2, 16, 128)
        fqk, fpv, nf = fixup(0, 0, [(0, 2), (0, 3), (1, 0), (1, 1)], 0, store)
        order = [NV - 1] + list(range(NV - 1))

        def conly(pr, vi, toks):
            l = jnp.concatenate(qrows([(0, k) for k in range(3)], pr, vi), axis=0)
            for tok in toks:
                l = jnp.concatenate([jnp.where(never, tok, l[0:8]), l[8:24]], axis=0)
            c_ref[pr, vi] = _nt(_b(l), keytile([(0, p) for p in range(4)], pr, vi))
        nslot = nf + DF
        for n in range(nslot):
            if n < nf:
                fqk(n)
                conly(0, order[n], fence.pop(n, []))
                conly(1, order[n], [])
            if n >= DF:
                fpv(n - DF)
            for un in range(len(PRE_UNITS)):
                if (un * (nf - FK1)) // len(PRE_UNITS) == n:
                    pre_unit(xbuf_ref.at[0], 18, 1, 1, *PRE_UNITS[un])
                    if FENCE1:
                        fence.setdefault(n + FK1, []).append(x2_ref[sd, 0, 0, 0:8] | q2_ref[sd, 0, 0, 0:8])

    @pl.when(t >= 1)
    def _():
        @pl.when(t < NP)
        def _():
            in_copy(t).wait()

        @pl.when(t < NP - 1)
        def _():
            in_copy(t + 1).start()

        @pl.when(t >= 4)
        def _():
            out_copy(t - 4).wait()

    for par in range(2):
        @pl.when((t >= 1) & (t < NP) & (t % 2 == par))
        def _():
            main_block(par)

    @pl.when((t >= 2) & (t < NP))
    def _():
        out_copy(t - 2).start()

    last = obuf_ref.at[(NP - 1) % 3]
    prev = obuf_ref.at[(NP - 2) % 3]

    @pl.when(t == NP)
    def _tail_pairs():
        pad_plane = jnp.where(_iota((XR, 128), 1) == L_PAD, jnp.uint32(ONE2), jnp.uint32(0))
        for pr in range(2):
            for m in range(3):
                xa = _u(xbuf_ref[(NP - 1) % 2, 32 + pr, :, m * 128:(m + 1) * 128])
                key_words(xa, jnp.zeros_like(xa), augx_ref[m, 8], NB, pr, 2, m)
            x2_ref[NB % NR, pr, 3] = pad_plane
            xs_ref[NB % NR, pr, 3] = pad_word

    @pl.when(t == NP)
    def _():
        attn_stage(NB - 2, NB - 2, 1, False, None, prev, last, 16, 0, None)

    @pl.when(t == NP)
    def _():
        out_copy(NP - 2).start()

    @pl.when(t == NP)
    def _():
        attn_stage(NB - 1, NB - 1, 1, False, None, last, last, 0, 16, None)

    @pl.when(t == NP)
    def _():
        out_copy(NP - 1, 0, 16).start()
        for h, m in LATE_UNITS:
            if h < 10:
                out_unit(last, 16, h, m)
        out_copy(NP - 1, 16, 10, 7).start()

        def store(j, w):
            for pr in range(2):
                merge_fixup(pr, j, 2, 1, 0, 1, w[32 * pr + 16:32 * pr + 32], w[32 * pr:32 * pr + 16])
        fqk, fpv, nf = fixup(NB - 1, 2, [(NB - 1, 3), (NB, 0), (NB, 1), (NB, 2)], 1, store)
        for n in range(nf + DF):
            if n < nf:
                fqk(n)
            if n >= DF:
                fpv(n - DF)
        for h in range(10, 16):
            for m in range(3):
                out_unit(last, 16, h, m)
        out_copy(NP - 1, 26, 6, 8).start()
        out_copy(NP - 3).wait()
        out_copy(NP - 2).wait()
        out_copy(NP - 1, 0, 16).wait()
        out_copy(NP - 1, 16, 10, 7).wait()
        out_copy(NP - 1, 26, 6, 8).wait()


@jax.jit
def pallas_standalone__neighborhood_nat__vision_kernel(x, wqkv, wo):
    xt = jnp.transpose(x.reshape(H, W, C), (0, 2, 1))
    out = pl.pallas_call(
        _kernel,
        grid=(NP + 1,),
        in_specs=[
            pl.BlockSpec(memory_space=pl.ANY),
            pl.BlockSpec((C, 3 * C), lambda s: (0, 0)),
            pl.BlockSpec((C, C), lambda s: (0, 0)),
        ],
        out_specs=pl.BlockSpec(memory_space=pl.ANY),
        out_shape=jax.ShapeDtypeStruct((H, C, W), bf16),
        scratch_shapes=[
            pltpu.VMEM((48, 96), u32),
            pltpu.VMEM((56, 128), u32),
            pltpu.VMEM((3, 9, 32, 128), u32),
            pltpu.VMEM((3, 9, 32, 128), u32),
            pltpu.VMEM((NR, 2, 4, XR, 128), u32),
            pltpu.VMEM((NR, 2, 4, 8, 128), u32),
            pltpu.VMEM((NR, 2, 4, W, 128), u32),
            pltpu.VMEM((NR, 2, 4, 8, 128), u32),
            pltpu.VMEM((2, NV, 48, 128), f32),
            pltpu.VMEM((2, 4, NS, 16, 128), u32),
            pltpu.VMEM((2, 34, C, W), bf16),
            pltpu.VMEM((3, 32, C, W), bf16),
            pltpu.VMEM((2, 2, NS, 16, 128), u32),
            pltpu.SMEM((1,), i32),
            pltpu.SemaphoreType.DMA((9,)),
        ],
        compiler_params=pltpu.CompilerParams(
            dimension_semantics=("arbitrary",), vmem_limit_bytes=64 * 1024 * 1024,
            disable_bounds_checks=True),
        name="nat_kernel",
    )(xt, wqkv, wo)
    return jnp.transpose(out, (0, 2, 1)).reshape(1, H, W, C)
```

```python
import math

import jax
import jax.numpy as jnp
from jax import lax
from jax.experimental import pallas as pl
from jax.experimental.pallas import tpu as pltpu

H = 384
W = 384
C = 96
NP = 12
NB = 24
NS = 24
NR = 4
XR = W + 16
BIG = 2.0 ** 100
ONE = 0x3F80
ONE2 = 0x3F803F80
NBIG = 0xF180
RM = 14
CM = 15
L_COL = 110
L_ONE = 125
L_PAD = 126
D = 12
E = 8
POFF = 6
NFILL = 4
PEND = -8
PE1 = -8
FPOS = -6
FSTEP = 0
LE = 8
LOFF = 0
LSTEP = 1
DF = 6
ORD = 'aAbB'

bf16 = jnp.bfloat16
f32 = jnp.float32
u32 = jnp.uint32
i32 = jnp.int32


def _iota(shape, dim):
    return lax.broadcasted_iota(i32, shape, dim)


def _nt(a, b):
    return lax.dot_general(a, b, (((1,), (1,)), ((), ())), preferred_element_type=f32)


def _nn(a, b):
    return lax.dot_general(a, b, (((1,), (0,)), ((), ())), preferred_element_type=f32)


def _unpack(u, idx):
    return pltpu.unpack_elementwise(u, index=idx, packed_dtype=bf16, unpacked_dtype=f32)


def _packi(a, b):
    return pltpu.pack_elementwise([a, b], packed_dtype=bf16)


def _b(u):
    return pltpu.bitcast(u, bf16)


def _u(b):
    return pltpu.bitcast(b, u32)


def _s2(start):
    return pl.ds(start, 8, stride=2)


VSTRIPS = [(pc, j) for j in range(NS) for pc in range(2)] + [(0, NS)]
NV = len(VSTRIPS)
PRE_UNITS = [(pr, k, m) for pr in range(2) for k in range(4) for m in range(3)]
LATE_UNITS = [(2 * i + 1, 2) for i in range(8)]
EARLY_UNITS = [(h, m) for h in range(16) for m in range(3) if (h, m) not in LATE_UNITS]


def _kernel(x_hbm, wqkv_ref, wo_ref, out_ref,
            at_ref, bt_ref, augx_ref, augq_ref, x2_ref, xs_ref, q2_ref, qs_ref, ow_ref,
            xbuf_ref, obuf_ref, owf_ref, sem):
    t = pl.program_id(0)
    sub8 = _iota((8, 128), 0)
    lane8 = _iota((8, 128), 1)
    pad_word = jnp.where(lane8 == L_PAD, jnp.uint32(ONE2), jnp.uint32(0))
    lo4 = sub8 < 4

    def _setup():
        wq = wqkv_ref[:, 0:C]
        wk = wqkv_ref[:, C:2 * C]
        wv = wqkv_ref[:, 2 * C:3 * C]
        pl_ = _iota((C, C), 0)
        pc_ = _iota((C, C), 1)
        perm = jnp.where(pc_ == jnp.where(pl_ < C // 2, 2 * pl_, 2 * (pl_ - C // 2) + 1), 1.0, 0.0).astype(bf16)
        at = (_nt(wk, wq) * (C ** -0.5 * math.log2(math.e))).astype(bf16)
        at_ref[...] = _u(_nn(perm, at).astype(bf16))
        b = _nn(wv, wo_ref[...]).astype(bf16)
        bt = _nn(perm, b).T
        bt = jnp.concatenate([bt, jnp.zeros((C, 128 - C), f32)], axis=1)
        bt = jnp.concatenate([bt, jnp.zeros((112 - C, 128), f32)], axis=0)
        r = _iota((112, 128), 0)
        c = _iota((112, 128), 1)
        bt_ref[...] = _u(jnp.where((r == C) & (c == L_ONE), 1.0, bt).astype(bf16))
        rho = _iota((32, 128), 0)
        for m in range(3):
            ccol = (m * 128 + _iota((32, 128), 1)) // 2
            kcol = ((rho >= 14) & (rho < 29) & (rho - 14 == ccol % CM)) | (rho == 29)
            ccq = jnp.clip(ccol, 3, 188) % CM
            qcol = ((rho >= 14) & (rho < 29) & (((rho - 14 - ccq + 3 + CM) % CM) > 6)) | (rho == 30)

            def kaug(res):
                return rho == 30 if res is None else kcol | (rho == res)

            def qaug(res):
                return qcol | ((rho < 14) & (((rho - res + 3 + RM) % RM) > 6))

            def words(lo, hi, bits):
                return (jnp.where(lo, jnp.uint32(bits), jnp.uint32(0))
                        | jnp.where(hi, jnp.uint32(bits << 16), jnp.uint32(0)))
            kvar = [(2 * v + 1, (2 * v + 2) % RM) for v in range(7)] + [(None, 0), (191 % RM, None)]
            qvar = [(2 * v, 2 * v + 1) for v in range(7)] + [(3, 3), (188 % RM, 188 % RM)]
            for v in range(9):
                augx_ref[m, v] = words(kaug(kvar[v][0]), kaug(kvar[v][1]), ONE)
                augq_ref[m, v] = words(qaug(qvar[v][0]), qaug(qvar[v][1]), NBIG)
        pad_plane = jnp.where(_iota((XR, 128), 1) == L_PAD, jnp.uint32(ONE2), jnp.uint32(0))
        for pr in range(2):
            for sl in range(NR):
                for p in range(4):
                    x2_ref[sl, pr, p, 0:8] = pad_word
                    x2_ref[sl, pr, p, XR - 8:XR] = pad_word
                    if sl == 0 and p < 2:
                        x2_ref[sl, pr, p] = pad_plane
                        xs_ref[sl, pr, p] = pad_word
        xbuf_ref[0, 0:2] = jnp.zeros((2, C, W), bf16)

    colpatch_lane = (lane8 >= L_COL) & (lane8 < L_ONE)
    klabel = jnp.where(lane8 - L_COL == 7 + sub8, jnp.uint32(ONE2), jnp.uint32(0))
    qlabel = jnp.where(lane8 - L_COL < 8, jnp.uint32(NBIG * 0x10001), jnp.uint32(0))

    def key_words(xa, xb, aug, tile, pr, p, m):
        slot = tile % NR
        w = jnp.concatenate([_packi(_unpack(xa, 0), _unpack(xb, 0)), _packi(_unpack(xa, 1), _unpack(xb, 1)), aug],
                            axis=0)
        x2_ref[slot, pr, p, 8 + 128 * m:8 + 128 * (m + 1)] = w.T
        if m == 2:
            xs_ref[slot, pr, p] = jnp.where(colpatch_lane, klabel, x2_ref[slot, pr, p, _s2(8 + 369)])

    def pre_unit(xsrc, r0, blk, tile, pr, k, m):
        rows = [xsrc[r0 + 2 * il + pr, :, m * 128:(m + 1) * 128] for il in (2 * k - 1, 2 * k, 2 * k + 1)]
        ra = 8 * blk + 2 * k
        vx = jnp.where(ra < 1, 7, ((ra + RM - 1) % RM) // 2)
        vq = jnp.where(ra < 3, 7, jnp.where(ra >= 188, 8, (ra % RM) // 2))
        key_words(_u(rows[0]), _u(rows[1]), augx_ref[m, vx], tile + k // 2, pr, (k + 2) % 4, m)
        at = _b(at_ref[...])
        qw = jnp.concatenate([_packi(_nn(at, rows[1]), _nn(at, rows[2])), augq_ref[m, vq]], axis=0)
        slot = tile % NR
        q2_ref[slot, pr, k, 128 * m:128 * (m + 1)] = qw.T
        if m == 2:
            qs_ref[slot, pr, k] = jnp.where(lo4, q2_ref[slot, pr, k, _s2(1)],
                                            jnp.where(colpatch_lane, qlabel, q2_ref[slot, pr, k, _s2(368)]))

    def keytile(tiles_pairs, pr, vi):
        pc, j = VSTRIPS[vi]
        vs = []
        for tile, p in tiles_pairs:
            if j == NS:
                vs += [x2_ref[tile % NR, pr, p, _s2(8)], xs_ref[tile % NR, pr, p]]
            else:
                vs += [x2_ref[tile % NR, pr, p, _s2(16 * j + pc)], x2_ref[tile % NR, pr, p, _s2(16 * j + 16 + pc)]]
        return _b(jnp.concatenate(vs, axis=0))

    def qrows(tiles_pairs, pr, vi):
        pc, j = VSTRIPS[vi]
        return [qs_ref[tile % NR, pr, k] if j == NS else q2_ref[tile % NR, pr, k, _s2(16 * j + pc)]
                for tile, k in tiles_pairs]

    def out_unit(dst, r0, h, m):
        pr = h % 2
        i = h // 2
        w = _b(jnp.concatenate([ow_ref[pr, i // 2, 8 * m + v, _s2(i % 2), :] for v in range(8)], axis=0))
        r = _nt(_b(bt_ref[...]), w)
        inv = 1.0 / r[C:C + 1]
        dst[r0 + h, :, m * 128:(m + 1) * 128] = (r[0:C] * inv).astype(bf16)

    def in_copy(p):
        return pltpu.make_async_copy(x_hbm.at[pl.ds(32 * p - 2, 34)], xbuf_ref.at[p % 2], sem.at[p % 2])

    def in_copy0(i):
        return pltpu.make_async_copy(x_hbm.at[pl.ds(16 * i, 16)], xbuf_ref.at[0, pl.ds(2 + 16 * i, 16)], sem.at[2 + i])

    def out_copy(p, r0=0, nr=32, si=None):
        return pltpu.make_async_copy(obuf_ref.at[p % 3, pl.ds(r0, nr)], out_ref.at[pl.ds(32 * p + r0, nr)],
                                     sem.at[4 + p % 3 if si is None else si])

    def colidx(n):
        r = _iota((n, 128), 0)
        return 4 * ((r // 8) % 2) + (r % 8) // 2

    def store_pair(res, key0, key1, keysp, j, col):
        o0 = res.pop(key0)
        o1 = res.pop(key1)
        if j == 0:
            o1 = jnp.where(col < 3, res[keysp], o1)
        if j == NS - 1:
            o0 = jnp.where(col >= 5, res.pop(keysp), o0)
        return _packi(o0, o1)

    def attn_stage(base, blk0, nsub, with_pre, xsrc, o_prev, o_cur, o_prev_r0, o_cur_r0, top):
        tiles = []
        for pr in range(2):
            order = [NV - 1] + list(range(NV - 1))
            tiles += [(pr, vi) for vi in order]
        nt = len(tiles)
        gtiles = [(d,) + tl for d in range(nsub) for tl in tiles]
        ntot = len(gtiles)
        col = colidx(64)
        sl = _iota((32, 128), 0)
        ln = _iota((32, 128), 1)
        mnew = (2 * (ln // 32) + ln % 2) <= (2 + 2 * (sl // 16) + sl % 2)
        topmask = None if top is None else (top & ((sl < 16) | (sl % 2 == 0)))
        svals = {}
        pvals = {}
        res = {}

        def tile_a(d, pr, vi):
            g = base + d
            return keytile([(g + 1, 0), (g, 1), (g, 2), (g, 3)], pr, vi)

        def tile_b(d, pr, vi):
            return keytile([(base + d + 1, p) for p in range(4)], pr, vi)

        def qka(d, pr, vi):
            l = _b(jnp.concatenate(qrows([(base + d, k) for k in range(3)], pr, vi), axis=0))
            svals[(d, pr, vi)] = _nt(l, tile_a(d, pr, vi))

        def qkb(d, pr, vi):
            l = _b(jnp.concatenate(qrows([(base + d, k) for k in range(1, 4)], pr, vi), axis=0))
            sb = _nt(l, tile_b(d, pr, vi))
            sa = svals.pop((d, pr, vi))
            comb = jnp.concatenate([sa[0:16], jnp.maximum(sa[16:48], sb[0:32]), sb[32:48]], axis=0)
            m = jnp.max(comb, axis=1, keepdims=True)
            e = jnp.exp2(comb - m)
            pn = jnp.concatenate([jnp.where(mnew, e[16:48], 0.0), e[48:64]], axis=0).astype(bf16)
            po = jnp.concatenate([e[0:16], jnp.where(mnew, 0.0, e[16:48])], axis=0).astype(bf16)
            pvals[(d, pr, vi)] = (pn, po)

        def pva(d, pr, vi):
            res[(pr, vi, 'a')] = _nn(pvals[(d, pr, vi)][1], tile_a(d, pr, vi))

        def pvb(d, pr, vi):
            pn, po = pvals.pop((d, pr, vi))
            o = _nn(pn, tile_b(d, pr, vi))
            oa = res.pop((pr, vi, 'a'))
            res[(pr, vi)] = jnp.concatenate([oa[0:16], oa[16:48] + o[0:32], o[32:48]], axis=0)
            if vi < 2 * NS and vi % 2 == 1:
                j = vi // 2
                w = store_pair(res, (pr, vi - 1), (pr, vi), (pr, NV - 1), j, col)
                if d == 0 and topmask is not None:
                    w = jnp.concatenate([jnp.where(topmask, owf_ref[pr, :, j].reshape(32, 128), w[0:32]), w[32:64]],
                                        axis=0)
                ow_ref[pr, :, j] = w.reshape(4, 16, 128)

        extra = {}
        for d in range(nsub):
            off = d * nt
            dst_late = (o_prev, o_prev_r0) if d == 0 else (o_cur, o_cur_r0 + 16 * (d - 1))
            dst = (o_cur, o_cur_r0 + 16 * d)
            for n, (h, m) in enumerate(LATE_UNITS):
                pos_ = LOFF + LSTEP * n if d == 0 else off + D + LE + 2 * n
                extra.setdefault(pos_, []).append(('o', dst_late, h, m))
            for h, m in EARLY_UNITS:
                pr, i = h % 2, h // 2
                ready = pr * NV + 1 + 16 * (m + 1) - 1 + D
                pos_ = off + ready + E + 2 * i
                if d == nsub - 1 and pr == 1 and m == 1 and i >= 8 - NFILL:
                    pos_ = ntot + D + FPOS + (FSTEP * (i - 8 + NFILL)) // 2
                extra.setdefault(pos_, []).append(('o', dst, h, m))
            if with_pre:
                span = nt + (PEND if d == nsub - 1 else 0) - (POFF if d == 0 else 0)
                start = off + (POFF if d == 0 else 0)
                for n, un in enumerate(PRE_UNITS):
                    extra.setdefault(start + (n * span) // len(PRE_UNITS), []).append(('p', d) + un)
        nslot = max([ntot + D] + [k + 1 for k in extra])
        for n in range(nslot):
            q = gtiles[n] if n < ntot else None
            v = gtiles[n - D] if D <= n < ntot + D else None
            for op in ORD:
                if op in 'ab' and q:
                    (qka if op == 'a' else qkb)(*q)
                if op in 'AB' and v:
                    (pva if op == 'A' else pvb)(*v)
            for e in extra.get(n, []):
                if e[0] == 'o':
                    out_unit(e[1][0], e[1][1], e[2], e[3])
                else:
                    d = e[1]
                    pre_unit(xsrc, 2 + 16 * d, blk0 + 2 + d, base + 2 + d, *e[2:])

    def fixup(qslot, qp0, key_slots_pairs, key_pr, store):
        order = [NV - 1] + list(range(NV - 1))
        sv = {}
        res = {}
        col = colidx(64)

        def qk(n):
            vi = order[n]
            l = _b(jnp.concatenate(qrows([(qslot, qp0), (qslot, qp0 + 1)], 0, vi)
                                   + qrows([(qslot, qp0), (qslot, qp0 + 1)], 1, vi), axis=0))
            sc = _nt(l, keytile(key_slots_pairs, key_pr, vi))
            m = jnp.max(sc, axis=1, keepdims=True)
            sv[n] = jnp.exp2(sc - m).astype(bf16)

        def pv(n):
            vi = order[n]
            res[vi] = _nn(sv.pop(n), keytile(key_slots_pairs, key_pr, vi))
            if vi < 2 * NS and vi % 2 == 1:
                store(vi // 2, store_pair(res, vi - 1, vi, NV - 1, vi // 2, col))
        return qk, pv, NV

    def merge_fixup(pr, j, qp0, full, part, part_half, wfull, wpart):
        keepnew = (_iota((16, 128), 0) % 2) == part_half
        ow_ref[pr, qp0 + full, j] = wfull
        ow_ref[pr, qp0 + part, j] = jnp.where(keepnew, wpart, ow_ref[pr, qp0 + part, j])

    def main_block(par):
        attn_stage(2 * par + 2, 2 * t - 2, 2, True, xbuf_ref.at[par], obuf_ref.at[(t + 1) % 3],
                   obuf_ref.at[(t + 2) % 3], 16, 0, t == 1 if par == 1 else None)

    @pl.when(t == 0)
    def _():
        in_copy0(0).start()
        in_copy0(1).start()
        _setup()
        in_copy0(0).wait()

    @pl.when(t == 0)
    def _():
        for u in PRE_UNITS:
            pre_unit(xbuf_ref.at[0], 2, 0, 0, *u)

    @pl.when(t == 0)
    def _():
        in_copy0(1).wait()
        in_copy(1).start()

    @pl.when(t == 0)
    def _():
        def store(j, w):
            owf_ref[:, :, j] = w.reshape(2, 2, 16, 128)
        fqk, fpv, nf = fixup(0, 0, [(0, 2), (0, 3), (1, 0), (1, 1)], 0, store)
        nslot = nf + DF
        for n in range(nslot):
            if n < nf:
                fqk(n)
            if n >= DF:
                fpv(n - DF)
            for un in range(len(PRE_UNITS)):
                if (un * (nslot + PE1)) // len(PRE_UNITS) == n:
                    pre_unit(xbuf_ref.at[0], 18, 1, 1, *PRE_UNITS[un])

    @pl.when(t >= 1)
    def _():
        @pl.when(t < NP)
        def _():
            in_copy(t).wait()

        @pl.when(t < NP - 1)
        def _():
            in_copy(t + 1).start()

        @pl.when(t >= 4)
        def _():
            out_copy(t - 4).wait()

    for par in range(2):
        @pl.when((t >= 1) & (t < NP) & (t % 2 == par))
        def _():
            main_block(par)

    @pl.when((t >= 2) & (t < NP))
    def _():
        out_copy(t - 2).start()

    last = obuf_ref.at[(NP - 1) % 3]
    prev = obuf_ref.at[(NP - 2) % 3]

    @pl.when(t == NP)
    def _tail_pairs():
        pad_plane = jnp.where(_iota((XR, 128), 1) == L_PAD, jnp.uint32(ONE2), jnp.uint32(0))
        for pr in range(2):
            for m in range(3):
                xa = _u(xbuf_ref[(NP - 1) % 2, 32 + pr, :, m * 128:(m + 1) * 128])
                key_words(xa, jnp.zeros_like(xa), augx_ref[m, 8], NB, pr, 2, m)
            x2_ref[NB % NR, pr, 3] = pad_plane
            xs_ref[NB % NR, pr, 3] = pad_word

    @pl.when(t == NP)
    def _():
        attn_stage(NB - 2, NB - 2, 1, False, None, prev, last, 16, 0, None)

    @pl.when(t == NP)
    def _():
        out_copy(NP - 2).start()

    @pl.when(t == NP)
    def _():
        attn_stage(NB - 1, NB - 1, 1, False, None, last, last, 0, 16, None)

    @pl.when(t == NP)
    def _():
        out_copy(NP - 1, 0, 16).start()
        for h, m in LATE_UNITS:
            if h < 10:
                out_unit(last, 16, h, m)
        out_copy(NP - 1, 16, 10, 7).start()

        def store(j, w):
            for pr in range(2):
                merge_fixup(pr, j, 2, 1, 0, 1, w[32 * pr + 16:32 * pr + 32], w[32 * pr:32 * pr + 16])
        fqk, fpv, nf = fixup(NB - 1, 2, [(NB - 1, 3), (NB, 0), (NB, 1), (NB, 2)], 1, store)
        for n in range(nf + DF):
            if n < nf:
                fqk(n)
            if n >= DF:
                fpv(n - DF)
        for h in range(10, 16):
            for m in range(3):
                out_unit(last, 16, h, m)
        out_copy(NP - 1, 26, 6, 8).start()
        out_copy(NP - 3).wait()
        out_copy(NP - 2).wait()
        out_copy(NP - 1, 0, 16).wait()
        out_copy(NP - 1, 16, 10, 7).wait()
        out_copy(NP - 1, 26, 6, 8).wait()


@jax.jit
def pallas_standalone__neighborhood_nat__vision_kernel(x, wqkv, wo):
    xt = jnp.transpose(x.reshape(H, W, C), (0, 2, 1))
    out = pl.pallas_call(
        _kernel,
        grid=(NP + 1,),
        in_specs=[
            pl.BlockSpec(memory_space=pl.ANY),
            pl.BlockSpec((C, 3 * C), lambda s: (0, 0)),
            pl.BlockSpec((C, C), lambda s: (0, 0)),
        ],
        out_specs=pl.BlockSpec(memory_space=pl.ANY),
        out_shape=jax.ShapeDtypeStruct((H, C, W), bf16),
        scratch_shapes=[
            pltpu.VMEM((48, 96), u32),
            pltpu.VMEM((56, 128), u32),
            pltpu.VMEM((3, 9, 32, 128), u32),
            pltpu.VMEM((3, 9, 32, 128), u32),
            pltpu.VMEM((NR, 2, 4, XR, 128), u32),
            pltpu.VMEM((NR, 2, 4, 8, 128), u32),
            pltpu.VMEM((NR, 2, 4, W, 128), u32),
            pltpu.VMEM((NR, 2, 4, 8, 128), u32),
            pltpu.VMEM((2, 4, NS, 16, 128), u32),
            pltpu.VMEM((2, 34, C, W), bf16),
            pltpu.VMEM((3, 32, C, W), bf16),
            pltpu.VMEM((2, 2, NS, 16, 128), u32),
            pltpu.SemaphoreType.DMA((9,)),
        ],
        compiler_params=pltpu.CompilerParams(
            dimension_semantics=("arbitrary",), vmem_limit_bytes=64 * 1024 * 1024,
            disable_bounds_checks=True),
        name="nat_kernel",
    )(xt, wqkv, wo)
    return jnp.transpose(out, (0, 2, 1)).reshape(1, H, W, C)
```

```python
import math

import jax
import jax.numpy as jnp
from jax import lax
from jax.experimental import pallas as pl
from jax.experimental.pallas import tpu as pltpu

H = 384
W = 384
C = 96
NP = 12
NB = 24
NS = 24
NR = 4
XR = W + 16
BIG = 2.0 ** 100
ONE = 0x3F80
ONE2 = 0x3F803F80
NBIG = 0xF180
RM = 14
CM = 15
L_COL = 110
L_ONE = 125
L_PAD = 126
D = 12
E = 8
POFF = 6
NFILL = 4
PEND = -8
PE1 = -8
FPOS = -6
FSTEP = 0
LE = 8
LOFF = 0
LSTEP = 1
DF = 6
S1POS = 1
LEND = 4
TPOS = 10
ORD = 'aAbB'
OPS = [(c, ORD[i + 1:i + 2].isdigit() and int(ORD[i + 1]) or 0) for i, c in enumerate(ORD) if c.isalpha()]

IN_PARTS = [(0, 2, 4), (0, 6, 4), (0, 10, 4), (0, 14, 4), (0, 18, 8), (0, 26, 8), (1, 0, 10), (1, 10, 8), (1, 18, 16)]
KPRE_UNITS = [(pr, k, m) for k in range(4) for pr in range(2) for m in range(3)]

bf16 = jnp.bfloat16
f32 = jnp.float32
u32 = jnp.uint32
i32 = jnp.int32


def _iota(shape, dim):
    return lax.broadcasted_iota(i32, shape, dim)


def _nt(a, b):
    return lax.dot_general(a, b, (((1,), (1,)), ((), ())), preferred_element_type=f32)


def _nn(a, b):
    return lax.dot_general(a, b, (((1,), (0,)), ((), ())), preferred_element_type=f32)


def _unpack(u, idx):
    return pltpu.unpack_elementwise(u, index=idx, packed_dtype=bf16, unpacked_dtype=f32)


def _packi(a, b):
    return pltpu.pack_elementwise([a, b], packed_dtype=bf16)


def _b(u):
    return pltpu.bitcast(u, bf16)


def _u(b):
    return pltpu.bitcast(b, u32)


def _s2(start):
    return pl.ds(start, 8, stride=2)


VSTRIPS = [(pc, j) for j in range(NS) for pc in range(2)] + [(0, NS)]
NV = len(VSTRIPS)
PRE_UNITS = [(pr, k, m) for pr in range(2) for k in range(4) for m in range(3)]
LATE_UNITS = [(2 * i + 1, 2) for i in range(8)]
EARLY_UNITS = [(h, m) for h in range(16) for m in range(3) if (h, m) not in LATE_UNITS]


def _kernel(x_hbm, wqkv_hbm, wo_hbm, out_ref,
            wqkv_ref, wo_ref, at_ref, bt_ref, augx_ref, augq_ref, x2_ref, xs_ref, q2_ref, qs_ref, ow_ref,
            xbuf_ref, obuf_ref, owf_ref, sem):
    t = pl.program_id(0)
    sub8 = _iota((8, 128), 0)
    lane8 = _iota((8, 128), 1)
    pad_word = jnp.where(lane8 == L_PAD, jnp.uint32(ONE2), jnp.uint32(0))
    lo4 = sub8 < 4

    def _setup_weights():
        wq = wqkv_ref[:, 0:C]
        wk = wqkv_ref[:, C:2 * C]
        wv = wqkv_ref[:, 2 * C:3 * C]
        pl_ = _iota((C, C), 0)
        pc_ = _iota((C, C), 1)
        perm = jnp.where(pc_ == jnp.where(pl_ < C // 2, 2 * pl_, 2 * (pl_ - C // 2) + 1), 1.0, 0.0).astype(bf16)
        at = (_nt(wk, wq) * (C ** -0.5 * math.log2(math.e))).astype(bf16)
        at_ref[...] = _u(_nn(perm, at).astype(bf16))
        b = _nn(wv, wo_ref[...]).astype(bf16)
        bt = _nn(perm, b).T
        bt = jnp.concatenate([bt, jnp.zeros((C, 128 - C), f32)], axis=1)
        bt = jnp.concatenate([bt, jnp.zeros((112 - C, 128), f32)], axis=0)
        r = _iota((112, 128), 0)
        c = _iota((112, 128), 1)
        bt_ref[...] = _u(jnp.where((r == C) & (c == L_ONE), 1.0, bt).astype(bf16))

    def _setup_tables():
        rho = _iota((32, 128), 0)
        for m in range(3):
            ccol = (m * 128 + _iota((32, 128), 1)) // 2
            kcol = ((rho >= 14) & (rho < 29) & (rho - 14 == ccol % CM)) | (rho == 29)
            ccq = jnp.clip(ccol, 3, 188) % CM
            qcol = ((rho >= 14) & (rho < 29) & (((rho - 14 - ccq + 3 + CM) % CM) > 6)) | (rho == 30)

            def kaug(res):
                return rho == 30 if res is None else kcol | (rho == res)

            def qaug(res):
                return qcol | ((rho < 14) & (((rho - res + 3 + RM) % RM) > 6))

            def words(lo, hi, bits):
                return (jnp.where(lo, jnp.uint32(bits), jnp.uint32(0))
                        | jnp.where(hi, jnp.uint32(bits << 16), jnp.uint32(0)))
            kvar = [(2 * v + 1, (2 * v + 2) % RM) for v in range(7)] + [(None, 0), (191 % RM, None)]
            qvar = [(2 * v, 2 * v + 1) for v in range(7)] + [(3, 3), (188 % RM, 188 % RM)]
            for v in range(9):
                augx_ref[m, v] = words(kaug(kvar[v][0]), kaug(kvar[v][1]), ONE)
                augq_ref[m, v] = words(qaug(qvar[v][0]), qaug(qvar[v][1]), NBIG)
        pad_plane = jnp.where(_iota((XR, 128), 1) == L_PAD, jnp.uint32(ONE2), jnp.uint32(0))
        for pr in range(2):
            for sl in range(NR):
                for p in range(4):
                    x2_ref[sl, pr, p, 0:8] = pad_word
                    x2_ref[sl, pr, p, XR - 8:XR] = pad_word
                    if sl == 0 and p < 2:
                        x2_ref[sl, pr, p] = pad_plane
                        xs_ref[sl, pr, p] = pad_word
        xbuf_ref[0, 0:2] = jnp.zeros((2, C, W), bf16)

    colpatch_lane = (lane8 >= L_COL) & (lane8 < L_ONE)
    klabel = jnp.where(lane8 - L_COL == 7 + sub8, jnp.uint32(ONE2), jnp.uint32(0))
    qlabel = jnp.where(lane8 - L_COL < 8, jnp.uint32(NBIG * 0x10001), jnp.uint32(0))

    def key_words(xa, xb, aug, tile, pr, p, m, dup=None):
        slot = tile % NR
        w = jnp.concatenate([_packi(_unpack(xa, 0), _unpack(xb, 0)), _packi(_unpack(xa, 1), _unpack(xb, 1)), aug],
                            axis=0)
        wt = w.T
        for sl_, p_ in [(slot, p)] + ([dup] if dup else []):
            x2_ref[sl_, pr, p_, 8 + 128 * m:8 + 128 * (m + 1)] = wt
            if m == 2:
                xs_ref[sl_, pr, p_] = jnp.where(colpatch_lane, klabel, x2_ref[sl_, pr, p_, _s2(8 + 369)])

    def pre_unit(xsrc, r0, blk, tile, pr, k, m, dup=None):
        rows = [xsrc[r0 + 2 * il + pr, :, m * 128:(m + 1) * 128] for il in (2 * k - 1, 2 * k, 2 * k + 1)]
        ra = 8 * blk + 2 * k
        vx = jnp.where(ra < 1, 7, ((ra + RM - 1) % RM) // 2)
        vq = jnp.where(ra < 3, 7, jnp.where(ra >= 188, 8, (ra % RM) // 2))
        key_words(_u(rows[0]), _u(rows[1]), augx_ref[m, vx], tile + k // 2, pr, (k + 2) % 4, m, dup)
        at = _b(at_ref[...])
        qw = jnp.concatenate([_packi(_nn(at, rows[1]), _nn(at, rows[2])), augq_ref[m, vq]], axis=0)
        slot = tile % NR
        q2_ref[slot, pr, k, 128 * m:128 * (m + 1)] = qw.T
        if m == 2:
            qs_ref[slot, pr, k] = jnp.where(lo4, q2_ref[slot, pr, k, _s2(1)],
                                            jnp.where(colpatch_lane, qlabel, q2_ref[slot, pr, k, _s2(368)]))

    def keytile(tiles_pairs, pr, vi):
        pc, j = VSTRIPS[vi]
        vs = []
        for tile, p in tiles_pairs:
            if j == NS:
                vs += [x2_ref[tile % NR, pr, p, _s2(8)], xs_ref[tile % NR, pr, p]]
            else:
                vs += [x2_ref[tile % NR, pr, p, _s2(16 * j + pc)], x2_ref[tile % NR, pr, p, _s2(16 * j + 16 + pc)]]
        return _b(jnp.concatenate(vs, axis=0))

    def qrows(tiles_pairs, pr, vi):
        pc, j = VSTRIPS[vi]
        return [qs_ref[tile % NR, pr, k] if j == NS else q2_ref[tile % NR, pr, k, _s2(16 * j + pc)]
                for tile, k in tiles_pairs]

    def out_unit(dst, r0, h, m):
        pr = h % 2
        i = h // 2
        w = _b(jnp.concatenate([ow_ref[pr, i // 2, 8 * m + v, _s2(i % 2), :] for v in range(8)], axis=0))
        r = _nt(_b(bt_ref[...]), w)
        inv = 1.0 / r[C:C + 1]
        dst[r0 + h, :, m * 128:(m + 1) * 128] = (r[0:C] * inv).astype(bf16)

    def in_copy(p):
        return pltpu.make_async_copy(x_hbm.at[pl.ds(32 * p - 2, 34)], xbuf_ref.at[p % 2], sem.at[p % 2])

    def in_part(i):
        b, r0, nr = IN_PARTS[i]
        return pltpu.make_async_copy(x_hbm.at[pl.ds(32 * b - 2 + r0, nr)], xbuf_ref.at[b, pl.ds(r0, nr)],
                                     sem.at[5 + i])

    def w_copy(i):
        return pltpu.make_async_copy((wqkv_hbm, wo_hbm)[i], (wqkv_ref, wo_ref)[i], sem.at[14 + i])

    def out_copy(p, r0=0, nr=32):
        return pltpu.make_async_copy(obuf_ref.at[p % 3, pl.ds(r0, nr)], out_ref.at[pl.ds(32 * p + r0, nr)],
                                     sem.at[2 + p % 3])

    def out_part(r0, nr, c0, nc, si):
        return pltpu.make_async_copy(obuf_ref.at[(NP - 1) % 3, pl.ds(r0, nr), :, pl.ds(c0, nc)],
                                     out_ref.at[pl.ds(32 * (NP - 1) + r0, nr), :, pl.ds(c0, nc)], sem.at[si])

    def colidx(n):
        r = _iota((n, 128), 0)
        return 4 * ((r // 8) % 2) + (r % 8) // 2

    def store_pair(res, key0, key1, keysp, j, col):
        o0 = res.pop(key0)
        o1 = res.pop(key1)
        if j == 0:
            o1 = jnp.where(col < 3, res[keysp], o1)
        if j == NS - 1:
            o0 = jnp.where(col >= 5, res.pop(keysp), o0)
        return _packi(o0, o1)

    def attn_stage(base, blk0, nsub, with_pre, xsrc, o_prev, o_cur, o_prev_r0, o_cur_r0, top, calls=(), bot=False):
        tiles = []
        for pr in range(2):
            order = [NV - 1] + list(range(NV - 1))
            tiles += [(pr, vi) for vi in order]
        nt = len(tiles)
        gtiles = [(d,) + tl for d in range(nsub) for tl in tiles]
        ntot = len(gtiles)
        col = colidx(64)
        sl = _iota((32, 128), 0)
        ln = _iota((32, 128), 1)
        mnew = (2 * (ln // 32) + ln % 2) <= (2 + 2 * (sl // 16) + sl % 2)
        topmask = (sl < 16) | (sl % 2 == 0)
        svals = {}
        pvals = {}
        res = {}

        def tile_a(d, pr, vi):
            g = base + d
            return keytile([(g + 1, 0), (g, 1), (g, 2), (g, 3)], pr, vi)

        def tile_b(d, pr, vi):
            return keytile([(base + d + 1, p) for p in range(4)], pr, vi)

        def cross(d, pr):
            return bot and d == nsub - 1 and pr == 1

        def cross_top(d, pr):
            return top and d == 0 and pr == 0

        def qka(d, pr, vi):
            ql = qrows([(base + d, k) for k in range(3)], pr, vi)
            if cross_top(d, pr):
                ql = ql + qrows([(base, 0), (base, 1)], 1, vi)
            svals[(d, pr, vi)] = _nt(_b(jnp.concatenate(ql, axis=0)), tile_a(d, pr, vi))

        def qkb(d, pr, vi):
            ql = qrows([(base + d, k) for k in range(1, 4)], pr, vi)
            if cross(d, pr):
                ql = ql + qrows([(base + d, 2), (base + d, 3)], 0, vi)
            sb = _nt(_b(jnp.concatenate(ql, axis=0)), tile_b(d, pr, vi))
            sa = svals.pop((d, pr, vi))
            comb = jnp.concatenate([sa[0:16], jnp.maximum(sa[16:48], sb[0:32]), sb[32:]]
                                   + ([sa[48:80]] if cross_top(d, pr) else []), axis=0)
            m = jnp.max(comb, axis=1, keepdims=True)
            e = jnp.exp2(comb - m)
            ne = 64 if cross_top(d, pr) else e.shape[0]
            pn = jnp.concatenate([jnp.where(mnew, e[16:48], 0.0), e[48:ne]], axis=0).astype(bf16)
            po = jnp.concatenate([e[0:16], jnp.where(mnew, 0.0, e[16:48])]
                                 + ([e[64:96]] if cross_top(d, pr) else []), axis=0).astype(bf16)
            pvals[(d, pr, vi)] = (pn, po)

        def pva(d, pr, vi):
            res[(pr, vi, 'a')] = _nn(pvals[(d, pr, vi)][1], tile_a(d, pr, vi))

        def pvb(d, pr, vi):
            pn, po = pvals.pop((d, pr, vi))
            o = _nn(pn, tile_b(d, pr, vi))
            oa = res.pop((pr, vi, 'a'))
            res[(pr, vi)] = jnp.concatenate([oa[0:16], oa[16:48] + o[0:32], o[32:48]], axis=0)
            if cross(d, pr):
                res[('x', vi)] = o[48:80]
            if cross_top(d, pr):
                res[('x', vi)] = oa[48:80]
            if vi < 2 * NS and vi % 2 == 1:
                j = vi // 2
                w = store_pair(res, (pr, vi - 1), (pr, vi), (pr, NV - 1), j, col)
                if cross_top(d, 1 - pr):
                    w = jnp.concatenate([jnp.where(topmask, owf_ref[:, j].reshape(32, 128), w[0:32]), w[32:64]],
                                        axis=0)
                ow_ref[pr, :, j] = w.reshape(4, 16, 128)
                if cross(d, pr):
                    wx = store_pair(res, ('x', vi - 1), ('x', vi), ('x', NV - 1), j, col[0:32])
                    ow_ref[0, 3, j] = wx[16:32]
                    ow_ref[0, 2, j] = jnp.where(_iota((16, 128), 0) % 2 == 1, wx[0:16], ow_ref[0, 2, j])
                if cross_top(d, pr):
                    wx = store_pair(res, ('x', vi - 1), ('x', vi), ('x', NV - 1), j, col[0:32])
                    owf_ref[:, j] = wx.reshape(2, 16, 128)

        extra = {}
        mark = {}
        for d in range(nsub):
            off = d * nt
            dst_late = (o_prev, o_prev_r0) if d == 0 else (o_cur, o_cur_r0 + 16 * (d - 1))
            dst = (o_cur, o_cur_r0 + 16 * d)
            for n, (h, m) in enumerate([] if top and d == 0 else LATE_UNITS):
                pos_ = LOFF + LSTEP * n if d == 0 else off + D + LE + 2 * n
                extra.setdefault(pos_, []).append(('o', dst_late, h, m))
                mark['late', d] = max(mark.get(('late', d), 0), pos_)
            for h, m in EARLY_UNITS:
                pr, i = h % 2, h // 2
                if cross(d, 1) and pr == 0 and i >= 5:
                    if m == 2:
                        continue
                    pr = 1
                ready = pr * NV + 1 + 16 * (m + 1) - 1 + D
                pos_ = off + ready + E + 2 * i
                if with_pre and d == nsub - 1 and pr == 1 and m == 1 and i >= 8 - NFILL:
                    pos_ = ntot + D + FPOS + (FSTEP * (i - 8 + NFILL)) // 2
                extra.setdefault(pos_, []).append(('o', dst, h, m))
                mark['early', d] = max(mark.get(('early', d), 0), pos_)
            if with_pre:
                span = nt + (PEND if d == nsub - 1 else 0) - (POFF if d == 0 else 0)
                start = off + (POFF if d == 0 else 0)
                for n, un in enumerate(KPRE_UNITS if top else PRE_UNITS):
                    pos_ = start + (n * span) // len(PRE_UNITS)
                    if top and (d, n) in ((0, 12), (1, 0)):
                        extra.setdefault(pos_, []).append(('c', lambda i=7 + d: in_part(i).wait()))
                        if d == 1:
                            extra[pos_].append(('c', lambda: in_copy(2).start()))
                    extra.setdefault(pos_, []).append(('p', d) + un)
        if bot:
            ends = [(h, 2) for h in (1, 3, 5, 7, 9, 10, 11, 12, 13, 14, 15)]
            for n, (h, m) in enumerate(ends):
                extra.setdefault(ntot + D + LEND, []).append(('o', (o_cur, o_cur_r0 + 16 * (nsub - 1)), h, m))
        mark['end'] = max(extra)
        for pos_, fn in calls:
            extra.setdefault(mark.get(pos_, pos_), []).append(('c', fn))
        nslot = max([ntot + D + 2] + [k + 1 for k in extra])
        for n in range(nslot):
            for op, lag in OPS:
                k = n - lag - (D if op in 'AB' else 0)
                if 0 <= k < ntot:
                    {'a': qka, 'b': qkb, 'A': pva, 'B': pvb}[op](*gtiles[k])
            for e in extra.get(n, []):
                if e[0] == 'o':
                    out_unit(e[1][0], e[1][1], e[2], e[3])
                elif e[0] == 'c':
                    e[1]()
                else:
                    d = e[1]
                    pre_unit(xsrc, 2 + 16 * d, blk0 + 2 + d, base + 2 + d, *e[2:])

    def main_block(par):
        attn_stage(2 * par + 2, 2 * t - 2, 2, True, xbuf_ref.at[par], obuf_ref.at[(t + 1) % 3],
                   obuf_ref.at[(t + 2) % 3], 16, 0, False)

    @pl.when(t == 0)
    def _():
        w_copy(0).start()
        w_copy(1).start()
        for i in range(6 if S1POS else 9):
            in_part(i).start()
        _setup_tables()
        w_copy(0).wait()
        w_copy(1).wait()
        in_part(0).wait()
        _setup_weights()
        for k in range(4):
            if k > 0:
                in_part(k).wait()
            if k == S1POS > 0:
                for i in range(6, 9):
                    in_part(i).start()
            for pr in range(2):
                for m in range(3):
                    pre_unit(xbuf_ref.at[0], 2, 0, 0, pr, k, m, (0, 1) if (pr, k) == (0, 3) else None)
        for k in range(4):
            if k % 2 == 0:
                in_part(4 + k // 2).wait()
            for pr in range(2):
                for m in range(3):
                    pre_unit(xbuf_ref.at[0], 18, 1, 1, pr, k, m)

    @pl.when(t >= 1)
    def _():
        @pl.when((t >= 2) & (t < NP))
        def _():
            in_copy(t).wait()

        @pl.when((t >= 2) & (t < NP - 1))
        def _():
            in_copy(t + 1).start()

        @pl.when(t >= 4)
        def _():
            out_copy(t - 4).wait()

    @pl.when(t == 1)
    def _():
        in_part(6).wait()
        attn_stage(0, 0, 2, True, xbuf_ref.at[1], None, obuf_ref.at[0], 0, 0, True)

    for par in range(2):
        @pl.when((t >= 2) & (t < NP) & (t % 2 == par))
        def _():
            main_block(par)

    @pl.when((t >= 2) & (t < NP))
    def _():
        out_copy(t - 2).start()

    @pl.when(t == NP)
    def _():
        last = obuf_ref.at[(NP - 1) % 3]
        prev = obuf_ref.at[(NP - 2) % 3]

        def tail_keys(pr, m):
            xa = _u(xbuf_ref[(NP - 1) % 2, 32 + pr, :, m * 128:(m + 1) * 128])
            key_words(xa, jnp.zeros_like(xa), augx_ref[m, 8], NB, pr, 2, m)

        def tail_fill():
            x2_ref[NB % NR, 0, 3] = jnp.where(_iota((XR, 128), 1) == L_PAD, jnp.uint32(ONE2), jnp.uint32(0))
            xs_ref[NB % NR, 0, 3] = pad_word
            x2_ref[NB % NR, 1, 3] = x2_ref[(NB - 1) % NR, 1, 3]
            xs_ref[NB % NR, 1, 3] = xs_ref[(NB - 1) % NR, 1, 3]

        calls = [(TPOS + 6 * n, lambda pr=n // 3, m=n % 3: tail_keys(pr, m)) for n in range(6)]
        calls += [(TPOS + 36, tail_fill),
                  (('late', 0), lambda: out_copy(NP - 2).start()),
                  (('late', 1), lambda: out_copy(NP - 1, 0, 16).start()),
                  (('early', 1), lambda: out_part(16, 16, 0, 256, 5).start()),
                  ('end', lambda: out_part(16, 16, 256, 128, 6).start())]
        attn_stage(NB - 2, NB - 2, 2, False, None, prev, last, 16, 0, False, calls, True)
        out_copy(NP - 3).wait()
        out_copy(NP - 2).wait()
        out_copy(NP - 1, 0, 16).wait()
        out_part(16, 16, 0, 256, 5).wait()
        out_part(16, 16, 256, 128, 6).wait()


@jax.jit
def pallas_standalone__neighborhood_nat__vision_kernel(x, wqkv, wo):
    xt = jnp.transpose(x.reshape(H, W, C), (0, 2, 1))
    out = pl.pallas_call(
        _kernel,
        grid=(NP + 1,),
        in_specs=[
            pl.BlockSpec(memory_space=pl.ANY),
            pl.BlockSpec(memory_space=pl.ANY),
            pl.BlockSpec(memory_space=pl.ANY),
        ],
        out_specs=pl.BlockSpec(memory_space=pl.ANY),
        out_shape=jax.ShapeDtypeStruct((H, C, W), bf16),
        scratch_shapes=[
            pltpu.VMEM((C, 3 * C), bf16),
            pltpu.VMEM((C, C), bf16),
            pltpu.VMEM((48, 96), u32),
            pltpu.VMEM((56, 128), u32),
            pltpu.VMEM((3, 9, 32, 128), u32),
            pltpu.VMEM((3, 9, 32, 128), u32),
            pltpu.VMEM((NR, 2, 4, XR, 128), u32),
            pltpu.VMEM((NR, 2, 4, 8, 128), u32),
            pltpu.VMEM((NR, 2, 4, W, 128), u32),
            pltpu.VMEM((NR, 2, 4, 8, 128), u32),
            pltpu.VMEM((2, 4, NS, 16, 128), u32),
            pltpu.VMEM((2, 34, C, W), bf16),
            pltpu.VMEM((3, 32, C, W), bf16),
            pltpu.VMEM((2, NS, 16, 128), u32),
            pltpu.SemaphoreType.DMA((16,)),
        ],
        compiler_params=pltpu.CompilerParams(
            dimension_semantics=("arbitrary",), vmem_limit_bytes=64 * 1024 * 1024,
            disable_bounds_checks=True),
        name="nat_kernel",
    )(xt, wqkv, wo)
    return jnp.transpose(out, (0, 2, 1)).reshape(1, H, W, C)
```

```python
import math

import jax
import jax.numpy as jnp
from jax import lax
from jax.experimental import pallas as pl
from jax.experimental.pallas import tpu as pltpu

H = 384
W = 384
C = 96
NP = 12
NB = 24
NS = 24
NR = 4
XR = W + 16
BIG = 2.0 ** 100
ONE = 0x3F80
ONE2 = 0x3F803F80
NBIG = 0xF180
RM = 14
CM = 15
L_COL = 110
L_ONE = 125
L_PAD = 126
D = 13
E = 7
POFF = 14
NFILL = 5
PEND = -7
PE1 = -8
FPOS = -7
FSTEP = 1
LE = 4
LOFF = 1
LSTEP = 1
DF = 6
S1POS = 1
LST = 0
SKT = 1
SKB = 1
EB = 8
SB = 2
DLY = 4
WSEP = 1
WORD = 0
ONEB = 1
KORD = 1
PS = -5
EL = 8
SPL = 2
LEAD = 49
LEL = 4
LOFL = 0
LEND = 3
TPOS = 40
POFF1 = 10
PEND1 = -12
NFILL1 = 5
FPOS1 = -8
FSTEP1 = 0
PS1 = 99
LE1 = 4
E1 = 8
D1 = 12
DL = 12
MAIN = (POFF, PEND, NFILL, FPOS, FSTEP, PS, LE, E, D)
FIRST = (POFF1, PEND1, NFILL1, FPOS1, FSTEP1, PS1, LE1, E1, D1)
LAST = (POFF, PEND, NFILL, FPOS, FSTEP, PS, LE, E, DL)
ORD = 'aAbB'
OPS = [(c, ORD[i + 1:i + 2].isdigit() and int(ORD[i + 1]) or 0) for i, c in enumerate(ORD) if c.isalpha()]

IN_PARTS = [(0, 2, 4), (0, 6, 4), (0, 10, 4), (0, 14, 4), (0, 18, 8), (0, 26, 8), (1, 0, 10), (1, 10, 8), (1, 18, 16)]
OUT_PARTS = [(0, 8, 1, 0, W, 1, 2), (5, 3, 0, 0, W, 1, 2), (0, 5, 0, 0, W, 0, 2)]
KPRE_UNITS = [(pr, k, m) for k in range(4) for pr in range(2) for m in range(3)]

bf16 = jnp.bfloat16
f32 = jnp.float32
u32 = jnp.uint32
i32 = jnp.int32


def _iota(shape, dim):
    return lax.broadcasted_iota(i32, shape, dim)


def _nt(a, b):
    return lax.dot_general(a, b, (((1,), (1,)), ((), ())), preferred_element_type=f32)


def _nn(a, b):
    return lax.dot_general(a, b, (((1,), (0,)), ((), ())), preferred_element_type=f32)


def _unpack(u, idx):
    return pltpu.unpack_elementwise(u, index=idx, packed_dtype=bf16, unpacked_dtype=f32)


def _packi(a, b):
    return pltpu.pack_elementwise([a, b], packed_dtype=bf16)


def _b(u):
    return pltpu.bitcast(u, bf16)


def _u(b):
    return pltpu.bitcast(b, u32)


def _s2(start):
    return pl.ds(start, 8, stride=2)


VSTRIPS = [(pc, j) for j in range(NS) for pc in range(2)] + [(0, NS)]
NV = len(VSTRIPS)
PRE_UNITS = [(pr, k, m) for pr in range(2) for k in range(4) for m in range(3)]
LATE_UNITS = [(2 * i + 1, 2) for i in range(8)]
EARLY_UNITS = [(h, m) for h in range(16) for m in range(3) if (h, m) not in LATE_UNITS]


def _kernel(x_hbm, wqkv_hbm, wo_hbm, out_ref,
            wqkv_ref, wo_ref, at_ref, bt_ref, augx_ref, augq_ref, x2_ref, xs_ref, q2_ref, qs_ref, ow_ref,
            xbuf_ref, obuf_ref, sem):
    t = pl.program_id(0)
    sub8 = _iota((8, 128), 0)
    lane8 = _iota((8, 128), 1)
    pad_word = jnp.where(lane8 == L_PAD, jnp.uint32(ONE2), jnp.uint32(0))
    lo4 = sub8 < 4

    def _setup_weights():
        wq = wqkv_ref[:, 0:C]
        wk = wqkv_ref[:, C:2 * C]
        wv = wqkv_ref[:, 2 * C:3 * C]
        pl_ = _iota((C, C), 0)
        pc_ = _iota((C, C), 1)
        perm = jnp.where(pc_ == jnp.where(pl_ < C // 2, 2 * pl_, 2 * (pl_ - C // 2) + 1), 1.0, 0.0).astype(bf16)
        at = (_nt(wk, wq) * (C ** -0.5 * math.log2(math.e))).astype(bf16)
        at_ref[...] = _u(_nn(perm, at).astype(bf16))
        b = _nn(wv, wo_ref[...]).astype(bf16)
        bt = _nn(perm, b).T
        bt = jnp.concatenate([bt, jnp.zeros((C, 128 - C), f32)], axis=1)
        bt = jnp.concatenate([bt, jnp.zeros((112 - C, 128), f32)], axis=0)
        r = _iota((112, 128), 0)
        c = _iota((112, 128), 1)
        bt_ref[...] = _u(jnp.where((r == C) & (c == L_ONE), 1.0, bt).astype(bf16))

    def _setup_tables():
        rho = _iota((32, 128), 0)
        for m in range(3):
            ccol = (m * 128 + _iota((32, 128), 1)) // 2
            kcol = ((rho >= 14) & (rho < 29) & (rho - 14 == ccol % CM)) | (rho == 29)
            ccq = jnp.clip(ccol, 3, 188) % CM
            qcol = ((rho >= 14) & (rho < 29) & (((rho - 14 - ccq + 3 + CM) % CM) > 6)) | (rho == 30)

            def kaug(res):
                return rho == 30 if res is None else kcol | (rho == res)

            def qaug(res):
                return qcol | ((rho < 14) & (((rho - res + 3 + RM) % RM) > 6))

            def words(lo, hi, bits):
                return (jnp.where(lo, jnp.uint32(bits), jnp.uint32(0))
                        | jnp.where(hi, jnp.uint32(bits << 16), jnp.uint32(0)))
            kvar = [(2 * v + 1, (2 * v + 2) % RM) for v in range(7)] + [(None, 0), (191 % RM, None)]
            qvar = [(2 * v, 2 * v + 1) for v in range(7)] + [(3, 3), (188 % RM, 188 % RM)]
            for v in range(9):
                augx_ref[m, v] = words(kaug(kvar[v][0]), kaug(kvar[v][1]), ONE)
                augq_ref[m, v] = words(qaug(qvar[v][0]), qaug(qvar[v][1]), NBIG)
        pad_plane = jnp.where(_iota((XR, 128), 1) == L_PAD, jnp.uint32(ONE2), jnp.uint32(0))
        for pr in range(2):
            for sl in range(NR):
                for p in range(4):
                    x2_ref[sl, pr, p, 0:8] = pad_word
                    x2_ref[sl, pr, p, XR - 8:XR] = pad_word
                    if sl == 0 and p < 2:
                        x2_ref[sl, pr, p] = pad_plane
                        xs_ref[sl, pr, p] = pad_word
        xbuf_ref[0, 0:2] = jnp.zeros((2, C, W), bf16)

    colpatch_lane = (lane8 >= L_COL) & (lane8 < L_ONE)
    klabel = jnp.where(lane8 - L_COL == 7 + sub8, jnp.uint32(ONE2), jnp.uint32(0))
    qlabel = jnp.where(lane8 - L_COL < 8, jnp.uint32(NBIG * 0x10001), jnp.uint32(0))

    def key_words(xa, xb, aug, tile, pr, p, m, dup=None):
        slot = tile % NR
        w = jnp.concatenate([_packi(_unpack(xa, 0), _unpack(xb, 0)), _packi(_unpack(xa, 1), _unpack(xb, 1)), aug],
                            axis=0)
        wt = w.T
        for sl_, p_ in [(slot, p)] + ([dup] if dup else []):
            x2_ref[sl_, pr, p_, 8 + 128 * m:8 + 128 * (m + 1)] = wt
            if m == 2:
                xs_ref[sl_, pr, p_] = jnp.where(colpatch_lane, klabel, x2_ref[sl_, pr, p_, _s2(8 + 369)])

    def pre_unit(xsrc, r0, blk, tile, pr, k, m, dup=None, part=3):
        rows = [xsrc[r0 + 2 * il + pr, :, m * 128:(m + 1) * 128] for il in (2 * k - 1, 2 * k, 2 * k + 1)]
        ra = 8 * blk + 2 * k
        vx = jnp.where(ra < 1, 7, ((ra + RM - 1) % RM) // 2)
        vq = jnp.where(ra < 3, 7, jnp.where(ra >= 188, 8, (ra % RM) // 2))
        if part & 1:
            key_words(_u(rows[0]), _u(rows[1]), augx_ref[m, vx], tile + k // 2, pr, (k + 2) % 4, m, dup)
        if not part & 2:
            return
        at = _b(at_ref[...])
        qw = jnp.concatenate([_packi(_nn(at, rows[1]), _nn(at, rows[2])), augq_ref[m, vq]], axis=0)
        slot = tile % NR
        q2_ref[slot, pr, k, 128 * m:128 * (m + 1)] = qw.T
        if m == 2:
            qs_ref[slot, pr, k] = jnp.where(lo4, q2_ref[slot, pr, k, _s2(1)],
                                            jnp.where(colpatch_lane, qlabel, q2_ref[slot, pr, k, _s2(368)]))

    def keytile(tiles_pairs, pr, vi):
        pc, j = VSTRIPS[vi]
        vs = []
        for tile, p in tiles_pairs:
            if j == NS:
                vs += [x2_ref[tile % NR, pr, p, _s2(8)], xs_ref[tile % NR, pr, p]]
            else:
                vs += [x2_ref[tile % NR, pr, p, _s2(16 * j + pc)], x2_ref[tile % NR, pr, p, _s2(16 * j + 16 + pc)]]
        return _b(jnp.concatenate(vs, axis=0))

    def qrows(tiles_pairs, pr, vi):
        pc, j = VSTRIPS[vi]
        return [qs_ref[tile % NR, pr, k] if j == NS else q2_ref[tile % NR, pr, k, _s2(16 * j + pc)]
                for tile, k in tiles_pairs]

    def out_unit(dst, r0, h, m):
        pr = h % 2
        i = h // 2
        w = _b(jnp.concatenate([ow_ref[pr, i // 2, 8 * m + v, _s2(i % 2), :] for v in range(8)], axis=0))
        r = _nt(_b(bt_ref[...]), w)
        inv = 1.0 / r[C:C + 1]
        dst[(r0 + h) // 2, h % 2, :, m * 128:(m + 1) * 128] = (r[0:C] * inv).astype(bf16)

    def in_copy(p):
        return pltpu.make_async_copy(x_hbm.at[pl.ds(32 * p - 2, 34)], xbuf_ref.at[p % 2], sem.at[p % 2])

    def in_part(i):
        b, r0, nr = IN_PARTS[i]
        return pltpu.make_async_copy(x_hbm.at[pl.ds(32 * b - 2 + r0, nr)], xbuf_ref.at[b, pl.ds(r0, nr)],
                                     sem.at[5 + i])

    def w_copy(i):
        return pltpu.make_async_copy((wqkv_hbm, wo_hbm)[i], (wqkv_ref, wo_ref)[i], sem.at[14 + i])

    def out_copy(p, half):
        return pltpu.make_async_copy(obuf_ref.at[p % 3, pl.ds(8 * half, 8)], out_ref.at[pl.ds(16 * p + 8 * half, 8)],
                                     sem.at[(2, 16)[half] + p % 3])

    def out_part(i):
        r0, nr, par, c0, nc, _, _ = OUT_PARTS[i]
        return pltpu.make_async_copy(obuf_ref.at[(NP - 1) % 3, pl.ds(8 + r0, nr), par, :, pl.ds(c0, nc)],
                                     out_ref.at[pl.ds(16 * (NP - 1) + 8 + r0, nr), par, :, pl.ds(c0, nc)],
                                     sem.at[5 + i])

    def colidx(n):
        r = _iota((n, 128), 0)
        return 4 * ((r // 8) % 2) + (r % 8) // 2

    def store_pair(res, key0, key1, keysp, j, col):
        o0 = res.pop(key0)
        o1 = res.pop(key1)
        if j == 0:
            o1 = jnp.where(col < 3, res[keysp], o1)
        if j == NS - 1:
            o0 = jnp.where(col >= 5, res.pop(keysp), o0)
        return _packi(o0, o1)

    def attn_stage(base, blk0, nsub, with_pre, xsrc, o_prev, o_cur, o_prev_r0, o_cur_r0, top, calls=(), bot=False):
        nt = 2 * NV
        poff_, pend_, nfill_, fpos_, fstep_, ps_, le_, e_, d_ = FIRST if top else LAST if bot else MAIN
        gtiles = []
        for d in range(nsub):
            if bot and d == nsub - 1:
                if LEAD:
                    seq = [NV - 1] + list(range(NV - 1))
                    for n in range(NV + LEAD):
                        gtiles += [(d, 1, seq[n])] if n < NV else []
                        gtiles += [(d, 0, seq[n - LEAD])] if n >= LEAD else []
                else:
                    for m in range(3):
                        for pr in (1, 0):
                            gtiles += [(d, pr, vi)
                                       for vi in ([NV - 1] if m == 0 else []) + list(range(16 * m, 16 * m + 16))]
            else:
                gtiles += [(d, pr, vi) for pr in range(2) for vi in [NV - 1] + list(range(NV - 1))]
        ntot = len(gtiles)
        col = colidx(64)
        sl = _iota((32, 128), 0)
        ln = _iota((32, 128), 1)
        mnew = (2 * (ln // 32) + ln % 2) <= (2 + 2 * (sl // 16) + sl % 2)
        odd16 = _iota((16, 128), 0) % 2 == 1
        svals = {}
        pvals = {}
        res = {}

        def tile_a(d, pr, vi):
            g = base + d
            return keytile([(g + 1, 0), (g, 1), (g, 2), (g, 3)], pr, vi)

        def tile_b(d, pr, vi):
            return keytile([(base + d + 1, p) for p in range(4)], pr, vi)

        def border(d):
            return 'top' if top and d == 0 else 'bot' if bot and d == nsub - 1 else None

        def pairs(d, pr):
            bd = border(d)
            pa, pb = [0, 1, 2], [1, 2, 3]
            if (bd, pr) == ('top', 1) and SKT:
                pa = [1, 2]
            if (bd, pr) == ('bot', 0) and SKB:
                pb = [1, 2]
            return pa, pb, (bd, pr) == ('top', 0), (bd, pr) == ('bot', 1)

        def qka(d, pr, vi):
            pa, _, xa, _ = pairs(d, pr)
            ql = qrows([(base + d, k) for k in pa], pr, vi)
            if xa:
                ql = ql + qrows([(base + d, 0), (base + d, 1)], 1, vi)
            svals[(d, pr, vi)] = _nt(_b(jnp.concatenate(ql, axis=0)), tile_a(d, pr, vi))

        def qkb(d, pr, vi):
            pa, pb, xa, xb = pairs(d, pr)
            ql = qrows([(base + d, k) for k in pb], pr, vi)
            if xb:
                ql = ql + qrows([(base + d, 2), (base + d, 3)], 0, vi)
            sb = _nt(_b(jnp.concatenate(ql, axis=0)), tile_b(d, pr, vi))
            sa = svals.pop((d, pr, vi))
            na = 16 * (len(pa) - 2)
            parts = [sa[0:na]] if na else []
            parts += [jnp.maximum(sa[na:na + 32], sb[0:32])]
            parts += [sb[32:]] if sb.shape[0] > 32 else []
            parts += [sa[48:80]] if xa else []
            comb = jnp.concatenate(parts, axis=0)
            m = jnp.max(comb, axis=1, keepdims=True)
            e = jnp.exp2(comb - m)
            nb = na + 32 + sb.shape[0] - 32
            mid = e[na:na + 32]
            pn = jnp.concatenate([jnp.where(mnew, mid, 0.0)] + ([e[na + 32:nb]] if sb.shape[0] > 32 else []), axis=0)
            po = jnp.concatenate(([e[0:na]] if na else []) + [jnp.where(mnew, 0.0, mid)]
                                 + ([e[nb:]] if xa else []), axis=0)
            pvals[(d, pr, vi)] = (pn.astype(bf16), po.astype(bf16))

        def pva(d, pr, vi):
            res[(pr, vi, 'a')] = _nn(pvals[(d, pr, vi)][1], tile_a(d, pr, vi))

        def pvb(d, pr, vi):
            pa, pb, xa, xb = pairs(d, pr)
            pn, po = pvals.pop((d, pr, vi))
            o = _nn(pn, tile_b(d, pr, vi))
            oa = res.pop((pr, vi, 'a'))
            na = 16 * (len(pa) - 2)
            res[(pr, vi)] = jnp.concatenate(([oa[0:na]] if na else []) + [oa[na:na + 32] + o[0:32]]
                                            + ([o[32:48]] if len(pb) == 3 else []), axis=0)
            if xa or xb:
                res[(pr, vi, 'x')] = oa[48:80] if xa else o[48:80]
            if vi < 2 * NS and vi % 2 == 1:
                j = vi // 2
                w = store_pair(res, (pr, vi - 1), (pr, vi), (pr, NV - 1), j, col[0:16 * (len(pa) + len(pb) - 2)])
                if (border(d), pr) == ('top', 1):
                    w = w[16 * (len(pa) - 2):]
                    ow_ref[pr, 1, j] = jnp.where(odd16, w[0:16], ow_ref[pr, 1, j])
                    ow_ref[pr, 2:4, j] = w[16:48].reshape(2, 16, 128)
                elif (border(d), pr) == ('bot', 0):
                    ow_ref[pr, 0:2, j] = w[0:32].reshape(2, 16, 128)
                    ow_ref[pr, 2, j] = jnp.where(odd16, ow_ref[pr, 2, j], w[32:48])
                else:
                    ow_ref[pr, :, j] = w.reshape(4, 16, 128)
                if xa or xb:
                    wx = store_pair(res, (pr, vi - 1, 'x'), (pr, vi, 'x'), (pr, NV - 1, 'x'), j, col[0:32])
                    p0 = 0 if xa else 2
                    ow_ref[1 - pr, p0:p0 + 2, j] = wx.reshape(2, 16, 128)

        extra = {}
        mark = {}
        done = {}
        for n, (d, pr, vi) in enumerate(gtiles):
            if vi < 2 * NS:
                done[d, pr, vi // 16] = n + d_
        for d in range(nsub):
            off = d * nt
            dst_late = (o_prev, o_prev_r0) if d == 0 else (o_cur, o_cur_r0 + 16 * (d - 1))
            dst = (o_cur, o_cur_r0 + 16 * d)
            for n, (h, m) in enumerate([] if top and d == 0 else LATE_UNITS):
                pos_ = ((LOFL if bot else LOFF) + LSTEP * n if d == 0
                        else off + d_ + (LEL if bot else le_) + 2 * n)
                extra.setdefault(pos_, []).append(('o', dst_late, h, m))
                mark['late', d] = max(mark.get(('late', d), 0), pos_)
            for h, m in (EARLY_UNITS + LATE_UNITS if border(d) == 'bot' else EARLY_UNITS):
                pr, i = h % 2, h // 2
                if border(d) == 'bot' and i >= 5:
                    pr = 1
                pos_ = done[d, pr, m] + e_ + 2 * i
                if bot:
                    pos_ = done[d, pr, m] + EL + SPL * i
                if with_pre and d == nsub - 1 and pr == 1 and m == 1 and i >= 8 - nfill_:
                    pos_ = ntot + d_ + fpos_ + (fstep_ * (i - 8 + nfill_)) // 2
                if border(d) == 'bot':
                    pos_ = done[d, pr, m] + EB + (SB * i) // 2
                if border(d) == 'bot' and m == 2 and pr == 0:
                    pos_ = done[d, pr, m] + LEND + (LST * i) // 2
                extra.setdefault(pos_, []).append(('o', dst, h, m))
                mark['blk', d, pr, m] = max(mark.get(('blk', d, pr, m), 0), pos_)
                mark['col', d, m] = max(mark.get(('col', d, m), 0), pos_)
            if with_pre:
                span = nt + (pend_ if d == nsub - 1 else 0) - (poff_ if d == 0 else 0)
                start = off + (poff_ if d == 0 else 0)
                for n, un in enumerate(KPRE_UNITS if top or KORD else PRE_UNITS):
                    pos_ = start + (n * span) // len(PRE_UNITS)
                    if top and (d, n) in ((0, 12), (1, 0)):
                        if ONEB:
                            if d == 0:
                                extra.setdefault(pos_, []).append(('c', lambda: in_part(7).wait()))
                                extra[pos_].append(('c', lambda: in_part(8).wait()))
                                extra[pos_].append(('c', lambda: in_copy(2).start()))
                        else:
                            extra.setdefault(pos_, []).append(('c', lambda i=7 + d: in_part(i).wait()))
                            if d == 1:
                                extra[pos_].append(('c', lambda: in_copy(2).start()))
                    if ps_ == 99:
                        extra.setdefault(pos_, []).append(('p', d) + un + (None, 3))
                    else:
                        extra.setdefault(pos_ + max(ps_, 0), []).append(('p', d) + un + (None, 2))
                        extra.setdefault(pos_ + max(-ps_, 0), []).append(('p', d) + un + (None, 1))
        mark['end'] = max(extra)
        for pos_, fn in calls:
            pos_ = min(mark[pos_] + DLY, mark['end']) if pos_ in mark else pos_
            extra.setdefault(pos_, []).append(('c', fn))
        nslot = max([ntot + d_ + 2] + [k + 1 for k in extra])
        for n in range(nslot):
            for op, lag in OPS:
                k = n - lag - (d_ if op in 'AB' else 0)
                if 0 <= k < ntot:
                    {'a': qka, 'b': qkb, 'A': pva, 'B': pvb}[op](*gtiles[k])
            for e in extra.get(n, []):
                if e[0] == 'o':
                    out_unit(e[1][0], e[1][1], e[2], e[3])
                elif e[0] == 'c':
                    e[1]()
                else:
                    d = e[1]
                    pre_unit(xsrc, 2 + 16 * d, blk0 + 2 + d, base + 2 + d, *e[2:])

    def main_block(par):
        attn_stage(2 * par + 2, 2 * t - 2, 2, True, xbuf_ref.at[par], obuf_ref.at[(t + 1) % 3],
                   obuf_ref.at[(t + 2) % 3], 16, 0, False)

    def first_block():
        in_part(6).wait()
        attn_stage(0, 0, 2, True, xbuf_ref.at[1], None, obuf_ref.at[0], 0, 0, True)

    def last_block():
        last = obuf_ref.at[(NP - 1) % 3]
        prev = obuf_ref.at[(NP - 2) % 3]

        def tail_keys(pr, m):
            xa = _u(xbuf_ref[(NP - 1) % 2, 32 + pr, :, m * 128:(m + 1) * 128])
            key_words(xa, jnp.zeros_like(xa), augx_ref[m, 8], NB, pr, 2, m)

        def tail_fill():
            x2_ref[NB % NR, 0, 3] = jnp.where(_iota((XR, 128), 1) == L_PAD, jnp.uint32(ONE2), jnp.uint32(0))
            xs_ref[NB % NR, 0, 3] = pad_word
            x2_ref[NB % NR, 1, 3] = x2_ref[(NB - 1) % NR, 1, 3]
            xs_ref[NB % NR, 1, 3] = xs_ref[(NB - 1) % NR, 1, 3]

        calls = [(TPOS + 6 * n, lambda pr=n // 3, m=n % 3: tail_keys(pr, m)) for n in range(6)]
        calls += [(TPOS + 36, tail_fill),
                  (('late', 0), lambda: out_copy(NP - 2, 1).start()),
                  (('late', 1), lambda: out_copy(NP - 1, 0).start()),
                  ]
        calls += [(('blk', 1, part[5], part[6]), lambda i=i: out_part(i).start()) for i, part in enumerate(OUT_PARTS)]
        attn_stage(NB - 2, NB - 2, 2, False, None, prev, last, 16, 0, False, calls, True)
        for p, half in ((NP - 3, 0), (NP - 3, 1), (NP - 2, 0), (NP - 2, 1), (NP - 1, 0)):
            out_copy(p, half).wait()
        for i in range(len(OUT_PARTS)):
            out_part(i).wait()

    @pl.when(t == 0)
    def _():
        if WORD:
            in_part(0).start()
        w_copy(0).start()
        w_copy(1).start()
        for i in range(WORD, 6 if S1POS else 9):
            in_part(i).start()
        _setup_tables()
        w_copy(0).wait()
        w_copy(1).wait()
        if not WSEP:
            in_part(0).wait()
        _setup_weights()
        for k in range(4):
            if k > 0 or WSEP:
                in_part(k).wait()
            if k == S1POS > 0:
                for i in range(6, 9):
                    in_part(i).start()
            for pr in range(2):
                for m in range(3):
                    pre_unit(xbuf_ref.at[0], 2, 0, 0, pr, k, m, (0, 1) if (pr, k) == (0, 3) else None)
        for k in range(4):
            if k % 2 == 0:
                in_part(4 + k // 2).wait()
            for pr in range(2):
                for m in range(3):
                    pre_unit(xbuf_ref.at[0], 18, 1, 1, pr, k, m)

    @pl.when(t >= 1)
    def _():
        @pl.when((t >= 2) & (t < NP))
        def _():
            in_copy(t).wait()

        @pl.when((t >= 2) & (t < NP - 1))
        def _():
            in_copy(t + 1).start()

        @pl.when(t >= 4)
        def _():
            out_copy(t - 4, 0).wait()
            out_copy(t - 4, 1).wait()

    @pl.when(t == 1)
    def _():
        first_block()

    for par in range(2):
        @pl.when((t >= 2) & (t < NP) & (t % 2 == par))
        def _():
            main_block(par)

    @pl.when((t >= 2) & (t < NP))
    def _():
        out_copy(t - 2, 1).start()

    @pl.when((t >= 1) & (t < NP))
    def _():
        out_copy(t - 1, 0).start()

    @pl.when(t == NP)
    def _():
        last_block()


@jax.jit
def pallas_standalone__neighborhood_nat__vision_kernel(x, wqkv, wo):
    xt = jnp.transpose(x.reshape(H, W, C), (0, 2, 1))
    out = pl.pallas_call(
        _kernel,
        grid=(NP + 1,),
        in_specs=[
            pl.BlockSpec(memory_space=pl.ANY),
            pl.BlockSpec(memory_space=pl.ANY),
            pl.BlockSpec(memory_space=pl.ANY),
        ],
        out_specs=pl.BlockSpec(memory_space=pl.ANY),
        out_shape=jax.ShapeDtypeStruct((H // 2, 2, C, W), bf16),
        scratch_shapes=[
            pltpu.VMEM((C, 3 * C), bf16),
            pltpu.VMEM((C, C), bf16),
            pltpu.VMEM((48, 96), u32),
            pltpu.VMEM((56, 128), u32),
            pltpu.VMEM((3, 9, 32, 128), u32),
            pltpu.VMEM((3, 9, 32, 128), u32),
            pltpu.VMEM((NR, 2, 4, XR, 128), u32),
            pltpu.VMEM((NR, 2, 4, 8, 128), u32),
            pltpu.VMEM((NR, 2, 4, W, 128), u32),
            pltpu.VMEM((NR, 2, 4, 8, 128), u32),
            pltpu.VMEM((2, 4, NS, 16, 128), u32),
            pltpu.VMEM((2, 34, C, W), bf16),
            pltpu.VMEM((3, 16, 2, C, W), bf16),
            pltpu.SemaphoreType.DMA((19,)),
        ],
        compiler_params=pltpu.CompilerParams(
            dimension_semantics=("arbitrary",), vmem_limit_bytes=64 * 1024 * 1024,
            disable_bounds_checks=True),
        name="nat_kernel",
    )(xt, wqkv, wo)
    return jnp.transpose(out.reshape(H, C, W), (0, 2, 1)).reshape(1, H, W, C)
```

```python
import math

import jax
import jax.numpy as jnp
from jax import lax
from jax.experimental import pallas as pl
from jax.experimental.pallas import tpu as pltpu

H = 384
W = 384
C = 96
NP = 12
NB = 24
NS = 24
NR = 4
XR = W + 16
BIG = 2.0 ** 100
ONE = 0x3F80
ONE2 = 0x3F803F80
NBIG = 0xF180
RM = 14
CM = 15
L_COL = 110
L_ONE = 125
L_PAD = 126
D = 13
E = 7
POFF = 14
NFILL = 5
PEND = -7
PE1 = -8
FPOS = -7
FSTEP = 1
LE = 4
LOFF = 1
LSTEP = 1
DF = 6
S1POS = 1
LST = 0
SKT = 1
SKB = 1
EB = 8
SB = 2
DLY = 4
WSEP = 1
WORD = 0
ONEB = 1
SPM = 4
PS = -5
EL = 8
SPL = 2
LEAD = 49
LEL = 4
LOFL = 0
CH = 15
CHUNKS = [k for k in range(4) if (CH >> k) & 1]
LEND = 3
TPOS = 40
POFF1 = 10
PEND1 = -12
NFILL1 = 5
FPOS1 = -8
FSTEP1 = 0
PS1 = 99
LE1 = 4
E1 = 8
D1 = 12
DL = 12
MAIN = (POFF, PEND, NFILL, FPOS, FSTEP, PS, LE, E, D)
FIRST = (POFF1, PEND1, NFILL1, FPOS1, FSTEP1, PS1, LE1, E1, D1)
LAST = (POFF, PEND, NFILL, FPOS, FSTEP, PS, LE, E, DL)
PORD = 'kpm'
ORD = 'aAbB'
OPS = [(c, ORD[i + 1:i + 2].isdigit() and int(ORD[i + 1]) or 0) for i, c in enumerate(ORD) if c.isalpha()]

IN_PARTS = [(0, 2, 4), (0, 6, 4), (0, 10, 4), (0, 14, 4), (0, 18, 8), (0, 26, 8), (1, 0, 10), (1, 10, 8), (1, 18, 16)]
KPRE_UNITS = [(pr, k, m) for k in range(4) for pr in range(2) for m in range(3)]

MAIN_UNITS = sorted(KPRE_UNITS, key=lambda u: [u['pkm'.index(c)] for c in PORD])

bf16 = jnp.bfloat16
f32 = jnp.float32
u32 = jnp.uint32
i32 = jnp.int32


def _iota(shape, dim):
    return lax.broadcasted_iota(i32, shape, dim)


def _nt(a, b):
    return lax.dot_general(a, b, (((1,), (1,)), ((), ())), preferred_element_type=f32)


def _nn(a, b):
    return lax.dot_general(a, b, (((1,), (0,)), ((), ())), preferred_element_type=f32)


def _unpack(u, idx):
    return pltpu.unpack_elementwise(u, index=idx, packed_dtype=bf16, unpacked_dtype=f32)


def _packi(a, b):
    return pltpu.pack_elementwise([a, b], packed_dtype=bf16)


def _b(u):
    return pltpu.bitcast(u, bf16)


def _u(b):
    return pltpu.bitcast(b, u32)


def _s2(start):
    return pl.ds(start, 8, stride=2)


VSTRIPS = [(pc, j) for j in range(NS) for pc in range(2)] + [(0, NS)]
NV = len(VSTRIPS)
PRE_UNITS = [(pr, k, m) for pr in range(2) for k in range(4) for m in range(3)]
LATE_UNITS = [(2 * i + 1, 2) for i in range(8)]
EARLY_UNITS = [(h, m) for h in range(16) for m in range(3) if (h, m) not in LATE_UNITS]


def _kernel(x_hbm, wqkv_hbm, wo_hbm, out_ref,
            wqkv_ref, wo_ref, at_ref, bt_ref, augx_ref, augq_ref, x2_ref, xs_ref, q2_ref, qs_ref, ow_ref,
            xbuf_ref, obuf_ref, sem):
    t = pl.program_id(0)
    sub8 = _iota((8, 128), 0)
    lane8 = _iota((8, 128), 1)
    pad_word = jnp.where(lane8 == L_PAD, jnp.uint32(ONE2), jnp.uint32(0))
    lo4 = sub8 < 4

    def _perm():
        pl_ = _iota((C, C), 0)
        pc_ = _iota((C, C), 1)
        return jnp.where(pc_ == jnp.where(pl_ < C // 2, 2 * pl_, 2 * (pl_ - C // 2) + 1), 1.0, 0.0).astype(bf16)

    def _setup_at():
        wq = wqkv_ref[:, 0:C]
        wk = wqkv_ref[:, C:2 * C]
        perm = _perm()
        at = (_nt(wk, wq) * (C ** -0.5 * math.log2(math.e))).astype(bf16)
        at_ref[...] = _u(_nn(perm, at).astype(bf16))

    def _setup_bt():
        wv = wqkv_ref[:, 2 * C:3 * C]
        perm = _perm()
        b = _nn(wv, wo_ref[...]).astype(bf16)
        bt = _nn(perm, b).T
        bt = jnp.concatenate([bt, jnp.zeros((C, 128 - C), f32)], axis=1)
        bt = jnp.concatenate([bt, jnp.zeros((112 - C, 128), f32)], axis=0)
        r = _iota((112, 128), 0)
        c = _iota((112, 128), 1)
        bt_ref[...] = _u(jnp.where((r == C) & (c == L_ONE), 1.0, bt).astype(bf16))

    def _setup_tables():
        rho = _iota((32, 128), 0)
        for m in range(3):
            ccol = (m * 128 + _iota((32, 128), 1)) // 2
            kcol = ((rho >= 14) & (rho < 29) & (rho - 14 == ccol % CM)) | (rho == 29)
            ccq = jnp.clip(ccol, 3, 188) % CM
            qcol = ((rho >= 14) & (rho < 29) & (((rho - 14 - ccq + 3 + CM) % CM) > 6)) | (rho == 30)

            def kaug(res):
                return rho == 30 if res is None else kcol | (rho == res)

            def qaug(res):
                return qcol | ((rho < 14) & (((rho - res + 3 + RM) % RM) > 6))

            def words(lo, hi, bits):
                return (jnp.where(lo, jnp.uint32(bits), jnp.uint32(0))
                        | jnp.where(hi, jnp.uint32(bits << 16), jnp.uint32(0)))
            kvar = [(2 * v + 1, (2 * v + 2) % RM) for v in range(7)] + [(None, 0), (191 % RM, None)]
            qvar = [(2 * v, 2 * v + 1) for v in range(7)] + [(3, 3), (188 % RM, 188 % RM)]
            for v in range(9):
                augx_ref[m, v] = words(kaug(kvar[v][0]), kaug(kvar[v][1]), ONE)
                augq_ref[m, v] = words(qaug(qvar[v][0]), qaug(qvar[v][1]), NBIG)
        pad_plane = jnp.where(_iota((XR, 128), 1) == L_PAD, jnp.uint32(ONE2), jnp.uint32(0))
        for pr in range(2):
            for sl in range(NR):
                for p in range(4):
                    x2_ref[sl, pr, p, 0:8] = pad_word
                    x2_ref[sl, pr, p, XR - 8:XR] = pad_word
                    if sl == 0 and p < 2:
                        x2_ref[sl, pr, p] = pad_plane
                        xs_ref[sl, pr, p] = pad_word
        xbuf_ref[0, 0:2] = jnp.zeros((2, C, W), bf16)

    colpatch_lane = (lane8 >= L_COL) & (lane8 < L_ONE)
    klabel = jnp.where(lane8 - L_COL == 7 + sub8, jnp.uint32(ONE2), jnp.uint32(0))
    qlabel = jnp.where(lane8 - L_COL < 8, jnp.uint32(NBIG * 0x10001), jnp.uint32(0))

    def key_words(xa, xb, aug, tile, pr, p, m, dup=None):
        slot = tile % NR
        w = jnp.concatenate([_packi(_unpack(xa, 0), _unpack(xb, 0)), _packi(_unpack(xa, 1), _unpack(xb, 1)), aug],
                            axis=0)
        wt = w.T
        for sl_, p_ in [(slot, p)] + ([dup] if dup else []):
            x2_ref[sl_, pr, p_, 8 + 128 * m:8 + 128 * (m + 1)] = wt
            if m == 2:
                xs_ref[sl_, pr, p_] = jnp.where(colpatch_lane, klabel, x2_ref[sl_, pr, p_, _s2(8 + 369)])

    def pre_unit(xsrc, r0, blk, tile, pr, k, m, dup=None, part=3):
        rows = [xsrc[r0 + 2 * il + pr, :, m * 128:(m + 1) * 128] for il in (2 * k - 1, 2 * k, 2 * k + 1)]
        ra = 8 * blk + 2 * k
        vx = jnp.where(ra < 1, 7, ((ra + RM - 1) % RM) // 2)
        vq = jnp.where(ra < 3, 7, jnp.where(ra >= 188, 8, (ra % RM) // 2))
        if part & 1:
            key_words(_u(rows[0]), _u(rows[1]), augx_ref[m, vx], tile + k // 2, pr, (k + 2) % 4, m, dup)
        if not part & 2:
            return
        at = _b(at_ref[...])
        qw = jnp.concatenate([_packi(_nn(at, rows[1]), _nn(at, rows[2])), augq_ref[m, vq]], axis=0)
        slot = tile % NR
        q2_ref[slot, pr, k, 128 * m:128 * (m + 1)] = qw.T
        if m == 2:
            qs_ref[slot, pr, k] = jnp.where(lo4, q2_ref[slot, pr, k, _s2(1)],
                                            jnp.where(colpatch_lane, qlabel, q2_ref[slot, pr, k, _s2(368)]))

    def keytile(tiles_pairs, pr, vi):
        pc, j = VSTRIPS[vi]
        vs = []
        for tile, p in tiles_pairs:
            if j == NS:
                vs += [x2_ref[tile % NR, pr, p, _s2(8)], xs_ref[tile % NR, pr, p]]
            else:
                vs += [x2_ref[tile % NR, pr, p, _s2(16 * j + pc)], x2_ref[tile % NR, pr, p, _s2(16 * j + 16 + pc)]]
        return _b(jnp.concatenate(vs, axis=0))

    def qrows(tiles_pairs, pr, vi):
        pc, j = VSTRIPS[vi]
        return [qs_ref[tile % NR, pr, k] if j == NS else q2_ref[tile % NR, pr, k, _s2(16 * j + pc)]
                for tile, k in tiles_pairs]

    def out_unit(dst, r0, h, m):
        pr = h % 2
        i = h // 2
        w = _b(jnp.concatenate([ow_ref[pr, i // 2, 8 * m + v, _s2(i % 2), :] for v in range(8)], axis=0))
        r = _nt(_b(bt_ref[...]), w)
        inv = 1.0 / r[C:C + 1]
        dst[(r0 + h) // 2, h % 2, :, m * 128:(m + 1) * 128] = (r[0:C] * inv).astype(bf16)

    def in_copy(p):
        return pltpu.make_async_copy(x_hbm.at[pl.ds(32 * p - 2, 34)], xbuf_ref.at[p % 2], sem.at[p % 2])

    def in_part(i):
        b, r0, nr = IN_PARTS[i]
        return pltpu.make_async_copy(x_hbm.at[pl.ds(32 * b - 2 + r0, nr)], xbuf_ref.at[b, pl.ds(r0, nr)],
                                     sem.at[5 + i])

    def w_copy(i):
        return pltpu.make_async_copy((wqkv_hbm, wo_hbm)[i], (wqkv_ref, wo_ref)[i], sem.at[14 + i])

    def out_copy(p, half):
        return pltpu.make_async_copy(obuf_ref.at[p % 3, pl.ds(8 * half, 8)], out_ref.at[pl.ds(16 * p + 8 * half, 8)],
                                     sem.at[(2, 16)[half] + p % 3])

    def out_part(h, m):
        return pltpu.make_async_copy(obuf_ref.at[(NP - 1) % 3, 8 + h // 2, h % 2, :, pl.ds(128 * m, 128)],
                                     out_ref.at[16 * (NP - 1) + 8 + h // 2, h % 2, :, pl.ds(128 * m, 128)],
                                     sem.at[5 + m])

    def colidx(n):
        r = _iota((n, 128), 0)
        return 4 * ((r // 8) % 2) + (r % 8) // 2

    def store_pair(res, key0, key1, keysp, j, col):
        o0 = res.pop(key0)
        o1 = res.pop(key1)
        if j == 0:
            o1 = jnp.where(col < 3, res[keysp], o1)
        if j == NS - 1:
            o0 = jnp.where(col >= 5, res.pop(keysp), o0)
        return _packi(o0, o1)

    def attn_stage(base, blk0, nsub, with_pre, xsrc, o_prev, o_cur, o_prev_r0, o_cur_r0, top, calls=(), bot=False):
        nt = 2 * NV
        poff_, pend_, nfill_, fpos_, fstep_, ps_, le_, e_, d_ = FIRST if top else LAST if bot else MAIN
        gtiles = []
        for d in range(nsub):
            if bot and d == nsub - 1:
                if LEAD:
                    seq = [NV - 1] + list(range(NV - 1))
                    for n in range(NV + LEAD):
                        gtiles += [(d, 1, seq[n])] if n < NV else []
                        gtiles += [(d, 0, seq[n - LEAD])] if n >= LEAD else []
                else:
                    for m in range(3):
                        for pr in (1, 0):
                            gtiles += [(d, pr, vi)
                                       for vi in ([NV - 1] if m == 0 else []) + list(range(16 * m, 16 * m + 16))]
            else:
                gtiles += [(d, pr, vi) for pr in range(2) for vi in [NV - 1] + list(range(NV - 1))]
        ntot = len(gtiles)
        col = colidx(64)
        sl = _iota((32, 128), 0)
        ln = _iota((32, 128), 1)
        mnew = (2 * (ln // 32) + ln % 2) <= (2 + 2 * (sl // 16) + sl % 2)
        odd16 = _iota((16, 128), 0) % 2 == 1
        svals = {}
        pvals = {}
        res = {}

        def tile_a(d, pr, vi):
            g = base + d
            return keytile([(g + 1, 0), (g, 1), (g, 2), (g, 3)], pr, vi)

        def tile_b(d, pr, vi):
            return keytile([(base + d + 1, p) for p in range(4)], pr, vi)

        def border(d):
            return 'top' if top and d == 0 else 'bot' if bot and d == nsub - 1 else None

        def pairs(d, pr):
            bd = border(d)
            pa, pb = [0, 1, 2], [1, 2, 3]
            if (bd, pr) == ('top', 1) and SKT:
                pa = [1, 2]
            if (bd, pr) == ('bot', 0) and SKB:
                pb = [1, 2]
            return pa, pb, (bd, pr) == ('top', 0), (bd, pr) == ('bot', 1)

        def qka(d, pr, vi):
            pa, _, xa, _ = pairs(d, pr)
            ql = qrows([(base + d, k) for k in pa], pr, vi)
            if xa:
                ql = ql + qrows([(base + d, 0), (base + d, 1)], 1, vi)
            svals[(d, pr, vi)] = _nt(_b(jnp.concatenate(ql, axis=0)), tile_a(d, pr, vi))

        def qkb(d, pr, vi):
            pa, pb, xa, xb = pairs(d, pr)
            ql = qrows([(base + d, k) for k in pb], pr, vi)
            if xb:
                ql = ql + qrows([(base + d, 2), (base + d, 3)], 0, vi)
            sb = _nt(_b(jnp.concatenate(ql, axis=0)), tile_b(d, pr, vi))
            sa = svals.pop((d, pr, vi))
            na = 16 * (len(pa) - 2)
            parts = [sa[0:na]] if na else []
            parts += [jnp.maximum(sa[na:na + 32], sb[0:32])]
            parts += [sb[32:]] if sb.shape[0] > 32 else []
            parts += [sa[48:80]] if xa else []
            comb = jnp.concatenate(parts, axis=0)
            m = jnp.max(comb, axis=1, keepdims=True)
            e = jnp.exp2(comb - m)
            nb = na + 32 + sb.shape[0] - 32
            mid = e[na:na + 32]
            pn = jnp.concatenate([jnp.where(mnew, mid, 0.0)] + ([e[na + 32:nb]] if sb.shape[0] > 32 else []), axis=0)
            po = jnp.concatenate(([e[0:na]] if na else []) + [jnp.where(mnew, 0.0, mid)]
                                 + ([e[nb:]] if xa else []), axis=0)
            pvals[(d, pr, vi)] = (pn.astype(bf16), po.astype(bf16))

        def pva(d, pr, vi):
            res[(pr, vi, 'a')] = _nn(pvals[(d, pr, vi)][1], tile_a(d, pr, vi))

        def pvb(d, pr, vi):
            pa, pb, xa, xb = pairs(d, pr)
            pn, po = pvals.pop((d, pr, vi))
            o = _nn(pn, tile_b(d, pr, vi))
            oa = res.pop((pr, vi, 'a'))
            na = 16 * (len(pa) - 2)
            res[(pr, vi)] = jnp.concatenate(([oa[0:na]] if na else []) + [oa[na:na + 32] + o[0:32]]
                                            + ([o[32:48]] if len(pb) == 3 else []), axis=0)
            if xa or xb:
                res[(pr, vi, 'x')] = oa[48:80] if xa else o[48:80]
            if vi < 2 * NS and vi % 2 == 1:
                j = vi // 2
                w = store_pair(res, (pr, vi - 1), (pr, vi), (pr, NV - 1), j, col[0:16 * (len(pa) + len(pb) - 2)])
                if (border(d), pr) == ('top', 1):
                    w = w[16 * (len(pa) - 2):]
                    ow_ref[pr, 1, j] = jnp.where(odd16, w[0:16], ow_ref[pr, 1, j])
                    ow_ref[pr, 2:4, j] = w[16:48].reshape(2, 16, 128)
                elif (border(d), pr) == ('bot', 0):
                    ow_ref[pr, 0:2, j] = w[0:32].reshape(2, 16, 128)
                    ow_ref[pr, 2, j] = jnp.where(odd16, ow_ref[pr, 2, j], w[32:48])
                else:
                    ow_ref[pr, :, j] = w.reshape(4, 16, 128)
                if xa or xb:
                    wx = store_pair(res, (pr, vi - 1, 'x'), (pr, vi, 'x'), (pr, NV - 1, 'x'), j, col[0:32])
                    p0 = 0 if xa else 2
                    ow_ref[1 - pr, p0:p0 + 2, j] = wx.reshape(2, 16, 128)

        extra = {}
        mark = {}
        done = {}
        for n, (d, pr, vi) in enumerate(gtiles):
            if vi < 2 * NS:
                done[d, pr, vi // 16] = n + d_
        for d in range(nsub):
            off = d * nt
            dst_late = (o_prev, o_prev_r0) if d == 0 else (o_cur, o_cur_r0 + 16 * (d - 1))
            dst = (o_cur, o_cur_r0 + 16 * d)
            for n, (h, m) in enumerate([] if top and d == 0 else LATE_UNITS):
                pos_ = ((LOFL if bot else LOFF) + LSTEP * n if d == 0
                        else off + d_ + (LEL if bot else le_) + 2 * n)
                extra.setdefault(pos_, []).append(('o', dst_late, h, m))
                mark['late', d] = max(mark.get(('late', d), 0), pos_)
            for h, m in (EARLY_UNITS + LATE_UNITS if border(d) == 'bot' else EARLY_UNITS):
                pr, i = h % 2, h // 2
                if border(d) == 'bot' and i >= 5:
                    pr = 1
                pos_ = done[d, pr, m] + e_ + ((SPM * i) // 2 if not (top or bot) else 2 * i)
                if bot:
                    pos_ = done[d, pr, m] + EL + SPL * i
                if with_pre and d == nsub - 1 and pr == 1 and m == 1 and i >= 8 - nfill_:
                    pos_ = ntot + d_ + fpos_ + (fstep_ * (i - 8 + nfill_)) // 2
                if border(d) == 'bot':
                    pos_ = done[d, pr, m] + EB + (SB * i) // 2
                if border(d) == 'bot' and m == 2 and pr == 0:
                    pos_ = done[d, pr, m] + LEND + (LST * i) // 2
                extra.setdefault(pos_, []).append(('o', dst, h, m))
                mark['unit', d, h, m] = pos_
            if with_pre:
                span = nt + (pend_ if d == nsub - 1 else 0) - (poff_ if d == 0 else 0)
                start = off + (poff_ if d == 0 else 0)
                for n, un in enumerate(KPRE_UNITS if top else MAIN_UNITS):
                    pos_ = start + (n * span) // len(PRE_UNITS)
                    if top and (d, n) in ((0, 12), (1, 0)):
                        if ONEB:
                            if d == 0:
                                extra.setdefault(pos_, []).append(('c', lambda: in_part(7).wait()))
                                extra[pos_].append(('c', lambda: in_part(8).wait()))
                                extra[pos_].append(('c', lambda: in_copy(2).start()))
                        else:
                            extra.setdefault(pos_, []).append(('c', lambda i=7 + d: in_part(i).wait()))
                            if d == 1:
                                extra[pos_].append(('c', lambda: in_copy(2).start()))
                    if ps_ == 99:
                        extra.setdefault(pos_, []).append(('p', d) + un + (None, 3))
                    else:
                        extra.setdefault(pos_ + max(ps_, 0), []).append(('p', d) + un + (None, 2))
                        extra.setdefault(pos_ + max(-ps_, 0), []).append(('p', d) + un + (None, 1))
        mark['end'] = max(extra)
        for pos_, fn in calls:
            pos_ = min(mark[pos_] + DLY, mark['end']) if pos_ in mark else pos_
            extra.setdefault(pos_, []).append(('c', fn))
        nslot = max([ntot + d_ + 2] + [k + 1 for k in extra])
        for n in range(nslot):
            for op, lag in OPS:
                k = n - lag - (d_ if op in 'AB' else 0)
                if 0 <= k < ntot:
                    {'a': qka, 'b': qkb, 'A': pva, 'B': pvb}[op](*gtiles[k])
            for e in extra.get(n, []):
                if e[0] == 'o':
                    out_unit(e[1][0], e[1][1], e[2], e[3])
                elif e[0] == 'c':
                    e[1]()
                else:
                    d = e[1]
                    pre_unit(xsrc, 2 + 16 * d, blk0 + 2 + d, base + 2 + d, *e[2:])

    def main_block(par):
        attn_stage(2 * par + 2, 2 * t - 2, 2, True, xbuf_ref.at[par], obuf_ref.at[(t + 1) % 3],
                   obuf_ref.at[(t + 2) % 3], 16, 0, False)

    def first_block():
        in_part(6).wait()
        attn_stage(0, 0, 2, True, xbuf_ref.at[1], None, obuf_ref.at[0], 0, 0, True)

    def last_block():
        last = obuf_ref.at[(NP - 1) % 3]
        prev = obuf_ref.at[(NP - 2) % 3]

        def tail_keys(pr, m):
            xa = _u(xbuf_ref[(NP - 1) % 2, 32 + pr, :, m * 128:(m + 1) * 128])
            key_words(xa, jnp.zeros_like(xa), augx_ref[m, 8], NB, pr, 2, m)

        def tail_fill():
            x2_ref[NB % NR, 0, 3] = jnp.where(_iota((XR, 128), 1) == L_PAD, jnp.uint32(ONE2), jnp.uint32(0))
            xs_ref[NB % NR, 0, 3] = pad_word
            x2_ref[NB % NR, 1, 3] = x2_ref[(NB - 1) % NR, 1, 3]
            xs_ref[NB % NR, 1, 3] = xs_ref[(NB - 1) % NR, 1, 3]

        calls = [(TPOS + 6 * n, lambda pr=n // 3, m=n % 3: tail_keys(pr, m)) for n in range(6)]
        calls += [(TPOS + 36, tail_fill),
                  (('late', 0), lambda: out_copy(NP - 2, 1).start()),
                  (('late', 1), lambda: out_copy(NP - 1, 0).start()),
                  ]
        calls += [(('unit', 1, h, m), lambda h=h, m=m: out_part(h, m).start()) for m in range(3) for h in range(16)]
        attn_stage(NB - 2, NB - 2, 2, False, None, prev, last, 16, 0, False, calls, True)
        for p, half in ((NP - 3, 0), (NP - 3, 1), (NP - 2, 0), (NP - 2, 1), (NP - 1, 0)):
            out_copy(p, half).wait()
        for m in range(3):
            for h in range(16):
                out_part(h, m).wait()

    @pl.when(t == 0)
    def _():
        if WORD:
            in_part(0).start()
        w_copy(0).start()
        w_copy(1).start()
        for i in range(WORD, 6 if S1POS else 9):
            in_part(i).start()
        _setup_tables()
        w_copy(0).wait()
        w_copy(1).wait()
        if not WSEP:
            in_part(0).wait()
        _setup_at()
        _setup_bt()
        for k in range(4):
            if (k > 0 or WSEP) and k in CHUNKS:
                for i in range(k, min([c for c in CHUNKS if c > k] + [4])):
                    in_part(i).wait()
            if k == S1POS > 0:
                for i in range(6, 9):
                    in_part(i).start()
            for pr in range(2):
                for m in range(3):
                    pre_unit(xbuf_ref.at[0], 2, 0, 0, pr, k, m, (0, 1) if (pr, k) == (0, 3) else None)
        for k in range(4):
            if k % 2 == 0:
                in_part(4 + k // 2).wait()
            for pr in range(2):
                for m in range(3):
                    pre_unit(xbuf_ref.at[0], 18, 1, 1, pr, k, m)

    @pl.when(t >= 1)
    def _():
        @pl.when((t >= 2) & (t < NP))
        def _():
            in_copy(t).wait()

        @pl.when((t >= 2) & (t < NP - 1))
        def _():
            in_copy(t + 1).start()

        @pl.when(t >= 4)
        def _():
            out_copy(t - 4, 0).wait()
            out_copy(t - 4, 1).wait()

    @pl.when(t == 1)
    def _():
        first_block()

    for par in range(2):
        @pl.when((t >= 2) & (t < NP) & (t % 2 == par))
        def _():
            main_block(par)

    @pl.when((t >= 2) & (t < NP))
    def _():
        out_copy(t - 2, 1).start()

    @pl.when((t >= 1) & (t < NP))
    def _():
        out_copy(t - 1, 0).start()

    @pl.when(t == NP)
    def _():
        last_block()


@jax.jit
def pallas_standalone__neighborhood_nat__vision_kernel(x, wqkv, wo):
    xt = jnp.transpose(x.reshape(H, W, C), (0, 2, 1))
    out = pl.pallas_call(
        _kernel,
        grid=(NP + 1,),
        in_specs=[
            pl.BlockSpec(memory_space=pl.ANY),
            pl.BlockSpec(memory_space=pl.ANY),
            pl.BlockSpec(memory_space=pl.ANY),
        ],
        out_specs=pl.BlockSpec(memory_space=pl.ANY),
        out_shape=jax.ShapeDtypeStruct((H // 2, 2, C, W), bf16),
        scratch_shapes=[
            pltpu.VMEM((C, 3 * C), bf16),
            pltpu.VMEM((C, C), bf16),
            pltpu.VMEM((48, 96), u32),
            pltpu.VMEM((56, 128), u32),
            pltpu.VMEM((3, 9, 32, 128), u32),
            pltpu.VMEM((3, 9, 32, 128), u32),
            pltpu.VMEM((NR, 2, 4, XR, 128), u32),
            pltpu.VMEM((NR, 2, 4, 8, 128), u32),
            pltpu.VMEM((NR, 2, 4, W, 128), u32),
            pltpu.VMEM((NR, 2, 4, 8, 128), u32),
            pltpu.VMEM((2, 4, NS, 16, 128), u32),
            pltpu.VMEM((2, 34, C, W), bf16),
            pltpu.VMEM((3, 16, 2, C, W), bf16),
            pltpu.SemaphoreType.DMA((19,)),
        ],
        compiler_params=pltpu.CompilerParams(
            dimension_semantics=("arbitrary",), vmem_limit_bytes=64 * 1024 * 1024,
            disable_bounds_checks=True),
        name="nat_kernel",
    )(xt, wqkv, wo)
    return jnp.transpose(out.reshape(H, C, W), (0, 2, 1)).reshape(1, H, W, C)
```

```python
import math

import jax
import jax.numpy as jnp
from jax import lax
from jax.experimental import pallas as pl
from jax.experimental.pallas import tpu as pltpu

H = 384
W = 384
C = 96
NP = 12
NB = 24
NS = 24
NR = 4
XR = W + 16
ONE = 0x3F80
ONE2 = 0x3F803F80
NBIG = 0xF180
RM = 14
CM = 15
L_COL = 110
L_ONE = 125
L_PAD = 126

MAIN = dict(la=13, lag=7, p0=14, p1=-7, split=-5, nfill=5, fpos=-7, fstep=1, late=4, late0=1)
FIRST = dict(la=12, lag=8, p0=10, p1=-12, split=None, nfill=5, fpos=-8, fstep=0, late=4, late0=0)
LAST = dict(la=12, lag=8, late=4, late0=0, lag_b=8, lag_end=3, dma_lag=4, tail=40)

IN_PARTS = [(0, 2, 4), (0, 6, 4), (0, 10, 4), (0, 14, 4), (0, 18, 8), (0, 26, 8), (1, 0, 10), (1, 10, 8), (1, 18, 16)]
PRE_UNITS = [(pr, k, m) for k in range(4) for pr in range(2) for m in range(3)]

bf16 = jnp.bfloat16
f32 = jnp.float32
u32 = jnp.uint32
i32 = jnp.int32


def _iota(shape, dim):
    return lax.broadcasted_iota(i32, shape, dim)


def _nt(a, b):
    return lax.dot_general(a, b, (((1,), (1,)), ((), ())), preferred_element_type=f32)


def _nn(a, b):
    return lax.dot_general(a, b, (((1,), (0,)), ((), ())), preferred_element_type=f32)


def _unpack(u, idx):
    return pltpu.unpack_elementwise(u, index=idx, packed_dtype=bf16, unpacked_dtype=f32)


def _packi(a, b):
    return pltpu.pack_elementwise([a, b], packed_dtype=bf16)


def _b(u):
    return pltpu.bitcast(u, bf16)


def _u(b):
    return pltpu.bitcast(b, u32)


def _s2(start):
    return pl.ds(start, 8, stride=2)


VSTRIPS = [(pc, j) for j in range(NS) for pc in range(2)] + [(0, NS)]
NV = len(VSTRIPS)
LATE_UNITS = [(2 * i + 1, 2) for i in range(8)]
EARLY_UNITS = [(h, m) for h in range(16) for m in range(3) if (h, m) not in LATE_UNITS]


def _kernel(x_hbm, wqkv_hbm, wo_hbm, out_ref,
            wqkv_ref, wo_ref, at_ref, bt_ref, augx_ref, augq_ref, x2_ref, xs_ref, q2_ref, qs_ref, ow_ref,
            xbuf_ref, obuf_ref, sem):
    t = pl.program_id(0)
    sub8 = _iota((8, 128), 0)
    lane8 = _iota((8, 128), 1)
    pad_word = jnp.where(lane8 == L_PAD, jnp.uint32(ONE2), jnp.uint32(0))
    lo4 = sub8 < 4

    def _perm():
        pl_ = _iota((C, C), 0)
        pc_ = _iota((C, C), 1)
        return jnp.where(pc_ == jnp.where(pl_ < C // 2, 2 * pl_, 2 * (pl_ - C // 2) + 1), 1.0, 0.0).astype(bf16)

    def _setup_at():
        wq = wqkv_ref[:, 0:C]
        wk = wqkv_ref[:, C:2 * C]
        perm = _perm()
        at = (_nt(wk, wq) * (C ** -0.5 * math.log2(math.e))).astype(bf16)
        at_ref[...] = _u(_nn(perm, at).astype(bf16))

    def _setup_bt():
        wv = wqkv_ref[:, 2 * C:3 * C]
        perm = _perm()
        b = _nn(wv, wo_ref[...]).astype(bf16)
        bt = _nn(perm, b).T
        bt = jnp.concatenate([bt, jnp.zeros((C, 128 - C), f32)], axis=1)
        bt = jnp.concatenate([bt, jnp.zeros((112 - C, 128), f32)], axis=0)
        r = _iota((112, 128), 0)
        c = _iota((112, 128), 1)
        bt_ref[...] = _u(jnp.where((r == C) & (c == L_ONE), 1.0, bt).astype(bf16))

    def _setup_tables():
        rho = _iota((32, 128), 0)
        for m in range(3):
            ccol = (m * 128 + _iota((32, 128), 1)) // 2
            kcol = ((rho >= 14) & (rho < 29) & (rho - 14 == ccol % CM)) | (rho == 29)
            ccq = jnp.clip(ccol, 3, 188) % CM
            qcol = ((rho >= 14) & (rho < 29) & (((rho - 14 - ccq + 3 + CM) % CM) > 6)) | (rho == 30)

            def kaug(res):
                return rho == 30 if res is None else kcol | (rho == res)

            def qaug(res):
                return qcol | ((rho < 14) & (((rho - res + 3 + RM) % RM) > 6))

            def words(lo, hi, bits):
                return (jnp.where(lo, jnp.uint32(bits), jnp.uint32(0))
                        | jnp.where(hi, jnp.uint32(bits << 16), jnp.uint32(0)))
            kvar = [(2 * v + 1, (2 * v + 2) % RM) for v in range(7)] + [(None, 0), (191 % RM, None)]
            qvar = [(2 * v, 2 * v + 1) for v in range(7)] + [(3, 3), (188 % RM, 188 % RM)]
            for v in range(9):
                augx_ref[m, v] = words(kaug(kvar[v][0]), kaug(kvar[v][1]), ONE)
                augq_ref[m, v] = words(qaug(qvar[v][0]), qaug(qvar[v][1]), NBIG)
        pad_plane = jnp.where(_iota((XR, 128), 1) == L_PAD, jnp.uint32(ONE2), jnp.uint32(0))
        for pr in range(2):
            for sl in range(NR):
                for p in range(4):
                    x2_ref[sl, pr, p, 0:8] = pad_word
                    x2_ref[sl, pr, p, XR - 8:XR] = pad_word
                    if sl == 0 and p < 2:
                        x2_ref[sl, pr, p] = pad_plane
                        xs_ref[sl, pr, p] = pad_word
        xbuf_ref[0, 0:2] = jnp.zeros((2, C, W), bf16)

    colpatch_lane = (lane8 >= L_COL) & (lane8 < L_ONE)
    klabel = jnp.where(lane8 - L_COL == 7 + sub8, jnp.uint32(ONE2), jnp.uint32(0))
    qlabel = jnp.where(lane8 - L_COL < 8, jnp.uint32(NBIG * 0x10001), jnp.uint32(0))

    def key_words(xa, xb, aug, tile, pr, p, m, dup=None):
        slot = tile % NR
        w = jnp.concatenate([_packi(_unpack(xa, 0), _unpack(xb, 0)), _packi(_unpack(xa, 1), _unpack(xb, 1)), aug],
                            axis=0)
        wt = w.T
        for sl_, p_ in [(slot, p)] + ([dup] if dup else []):
            x2_ref[sl_, pr, p_, 8 + 128 * m:8 + 128 * (m + 1)] = wt
            if m == 2:
                xs_ref[sl_, pr, p_] = jnp.where(colpatch_lane, klabel, x2_ref[sl_, pr, p_, _s2(8 + 369)])

    def pre_unit(xsrc, r0, blk, tile, pr, k, m, dup=None, part=3):
        rows = [xsrc[r0 + 2 * il + pr, :, m * 128:(m + 1) * 128] for il in (2 * k - 1, 2 * k, 2 * k + 1)]
        ra = 8 * blk + 2 * k
        vx = jnp.where(ra < 1, 7, ((ra + RM - 1) % RM) // 2)
        vq = jnp.where(ra < 3, 7, jnp.where(ra >= 188, 8, (ra % RM) // 2))
        if part & 1:
            key_words(_u(rows[0]), _u(rows[1]), augx_ref[m, vx], tile + k // 2, pr, (k + 2) % 4, m, dup)
        if not part & 2:
            return
        at = _b(at_ref[...])
        qw = jnp.concatenate([_packi(_nn(at, rows[1]), _nn(at, rows[2])), augq_ref[m, vq]], axis=0)
        slot = tile % NR
        q2_ref[slot, pr, k, 128 * m:128 * (m + 1)] = qw.T
        if m == 2:
            qs_ref[slot, pr, k] = jnp.where(lo4, q2_ref[slot, pr, k, _s2(1)],
                                            jnp.where(colpatch_lane, qlabel, q2_ref[slot, pr, k, _s2(368)]))

    def keytile(tiles_pairs, pr, vi):
        pc, j = VSTRIPS[vi]
        vs = []
        for tile, p in tiles_pairs:
            if j == NS:
                vs += [x2_ref[tile % NR, pr, p, _s2(8)], xs_ref[tile % NR, pr, p]]
            else:
                vs += [x2_ref[tile % NR, pr, p, _s2(16 * j + pc)], x2_ref[tile % NR, pr, p, _s2(16 * j + 16 + pc)]]
        return _b(jnp.concatenate(vs, axis=0))

    def qrows(tiles_pairs, pr, vi):
        pc, j = VSTRIPS[vi]
        return [qs_ref[tile % NR, pr, k] if j == NS else q2_ref[tile % NR, pr, k, _s2(16 * j + pc)]
                for tile, k in tiles_pairs]

    def out_unit(dst, r0, h, m):
        pr = h % 2
        i = h // 2
        w = _b(jnp.concatenate([ow_ref[pr, i // 2, 8 * m + v, _s2(i % 2), :] for v in range(8)], axis=0))
        r = _nt(_b(bt_ref[...]), w)
        inv = 1.0 / r[C:C + 1]
        dst[(r0 + h) // 2, h % 2, :, m * 128:(m + 1) * 128] = (r[0:C] * inv).astype(bf16)

    def in_copy(p):
        return pltpu.make_async_copy(x_hbm.at[pl.ds(32 * p - 2, 34)], xbuf_ref.at[p % 2], sem.at[p % 2])

    def in_part(i):
        b, r0, nr = IN_PARTS[i]
        return pltpu.make_async_copy(x_hbm.at[pl.ds(32 * b - 2 + r0, nr)], xbuf_ref.at[b, pl.ds(r0, nr)],
                                     sem.at[5 + i])

    def w_copy(i):
        return pltpu.make_async_copy((wqkv_hbm, wo_hbm)[i], (wqkv_ref, wo_ref)[i], sem.at[14 + i])

    def out_copy(p, half):
        return pltpu.make_async_copy(obuf_ref.at[p % 3, pl.ds(8 * half, 8)], out_ref.at[pl.ds(16 * p + 8 * half, 8)],
                                     sem.at[(2, 16)[half] + p % 3])

    def out_part(h, m):
        return pltpu.make_async_copy(obuf_ref.at[(NP - 1) % 3, 8 + h // 2, h % 2, :, pl.ds(128 * m, 128)],
                                     out_ref.at[16 * (NP - 1) + 8 + h // 2, h % 2, :, pl.ds(128 * m, 128)],
                                     sem.at[5 + m])

    def colidx(n):
        r = _iota((n, 128), 0)
        return 4 * ((r // 8) % 2) + (r % 8) // 2

    def store_pair(res, key0, key1, keysp, j, col):
        o0 = res.pop(key0)
        o1 = res.pop(key1)
        if j == 0:
            o1 = jnp.where(col < 3, res[keysp], o1)
        if j == NS - 1:
            o0 = jnp.where(col >= 5, res.pop(keysp), o0)
        return _packi(o0, o1)

    def attn_stage(base, blk0, nsub, with_pre, xsrc, o_prev, o_cur, o_prev_r0, o_cur_r0, top, calls=(), bot=False):
        nt = 2 * NV
        sch = FIRST if top else LAST if bot else MAIN
        la = sch['la']
        gtiles = []
        for d in range(nsub):
            if bot and d == nsub - 1:
                gtiles += [(d, pr, vi) for pr in (1, 0) for vi in [NV - 1] + list(range(NV - 1))]
            else:
                gtiles += [(d, pr, vi) for pr in range(2) for vi in [NV - 1] + list(range(NV - 1))]
        ntot = len(gtiles)
        col = colidx(64)
        sl = _iota((32, 128), 0)
        ln = _iota((32, 128), 1)
        mnew = (2 * (ln // 32) + ln % 2) <= (2 + 2 * (sl // 16) + sl % 2)
        odd16 = _iota((16, 128), 0) % 2 == 1
        svals = {}
        pvals = {}
        res = {}

        def tile_a(d, pr, vi):
            g = base + d
            return keytile([(g + 1, 0), (g, 1), (g, 2), (g, 3)], pr, vi)

        def tile_b(d, pr, vi):
            return keytile([(base + d + 1, p) for p in range(4)], pr, vi)

        def border(d):
            return 'top' if top and d == 0 else 'bot' if bot and d == nsub - 1 else None

        def pairs(d, pr):
            bd = border(d)
            pa, pb = [0, 1, 2], [1, 2, 3]
            if (bd, pr) == ('top', 1):
                pa = [1, 2]
            if (bd, pr) == ('bot', 0):
                pb = [1, 2]
            return pa, pb, (bd, pr) == ('top', 0), (bd, pr) == ('bot', 1)

        def qka(d, pr, vi):
            pa, _, xa, _ = pairs(d, pr)
            ql = qrows([(base + d, k) for k in pa], pr, vi)
            if xa:
                ql = ql + qrows([(base + d, 0), (base + d, 1)], 1, vi)
            svals[(d, pr, vi)] = _nt(_b(jnp.concatenate(ql, axis=0)), tile_a(d, pr, vi))

        def qkb(d, pr, vi):
            pa, pb, xa, xb = pairs(d, pr)
            ql = qrows([(base + d, k) for k in pb], pr, vi)
            if xb:
                ql = ql + qrows([(base + d, 2), (base + d, 3)], 0, vi)
            sb = _nt(_b(jnp.concatenate(ql, axis=0)), tile_b(d, pr, vi))
            sa = svals.pop((d, pr, vi))
            na = 16 * (len(pa) - 2)
            parts = [sa[0:na]] if na else []
            parts += [jnp.maximum(sa[na:na + 32], sb[0:32])]
            parts += [sb[32:]] if sb.shape[0] > 32 else []
            parts += [sa[48:80]] if xa else []
            comb = jnp.concatenate(parts, axis=0)
            m = jnp.max(comb, axis=1, keepdims=True)
            e = jnp.exp2(comb - m)
            nb = na + 32 + sb.shape[0] - 32
            mid = e[na:na + 32]
            pn = jnp.concatenate([jnp.where(mnew, mid, 0.0)] + ([e[na + 32:nb]] if sb.shape[0] > 32 else []), axis=0)
            po = jnp.concatenate(([e[0:na]] if na else []) + [jnp.where(mnew, 0.0, mid)]
                                 + ([e[nb:]] if xa else []), axis=0)
            pvals[(d, pr, vi)] = (pn.astype(bf16), po.astype(bf16))

        def pva(d, pr, vi):
            res[(pr, vi, 'a')] = _nn(pvals[(d, pr, vi)][1], tile_a(d, pr, vi))

        def pvb(d, pr, vi):
            pa, pb, xa, xb = pairs(d, pr)
            pn, po = pvals.pop((d, pr, vi))
            o = _nn(pn, tile_b(d, pr, vi))
            oa = res.pop((pr, vi, 'a'))
            na = 16 * (len(pa) - 2)
            res[(pr, vi)] = jnp.concatenate(([oa[0:na]] if na else []) + [oa[na:na + 32] + o[0:32]]
                                            + ([o[32:48]] if len(pb) == 3 else []), axis=0)
            if xa or xb:
                res[(pr, vi, 'x')] = oa[48:80] if xa else o[48:80]
            if vi < 2 * NS and vi % 2 == 1:
                j = vi // 2
                w = store_pair(res, (pr, vi - 1), (pr, vi), (pr, NV - 1), j, col[0:16 * (len(pa) + len(pb) - 2)])
                if (border(d), pr) == ('top', 1):
                    w = w[16 * (len(pa) - 2):]
                    ow_ref[pr, 1, j] = jnp.where(odd16, w[0:16], ow_ref[pr, 1, j])
                    ow_ref[pr, 2:4, j] = w[16:48].reshape(2, 16, 128)
                elif (border(d), pr) == ('bot', 0):
                    ow_ref[pr, 0:2, j] = w[0:32].reshape(2, 16, 128)
                    ow_ref[pr, 2, j] = jnp.where(odd16, ow_ref[pr, 2, j], w[32:48])
                else:
                    ow_ref[pr, :, j] = w.reshape(4, 16, 128)
                if xa or xb:
                    wx = store_pair(res, (pr, vi - 1, 'x'), (pr, vi, 'x'), (pr, NV - 1, 'x'), j, col[0:32])
                    p0 = 0 if xa else 2
                    ow_ref[1 - pr, p0:p0 + 2, j] = wx.reshape(2, 16, 128)

        extra = {}
        mark = {}
        done = {}
        for n, (d, pr, vi) in enumerate(gtiles):
            if vi < 2 * NS:
                done[d, pr, vi // 16] = n + la
        for d in range(nsub):
            off = d * nt
            dst_late = (o_prev, o_prev_r0) if d == 0 else (o_cur, o_cur_r0 + 16 * (d - 1))
            dst = (o_cur, o_cur_r0 + 16 * d)
            for n, (h, m) in enumerate([] if top and d == 0 else LATE_UNITS):
                pos_ = sch['late0'] + n if d == 0 else off + la + sch['late'] + 2 * n
                extra.setdefault(pos_, []).append(('o', dst_late, h, m))
                mark['late', d] = pos_
            for h, m in (EARLY_UNITS + LATE_UNITS if border(d) == 'bot' else EARLY_UNITS):
                pr, i = h % 2, h // 2
                if border(d) == 'bot':
                    pr = 1 if i >= 5 else pr
                    pos_ = done[d, pr, m] + (sch['lag_end'] if (pr, m) == (0, 2) else sch['lag_b'] + i)
                elif with_pre and d == nsub - 1 and pr == 1 and m == 1 and i >= 8 - sch['nfill']:
                    pos_ = ntot + la + sch['fpos'] + (sch['fstep'] * (i - 8 + sch['nfill'])) // 2
                else:
                    pos_ = done[d, pr, m] + sch['lag'] + 2 * i
                extra.setdefault(pos_, []).append(('o', dst, h, m))
                mark['unit', d, h, m] = pos_
            if with_pre:
                span = nt + (sch['p1'] if d == nsub - 1 else 0) - (sch['p0'] if d == 0 else 0)
                start = off + (sch['p0'] if d == 0 else 0)
                for n, un in enumerate(PRE_UNITS):
                    pos_ = start + (n * span) // len(PRE_UNITS)
                    if top and (d, n) == (0, 12):
                        extra.setdefault(pos_, []).append(('c', lambda: in_part(7).wait()))
                        extra[pos_].append(('c', lambda: in_part(8).wait()))
                        extra[pos_].append(('c', lambda: in_copy(2).start()))
                    if sch['split'] is None:
                        extra.setdefault(pos_, []).append(('p', d) + un + (None, 3))
                    else:
                        extra.setdefault(pos_ + max(sch['split'], 0), []).append(('p', d) + un + (None, 2))
                        extra.setdefault(pos_ + max(-sch['split'], 0), []).append(('p', d) + un + (None, 1))
        mark['end'] = max(extra)
        for pos_, fn in calls:
            pos_ = min(mark[pos_] + sch['dma_lag'], mark['end']) if pos_ in mark else pos_
            extra.setdefault(pos_, []).append(('c', fn))
        nslot = max([ntot + la + 2] + [k + 1 for k in extra])
        for n in range(nslot):
            for op, k in ((qka, n), (pva, n - la), (qkb, n), (pvb, n - la)):
                if 0 <= k < ntot:
                    op(*gtiles[k])
            for e in extra.get(n, []):
                if e[0] == 'o':
                    out_unit(e[1][0], e[1][1], e[2], e[3])
                elif e[0] == 'c':
                    e[1]()
                else:
                    d = e[1]
                    pre_unit(xsrc, 2 + 16 * d, blk0 + 2 + d, base + 2 + d, *e[2:])

    def main_block(par):
        attn_stage(2 * par + 2, 2 * t - 2, 2, True, xbuf_ref.at[par], obuf_ref.at[(t + 1) % 3],
                   obuf_ref.at[(t + 2) % 3], 16, 0, False)

    def first_block():
        in_part(6).wait()
        attn_stage(0, 0, 2, True, xbuf_ref.at[1], None, obuf_ref.at[0], 0, 0, True)

    def last_block():
        last = obuf_ref.at[(NP - 1) % 3]
        prev = obuf_ref.at[(NP - 2) % 3]

        def tail_keys(pr, m):
            xa = _u(xbuf_ref[(NP - 1) % 2, 32 + pr, :, m * 128:(m + 1) * 128])
            key_words(xa, jnp.zeros_like(xa), augx_ref[m, 8], NB, pr, 2, m)

        def tail_fill():
            x2_ref[NB % NR, 0, 3] = jnp.where(_iota((XR, 128), 1) == L_PAD, jnp.uint32(ONE2), jnp.uint32(0))
            xs_ref[NB % NR, 0, 3] = pad_word
            x2_ref[NB % NR, 1, 3] = x2_ref[(NB - 1) % NR, 1, 3]
            xs_ref[NB % NR, 1, 3] = xs_ref[(NB - 1) % NR, 1, 3]

        calls = [(LAST['tail'] + 6 * n, lambda pr=n // 3, m=n % 3: tail_keys(pr, m)) for n in range(6)]
        calls += [(LAST['tail'] + 36, tail_fill),
                  (('late', 0), lambda: out_copy(NP - 2, 1).start()),
                  (('late', 1), lambda: out_copy(NP - 1, 0).start()),
                  ]
        calls += [(('unit', 1, h, m), lambda h=h, m=m: out_part(h, m).start()) for m in range(3) for h in range(16)]
        attn_stage(NB - 2, NB - 2, 2, False, None, prev, last, 16, 0, False, calls, True)
        for p, half in ((NP - 3, 0), (NP - 3, 1), (NP - 2, 0), (NP - 2, 1), (NP - 1, 0)):
            out_copy(p, half).wait()
        for m in range(3):
            for h in range(16):
                out_part(h, m).wait()

    @pl.when(t == 0)
    def _():
        w_copy(0).start()
        w_copy(1).start()
        for i in range(6):
            in_part(i).start()
        _setup_tables()
        w_copy(0).wait()
        w_copy(1).wait()
        _setup_at()
        _setup_bt()
        for k in range(4):
            in_part(k).wait()
            if k == 1:
                for i in range(6, 9):
                    in_part(i).start()
            for pr in range(2):
                for m in range(3):
                    pre_unit(xbuf_ref.at[0], 2, 0, 0, pr, k, m, (0, 1) if (pr, k) == (0, 3) else None)
        for k in range(4):
            if k % 2 == 0:
                in_part(4 + k // 2).wait()
            for pr in range(2):
                for m in range(3):
                    pre_unit(xbuf_ref.at[0], 18, 1, 1, pr, k, m)

    @pl.when(t >= 1)
    def _():
        @pl.when((t >= 2) & (t < NP))
        def _():
            in_copy(t).wait()

        @pl.when((t >= 2) & (t < NP - 1))
        def _():
            in_copy(t + 1).start()

        @pl.when(t >= 4)
        def _():
            out_copy(t - 4, 0).wait()
            out_copy(t - 4, 1).wait()

    @pl.when(t == 1)
    def _():
        first_block()

    for par in range(2):
        @pl.when((t >= 2) & (t < NP) & (t % 2 == par))
        def _():
            main_block(par)

    @pl.when((t >= 2) & (t < NP))
    def _():
        out_copy(t - 2, 1).start()

    @pl.when((t >= 1) & (t < NP))
    def _():
        out_copy(t - 1, 0).start()

    @pl.when(t == NP)
    def _():
        last_block()


@jax.jit
def pallas_standalone__neighborhood_nat__vision_kernel(x, wqkv, wo):
    xt = jnp.transpose(x.reshape(H, W, C), (0, 2, 1))
    out = pl.pallas_call(
        _kernel,
        grid=(NP + 1,),
        in_specs=[
            pl.BlockSpec(memory_space=pl.ANY),
            pl.BlockSpec(memory_space=pl.ANY),
            pl.BlockSpec(memory_space=pl.ANY),
        ],
        out_specs=pl.BlockSpec(memory_space=pl.ANY),
        out_shape=jax.ShapeDtypeStruct((H // 2, 2, C, W), bf16),
        scratch_shapes=[
            pltpu.VMEM((C, 3 * C), bf16),
            pltpu.VMEM((C, C), bf16),
            pltpu.VMEM((48, 96), u32),
            pltpu.VMEM((56, 128), u32),
            pltpu.VMEM((3, 9, 32, 128), u32),
            pltpu.VMEM((3, 9, 32, 128), u32),
            pltpu.VMEM((NR, 2, 4, XR, 128), u32),
            pltpu.VMEM((NR, 2, 4, 8, 128), u32),
            pltpu.VMEM((NR, 2, 4, W, 128), u32),
            pltpu.VMEM((NR, 2, 4, 8, 128), u32),
            pltpu.VMEM((2, 4, NS, 16, 128), u32),
            pltpu.VMEM((2, 34, C, W), bf16),
            pltpu.VMEM((3, 16, 2, C, W), bf16),
            pltpu.SemaphoreType.DMA((19,)),
        ],
        compiler_params=pltpu.CompilerParams(
            dimension_semantics=("arbitrary",), vmem_limit_bytes=64 * 1024 * 1024,
            disable_bounds_checks=True),
        name="nat_kernel",
    )(xt, wqkv, wo)
    return jnp.transpose(out.reshape(H, C, W), (0, 2, 1)).reshape(1, H, W, C)
```

```python
import math

import jax
import jax.numpy as jnp
from jax import lax
from jax.experimental import pallas as pl
from jax.experimental.pallas import tpu as pltpu

H = 384
W = 384
C = 96
NP = 12
NB = 24
NS = 24
NR = 4
XR = W + 16
ONE = 0x3F80
ONE2 = 0x3F803F80
NBIG = 0xF180
RM = 14
CM = 15
L_COL = 110
L_ONE = 125
L_PAD = 126
L_ONE2 = 127

MAIN = dict(la=12, lag=7, p0=8, p1=-7, split=-4, nfill=5, fpos=-7, fstep=1, late=8, late0=1)
FIRST = dict(la=13, lag=8, p0=12, p1=-12, split=None, nfill=4, fpos=-4, fstep=2, late=8, late0=0)
LAST = dict(la=13, lag=7, late=10, late0=1, lag_b=5, lag_end=2, dma_lag=4, tail=30)


IN_PARTS = [(0, 2, 4), (0, 6, 4), (0, 10, 4), (0, 14, 4), (0, 18, 8), (0, 26, 8), (1, 0, 10), (1, 10, 8), (1, 18, 16)]
PRE_UNITS = [(pr, k, m) for k in range(4) for pr in range(2) for m in range(3)]

bf16 = jnp.bfloat16
f32 = jnp.float32
u32 = jnp.uint32
i32 = jnp.int32


def _iota(shape, dim):
    return lax.broadcasted_iota(i32, shape, dim)


def _nt(a, b):
    return lax.dot_general(a, b, (((1,), (1,)), ((), ())), preferred_element_type=f32)


def _nn(a, b):
    return lax.dot_general(a, b, (((1,), (0,)), ((), ())), preferred_element_type=f32)


def _unpack(u, idx):
    return pltpu.unpack_elementwise(u, index=idx, packed_dtype=bf16, unpacked_dtype=f32)


def _packi(a, b):
    return pltpu.pack_elementwise([a, b], packed_dtype=bf16)


def _b(u):
    return pltpu.bitcast(u, bf16)


def _u(b):
    return pltpu.bitcast(b, u32)


def _s2(start):
    return pl.ds(start, 8, stride=2)


VSTRIPS = [(pc, j) for j in range(NS) for pc in range(2)] + [(0, NS)]
NV = len(VSTRIPS)
LATE_UNITS = [(2 * i + 1, 2) for i in range(8)]
EARLY_UNITS = [(h, m) for h in range(16) for m in range(3) if (h, m) not in LATE_UNITS]


def _kernel(x_hbm, wqkv_hbm, wo_hbm, out_ref,
            wqkv_ref, wo_ref, at_ref, bt_ref, augx_ref, augq_ref, x2_ref, xs_ref, q2_ref, qs_ref, ow_ref,
            xbuf_ref, obuf_ref, sem):
    t = pl.program_id(0)
    sub8 = _iota((8, 128), 0)
    lane8 = _iota((8, 128), 1)
    pad_word = jnp.where(lane8 == L_PAD, jnp.uint32(ONE2), jnp.uint32(0))
    lo4 = sub8 < 4

    def _perm():
        pl_ = _iota((C, C), 0)
        pc_ = _iota((C, C), 1)
        return jnp.where(pc_ == jnp.where(pl_ < C // 2, 2 * pl_, 2 * (pl_ - C // 2) + 1), 1.0, 0.0).astype(bf16)

    def _setup_at():
        wq = wqkv_ref[:, 0:C]
        wk = wqkv_ref[:, C:2 * C]
        perm = _perm()
        at = (_nt(wk, wq) * (C ** -0.5 * math.log2(math.e))).astype(bf16)
        at_ref[...] = _u(_nn(perm, at).astype(bf16))

    def _setup_bt():
        wv = wqkv_ref[:, 2 * C:3 * C]
        perm = _perm()
        b = _nn(wv, wo_ref[...]).astype(bf16)
        bt = _nn(perm, b).T
        bt = jnp.concatenate([bt, jnp.zeros((C, 128 - C), f32)], axis=1)
        bt = jnp.concatenate([bt, jnp.zeros((112 - C, 128), f32)], axis=0)
        r = _iota((112, 128), 0)
        c = _iota((112, 128), 1)
        sel = ((r == C) & (c == L_ONE)) | ((r == C + 1) & (c == L_ONE2))
        bt_ref[...] = _u(jnp.where(sel, 1.0, bt).astype(bf16))

    def _setup_tables():
        rho = _iota((32, 128), 0)
        for m in range(3):
            ccol = (m * 128 + _iota((32, 128), 1)) // 2
            kcol = ((rho >= 14) & (rho < 29) & (rho - 14 == ccol % CM)) | (rho == 29) | (rho == 31)
            ccq = jnp.clip(ccol, 3, 188) % CM
            qcol = ((rho >= 14) & (rho < 29) & (((rho - 14 - ccq + 3 + CM) % CM) > 6)) | (rho == 30)

            def kaug(res):
                return rho == 30 if res is None else kcol | (rho == res)

            def qaug(res):
                return qcol | ((rho < 14) & (((rho - res + 3 + RM) % RM) > 6))

            def words(lo, hi, bits):
                return (jnp.where(lo, jnp.uint32(bits), jnp.uint32(0))
                        | jnp.where(hi, jnp.uint32(bits << 16), jnp.uint32(0)))
            kvar = [(2 * v + 1, (2 * v + 2) % RM) for v in range(7)] + [(None, 0), (191 % RM, None)]
            qvar = [(2 * v, 2 * v + 1) for v in range(7)] + [(3, 3), (188 % RM, 188 % RM)]
            for v in range(9):
                augx_ref[m, v] = words(kaug(kvar[v][0]), kaug(kvar[v][1]), ONE)
                augq_ref[m, v] = words(qaug(qvar[v][0]), qaug(qvar[v][1]), NBIG)
        pad_plane = jnp.where(_iota((XR, 128), 1) == L_PAD, jnp.uint32(ONE2), jnp.uint32(0))
        for pr in range(2):
            for sl in range(NR):
                for p in range(4):
                    x2_ref[sl, pr, p, 0:8] = pad_word
                    x2_ref[sl, pr, p, XR - 8:XR] = pad_word
                    if sl == 0 and p < 2:
                        x2_ref[sl, pr, p] = pad_plane
                        xs_ref[sl, pr, p] = pad_word
        xbuf_ref[0, 0:2] = jnp.zeros((2, C, W), bf16)

    colpatch_lane = (lane8 >= L_COL) & (lane8 < L_ONE)
    klabel = jnp.where(lane8 - L_COL == 7 + sub8, jnp.uint32(ONE2), jnp.uint32(0))
    qlabel = jnp.where(lane8 - L_COL < 8, jnp.uint32(NBIG * 0x10001), jnp.uint32(0))

    def key_words(xa, xb, aug, tile, pr, p, m, dup=None):
        slot = tile % NR
        w = jnp.concatenate([_packi(_unpack(xa, 0), _unpack(xb, 0)), _packi(_unpack(xa, 1), _unpack(xb, 1)), aug],
                            axis=0)
        wt = w.T
        for sl_, p_ in [(slot, p)] + ([dup] if dup else []):
            x2_ref[sl_, pr, p_, 8 + 128 * m:8 + 128 * (m + 1)] = wt
            if m == 2:
                xs_ref[sl_, pr, p_] = jnp.where(colpatch_lane, klabel, x2_ref[sl_, pr, p_, _s2(8 + 369)])

    def pre_unit(xsrc, r0, blk, tile, pr, k, m, dup=None, part=3):
        rows = [xsrc[r0 + 2 * il + pr, :, m * 128:(m + 1) * 128] for il in (2 * k - 1, 2 * k, 2 * k + 1)]
        ra = 8 * blk + 2 * k
        vx = jnp.where(ra < 1, 7, ((ra + RM - 1) % RM) // 2)
        vq = jnp.where(ra < 3, 7, jnp.where(ra >= 188, 8, (ra % RM) // 2))
        if part & 1:
            key_words(_u(rows[0]), _u(rows[1]), augx_ref[m, vx], tile + k // 2, pr, (k + 2) % 4, m, dup)
        if not part & 2:
            return
        at = _b(at_ref[...])
        qw = jnp.concatenate([_packi(_nn(at, rows[1]), _nn(at, rows[2])), augq_ref[m, vq]], axis=0)
        slot = tile % NR
        q2_ref[slot, pr, k, 128 * m:128 * (m + 1)] = qw.T
        if m == 2:
            qs_ref[slot, pr, k] = jnp.where(lo4, q2_ref[slot, pr, k, _s2(1)],
                                            jnp.where(colpatch_lane, qlabel, q2_ref[slot, pr, k, _s2(368)]))

    def keytile(tiles_pairs, pr, vi):
        pc, j = VSTRIPS[vi]
        vs = []
        for tile, p in tiles_pairs:
            if j == NS:
                vs += [x2_ref[tile % NR, pr, p, _s2(8)], xs_ref[tile % NR, pr, p]]
            else:
                vs += [x2_ref[tile % NR, pr, p, _s2(16 * j + pc)], x2_ref[tile % NR, pr, p, _s2(16 * j + 16 + pc)]]
        return _b(jnp.concatenate(vs, axis=0))

    def qrows(tiles_pairs, pr, vi):
        pc, j = VSTRIPS[vi]
        return [qs_ref[tile % NR, pr, k] if j == NS else q2_ref[tile % NR, pr, k, _s2(16 * j + pc)]
                for tile, k in tiles_pairs]

    sib_inv = {}

    def out_unit(dst, r0, h, m):
        pr = h % 2
        i = h // 2

        def words(half):
            return jnp.concatenate([ow_ref[pr, i // 2, 8 * m + v, _s2(half), :] for v in range(8)], axis=0)
        if i % 2 == 0:
            w = jnp.where(_iota((64, 128), 1) == L_ONE2, words(1), words(0))
            r = _nt(_b(bt_ref[...]), _b(w))
            inv = 1.0 / r[C:C + 2]
            sib_inv[h + 2, m] = inv[1:2]
            inv = inv[0:1]
        else:
            r = _nt(_b(bt_ref[0:C // 2]), _b(words(1)))
            inv = sib_inv.pop((h, m))
        dst[(r0 + h) // 2, h % 2, :, m * 128:(m + 1) * 128] = (r[0:C] * inv).astype(bf16)

    def in_copy(p):
        return pltpu.make_async_copy(x_hbm.at[pl.ds(32 * p - 2, 34)], xbuf_ref.at[p % 2], sem.at[p % 2])

    def in_part(i):
        b, r0, nr = IN_PARTS[i]
        return pltpu.make_async_copy(x_hbm.at[pl.ds(32 * b - 2 + r0, nr)], xbuf_ref.at[b, pl.ds(r0, nr)],
                                     sem.at[5 + i])

    def w_copy(i):
        return pltpu.make_async_copy((wqkv_hbm, wo_hbm)[i], (wqkv_ref, wo_ref)[i], sem.at[14 + i])

    def out_copy(p, half):
        return pltpu.make_async_copy(obuf_ref.at[p % 3, pl.ds(8 * half, 8)], out_ref.at[pl.ds(16 * p + 8 * half, 8)],
                                     sem.at[(2, 16)[half] + p % 3])

    def out_part(h, m):
        return pltpu.make_async_copy(obuf_ref.at[(NP - 1) % 3, 8 + h // 2, h % 2, :, pl.ds(128 * m, 128)],
                                     out_ref.at[16 * (NP - 1) + 8 + h // 2, h % 2, :, pl.ds(128 * m, 128)],
                                     sem.at[5 + m])

    def colidx(n):
        r = _iota((n, 128), 0)
        return 4 * ((r // 8) % 2) + (r % 8) // 2

    def store_pair(res, key0, key1, keysp, j, col):
        o0 = res.pop(key0)
        o1 = res.pop(key1)
        if j == 0:
            o1 = jnp.where(col < 3, res[keysp], o1)
        if j == NS - 1:
            o0 = jnp.where(col >= 5, res.pop(keysp), o0)
        return _packi(o0, o1)

    def attn_stage(base, blk0, nsub, with_pre, xsrc, o_prev, o_cur, o_prev_r0, o_cur_r0, top, calls=(), bot=False):
        nt = 2 * NV
        sch = FIRST if top else LAST if bot else MAIN
        la = sch['la']
        gtiles = []
        for d in range(nsub):
            if bot and d == nsub - 1:
                gtiles += [(d, pr, vi) for pr in (1, 0) for vi in [NV - 1] + list(range(NV - 1))]
            else:
                gtiles += [(d, pr, vi) for pr in range(2) for vi in [NV - 1] + list(range(NV - 1))]
        ntot = len(gtiles)
        col = colidx(64)
        sl = _iota((32, 128), 0)
        ln = _iota((32, 128), 1)
        mnew = (2 * (ln // 32) + ln % 2) <= (2 + 2 * (sl // 16) + sl % 2)
        odd16 = _iota((16, 128), 0) % 2 == 1
        svals = {}
        pvals = {}
        res = {}

        def tile_a(d, pr, vi):
            g = base + d
            return keytile([(g + 1, 0), (g, 1), (g, 2), (g, 3)], pr, vi)

        def tile_b(d, pr, vi):
            return keytile([(base + d + 1, p) for p in range(4)], pr, vi)

        def border(d):
            return 'top' if top and d == 0 else 'bot' if bot and d == nsub - 1 else None

        def pairs(d, pr):
            bd = border(d)
            pa, pb = [0, 1, 2], [1, 2, 3]
            if (bd, pr) == ('top', 1):
                pa = [1, 2]
            if (bd, pr) == ('bot', 0):
                pb = [1, 2]
            return pa, pb, (bd, pr) == ('top', 0), (bd, pr) == ('bot', 1)

        def qka(d, pr, vi):
            pa, _, xa, _ = pairs(d, pr)
            ql = qrows([(base + d, k) for k in pa], pr, vi)
            if xa:
                ql = ql + qrows([(base + d, 0), (base + d, 1)], 1, vi)
            svals[(d, pr, vi)] = _nt(_b(jnp.concatenate(ql, axis=0)), tile_a(d, pr, vi))

        def qkb(d, pr, vi):
            pa, pb, xa, xb = pairs(d, pr)
            ql = qrows([(base + d, k) for k in pb], pr, vi)
            if xb:
                ql = ql + qrows([(base + d, 2), (base + d, 3)], 0, vi)
            sb = _nt(_b(jnp.concatenate(ql, axis=0)), tile_b(d, pr, vi))
            sa = svals.pop((d, pr, vi))
            na = 16 * (len(pa) - 2)
            parts = [sa[0:na]] if na else []
            parts += [jnp.maximum(sa[na:na + 32], sb[0:32])]
            parts += [sb[32:]] if sb.shape[0] > 32 else []
            parts += [sa[48:80]] if xa else []
            comb = jnp.concatenate(parts, axis=0)
            m = jnp.max(comb, axis=1, keepdims=True)
            e = jnp.exp2(comb - m)
            nb = na + 32 + sb.shape[0] - 32
            mid = e[na:na + 32]
            pn = jnp.concatenate([jnp.where(mnew, mid, 0.0)] + ([e[na + 32:nb]] if sb.shape[0] > 32 else []), axis=0)
            po = jnp.concatenate(([e[0:na]] if na else []) + [jnp.where(mnew, 0.0, mid)]
                                 + ([e[nb:]] if xa else []), axis=0)
            pvals[(d, pr, vi)] = (pn.astype(bf16), po.astype(bf16))

        def pva(d, pr, vi):
            res[(pr, vi, 'a')] = _nn(pvals[(d, pr, vi)][1], tile_a(d, pr, vi))

        def pvb(d, pr, vi):
            pa, pb, xa, xb = pairs(d, pr)
            pn, po = pvals.pop((d, pr, vi))
            o = _nn(pn, tile_b(d, pr, vi))
            oa = res.pop((pr, vi, 'a'))
            na = 16 * (len(pa) - 2)
            res[(pr, vi)] = jnp.concatenate(([oa[0:na]] if na else []) + [oa[na:na + 32] + o[0:32]]
                                            + ([o[32:48]] if len(pb) == 3 else []), axis=0)
            if xa or xb:
                res[(pr, vi, 'x')] = oa[48:80] if xa else o[48:80]
            if vi < 2 * NS and vi % 2 == 1:
                j = vi // 2
                w = store_pair(res, (pr, vi - 1), (pr, vi), (pr, NV - 1), j, col[0:16 * (len(pa) + len(pb) - 2)])
                if (border(d), pr) == ('top', 1):
                    w = w[16 * (len(pa) - 2):]
                    ow_ref[pr, 1, j] = jnp.where(odd16, w[0:16], ow_ref[pr, 1, j])
                    ow_ref[pr, 2:4, j] = w[16:48].reshape(2, 16, 128)
                elif (border(d), pr) == ('bot', 0):
                    ow_ref[pr, 0:2, j] = w[0:32].reshape(2, 16, 128)
                    ow_ref[pr, 2, j] = jnp.where(odd16, ow_ref[pr, 2, j], w[32:48])
                else:
                    ow_ref[pr, :, j] = w.reshape(4, 16, 128)
                if xa or xb:
                    wx = store_pair(res, (pr, vi - 1, 'x'), (pr, vi, 'x'), (pr, NV - 1, 'x'), j, col[0:32])
                    p0 = 0 if xa else 2
                    ow_ref[1 - pr, p0:p0 + 2, j] = wx.reshape(2, 16, 128)

        extra = {}
        mark = {}
        done = {}
        for n, (d, pr, vi) in enumerate(gtiles):
            if vi < 2 * NS:
                done[d, pr, vi // 16] = n + la
        for d in range(nsub):
            off = d * nt
            dst_late = (o_prev, o_prev_r0) if d == 0 else (o_cur, o_cur_r0 + 16 * (d - 1))
            dst = (o_cur, o_cur_r0 + 16 * d)
            for n, (h, m) in enumerate([] if top and d == 0 else LATE_UNITS):
                pos_ = sch['late0'] + n if d == 0 else off + la + sch['late'] + 2 * n
                extra.setdefault(pos_, []).append(('o', dst_late, h, m))
                mark['late', d] = pos_
            for h, m in (EARLY_UNITS + LATE_UNITS if border(d) == 'bot' else EARLY_UNITS):
                pr, i = h % 2, h // 2
                if border(d) == 'bot':
                    pr = 1 if i >= 6 else pr
                    pos_ = done[d, pr, m] + (sch['lag_end'] if (pr, m) == (0, 2) else sch['lag_b'] + i)
                elif with_pre and d == nsub - 1 and pr == 1 and m == 1 and i >= 8 - sch['nfill']:
                    pos_ = ntot + la + sch['fpos'] + (sch['fstep'] * (i - 8 + sch['nfill'])) // 2
                else:
                    pos_ = done[d, pr, m] + sch['lag'] + 2 * i
                if i % 2 == 1:
                    pos_ = max(pos_, mark['unit', d, h - 2, m])
                extra.setdefault(pos_, []).append(('o', dst, h, m))
                mark['unit', d, h, m] = pos_
            if with_pre:
                span = nt + (sch['p1'] if d == nsub - 1 else 0) - (sch['p0'] if d == 0 else 0)
                start = off + (sch['p0'] if d == 0 else 0)
                for n, un in enumerate(PRE_UNITS):
                    pos_ = start + (n * span) // len(PRE_UNITS)
                    if top and (d, n) == (0, 12):
                        extra.setdefault(pos_, []).append(('c', lambda: in_part(7).wait()))
                        extra[pos_].append(('c', lambda: in_part(8).wait()))
                        extra[pos_].append(('c', lambda: in_copy(2).start()))
                    if sch['split'] is None:
                        extra.setdefault(pos_, []).append(('p', d) + un + (None, 3))
                    else:
                        extra.setdefault(pos_ + max(sch['split'], 0), []).append(('p', d) + un + (None, 2))
                        extra.setdefault(pos_ + max(-sch['split'], 0), []).append(('p', d) + un + (None, 1))
        mark['end'] = max(extra)
        for pos_, fn in calls:
            pos_ = min(mark[pos_] + sch['dma_lag'], mark['end']) if pos_ in mark else pos_
            extra.setdefault(pos_, []).append(('c', fn))
        nslot = max([ntot + la + 2] + [k + 1 for k in extra])
        for n in range(nslot):
            for op, k in ((qka, n), (pva, n - la), (qkb, n), (pvb, n - la)):
                if 0 <= k < ntot:
                    op(*gtiles[k])
            for e in extra.get(n, []):
                if e[0] == 'o':
                    out_unit(e[1][0], e[1][1], e[2], e[3])
                elif e[0] == 'c':
                    e[1]()
                else:
                    d = e[1]
                    pre_unit(xsrc, 2 + 16 * d, blk0 + 2 + d, base + 2 + d, *e[2:])

    def main_block(par):
        attn_stage(2 * par + 2, 2 * t - 2, 2, True, xbuf_ref.at[par], obuf_ref.at[(t + 1) % 3],
                   obuf_ref.at[(t + 2) % 3], 16, 0, False)

    def first_block():
        in_part(6).wait()
        attn_stage(0, 0, 2, True, xbuf_ref.at[1], None, obuf_ref.at[0], 0, 0, True)

    def last_block():
        last = obuf_ref.at[(NP - 1) % 3]
        prev = obuf_ref.at[(NP - 2) % 3]

        def tail_keys(pr, m):
            xa = _u(xbuf_ref[(NP - 1) % 2, 32 + pr, :, m * 128:(m + 1) * 128])
            key_words(xa, jnp.zeros_like(xa), augx_ref[m, 8], NB, pr, 2, m)

        def tail_fill():
            x2_ref[NB % NR, 0, 3] = jnp.where(_iota((XR, 128), 1) == L_PAD, jnp.uint32(ONE2), jnp.uint32(0))
            xs_ref[NB % NR, 0, 3] = pad_word
            x2_ref[NB % NR, 1, 3] = x2_ref[(NB - 1) % NR, 1, 3]
            xs_ref[NB % NR, 1, 3] = xs_ref[(NB - 1) % NR, 1, 3]

        calls = [(LAST['tail'] + 6 * n, lambda pr=n // 3, m=n % 3: tail_keys(pr, m)) for n in range(6)]
        calls += [(LAST['tail'] + 36, tail_fill),
                  (('late', 0), lambda: out_copy(NP - 2, 1).start()),
                  (('late', 1), lambda: out_copy(NP - 1, 0).start()),
                  ]
        calls += [(('unit', 1, h, m), lambda h=h, m=m: out_part(h, m).start()) for m in range(3) for h in range(16)]
        attn_stage(NB - 2, NB - 2, 2, False, None, prev, last, 16, 0, False, calls, True)
        for p, half in ((NP - 3, 0), (NP - 3, 1), (NP - 2, 0), (NP - 2, 1), (NP - 1, 0)):
            out_copy(p, half).wait()
        for m in range(3):
            for h in range(16):
                out_part(h, m).wait()

    @pl.when(t == 0)
    def _():
        w_copy(0).start()
        w_copy(1).start()
        for i in range(6):
            in_part(i).start()
        _setup_tables()
        w_copy(0).wait()
        w_copy(1).wait()
        _setup_at()
        _setup_bt()
        for k in range(4):
            in_part(k).wait()
            if k == 1:
                for i in range(6, 9):
                    in_part(i).start()
            for pr in range(2):
                for m in range(3):
                    pre_unit(xbuf_ref.at[0], 2, 0, 0, pr, k, m, (0, 1) if (pr, k) == (0, 3) else None)
        for k in range(4):
            if k % 2 == 0:
                in_part(4 + k // 2).wait()
            for pr in range(2):
                for m in range(3):
                    pre_unit(xbuf_ref.at[0], 18, 1, 1, pr, k, m)

    @pl.when(t >= 1)
    def _():
        @pl.when((t >= 2) & (t < NP))
        def _():
            in_copy(t).wait()

        @pl.when((t >= 2) & (t < NP - 1))
        def _():
            in_copy(t + 1).start()

        @pl.when(t >= 4)
        def _():
            out_copy(t - 4, 0).wait()
            out_copy(t - 4, 1).wait()

    @pl.when(t == 1)
    def _():
        first_block()

    for par in range(2):
        @pl.when((t >= 2) & (t < NP) & (t % 2 == par))
        def _():
            main_block(par)

    @pl.when((t >= 2) & (t < NP))
    def _():
        out_copy(t - 2, 1).start()

    @pl.when((t >= 1) & (t < NP))
    def _():
        out_copy(t - 1, 0).start()

    @pl.when(t == NP)
    def _():
        last_block()


@jax.jit
def pallas_standalone__neighborhood_nat__vision_kernel(x, wqkv, wo):
    xt = jnp.transpose(x.reshape(H, W, C), (0, 2, 1))
    out = pl.pallas_call(
        _kernel,
        grid=(NP + 1,),
        in_specs=[
            pl.BlockSpec(memory_space=pl.ANY),
            pl.BlockSpec(memory_space=pl.ANY),
            pl.BlockSpec(memory_space=pl.ANY),
        ],
        out_specs=pl.BlockSpec(memory_space=pl.ANY),
        out_shape=jax.ShapeDtypeStruct((H // 2, 2, C, W), bf16),
        scratch_shapes=[
            pltpu.VMEM((C, 3 * C), bf16),
            pltpu.VMEM((C, C), bf16),
            pltpu.VMEM((48, 96), u32),
            pltpu.VMEM((56, 128), u32),
            pltpu.VMEM((3, 9, 32, 128), u32),
            pltpu.VMEM((3, 9, 32, 128), u32),
            pltpu.VMEM((NR, 2, 4, XR, 128), u32),
            pltpu.VMEM((NR, 2, 4, 8, 128), u32),
            pltpu.VMEM((NR, 2, 4, W, 128), u32),
            pltpu.VMEM((NR, 2, 4, 8, 128), u32),
            pltpu.VMEM((2, 4, NS, 16, 128), u32),
            pltpu.VMEM((2, 34, C, W), bf16),
            pltpu.VMEM((3, 16, 2, C, W), bf16),
            pltpu.SemaphoreType.DMA((19,)),
        ],
        compiler_params=pltpu.CompilerParams(
            dimension_semantics=("arbitrary",), vmem_limit_bytes=64 * 1024 * 1024,
            disable_bounds_checks=True),
        name="nat_kernel",
    )(xt, wqkv, wo)
    return jnp.transpose(out.reshape(H, C, W), (0, 2, 1)).reshape(1, H, W, C)
```

```python
import math

import jax
import jax.numpy as jnp
from jax import lax
from jax.experimental import pallas as pl
from jax.experimental.pallas import tpu as pltpu

H = 384
W = 384
C = 96
NP = 12
NB = 24
NS = 24
NR = 4
XR = W + 16
ONE = 0x3F80
ONE2 = 0x3F803F80
NBIG = 0xF180
RM = 14
CM = 15
L_COL = 110
L_ONE = 125
L_PAD = 126
L_ONE2 = 127

MAIN = dict(la=13, lag=6, p0=10, p1=-10, split=-3, nfill=4, fpos=-7, fstep=0, late=6, late0=0)
FIRST = dict(la=11, lag=10, p0=12, p1=-10, split=None, nfill=5, fpos=-5, fstep=0, late=8, late0=0)
LAST = dict(la=11, lag=6, late=6, late0=1, lag_b=5, lag_end=1, dma_lag=3, tail=4)


IN_PARTS = [(0, 2, 4), (0, 6, 4), (0, 10, 4), (0, 14, 4), (0, 18, 8), (0, 26, 8), (1, 0, 10), (1, 10, 8), (1, 18, 16)]
PRE_UNITS = [(pr, k, m) for k in range(4) for pr in range(2) for m in range(3)]

bf16 = jnp.bfloat16
f32 = jnp.float32
u32 = jnp.uint32
i32 = jnp.int32


def _iota(shape, dim):
    return lax.broadcasted_iota(i32, shape, dim)


def _nt(a, b):
    return lax.dot_general(a, b, (((1,), (1,)), ((), ())), preferred_element_type=f32)


def _nn(a, b):
    return lax.dot_general(a, b, (((1,), (0,)), ((), ())), preferred_element_type=f32)


def _unpack(u, idx):
    return pltpu.unpack_elementwise(u, index=idx, packed_dtype=bf16, unpacked_dtype=f32)


def _packi(a, b):
    return pltpu.pack_elementwise([a, b], packed_dtype=bf16)


def _b(u):
    return pltpu.bitcast(u, bf16)


def _u(b):
    return pltpu.bitcast(b, u32)


def _s2(start):
    return pl.ds(start, 8, stride=2)


VSTRIPS = [(pc, j) for j in range(NS) for pc in range(2)] + [(0, NS)]
NV = len(VSTRIPS)
LATE_UNITS = [(2 * i + 1, 2) for i in range(8)]
EARLY_UNITS = [(h, m) for h in range(16) for m in range(3) if (h, m) not in LATE_UNITS]


def _kernel(x_hbm, wqkv_hbm, wo_hbm, out_ref,
            wqkv_ref, wo_ref, at_ref, bt_ref, augx_ref, augq_ref, x2_ref, xs_ref, q2_ref, qs_ref, ow_ref,
            xbuf_ref, obuf_ref, sem):
    t = pl.program_id(0)
    sub8 = _iota((8, 128), 0)
    lane8 = _iota((8, 128), 1)
    pad_word = jnp.where(lane8 == L_PAD, jnp.uint32(ONE2), jnp.uint32(0))
    lo4 = sub8 < 4

    def _perm():
        pl_ = _iota((C, C), 0)
        pc_ = _iota((C, C), 1)
        return jnp.where(pc_ == jnp.where(pl_ < C // 2, 2 * pl_, 2 * (pl_ - C // 2) + 1), 1.0, 0.0).astype(bf16)

    def _setup_at():
        wq = wqkv_ref[:, 0:C]
        wk = wqkv_ref[:, C:2 * C]
        perm = _perm()
        at = (_nt(wk, wq) * (C ** -0.5 * math.log2(math.e))).astype(bf16)
        at_ref[...] = _u(_nn(perm, at).astype(bf16))

    def _setup_bt():
        wv = wqkv_ref[:, 2 * C:3 * C]
        perm = _perm()
        b = _nn(wv, wo_ref[...]).astype(bf16)
        bt = _nn(perm, b).T
        bt = jnp.concatenate([bt, jnp.zeros((C, 128 - C), f32)], axis=1)
        bt = jnp.concatenate([bt, jnp.zeros((112 - C, 128), f32)], axis=0)
        r = _iota((112, 128), 0)
        c = _iota((112, 128), 1)
        sel = (((r == C) & (c == L_ONE)) | ((r == C + 1) & (c == L_ONE2)) | ((r == C + 2) & (c >= C) & (c < L_COL))
               | ((r == C + 3) & (c >= L_COL) & (c < L_ONE)))
        bt_ref[...] = _u(jnp.where(sel, 1.0, bt).astype(bf16))

    def _setup_tables():
        rho = _iota((32, 128), 0)
        for m in range(3):
            ccol = (m * 128 + _iota((32, 128), 1)) // 2
            kcol = ((rho >= 14) & (rho < 29) & (rho - 14 == ccol % CM)) | (rho == 29) | (rho == 31)
            ccq = jnp.clip(ccol, 3, 188) % CM
            qcol = ((rho >= 14) & (rho < 29) & (((rho - 14 - ccq + 3 + CM) % CM) > 6)) | (rho == 30)

            def kaug(res):
                return rho == 30 if res is None else kcol | (rho == res)

            def qaug(res):
                return qcol | ((rho < 14) & (((rho - res + 3 + RM) % RM) > 6))

            def words(lo, hi, bits):
                return (jnp.where(lo, jnp.uint32(bits), jnp.uint32(0))
                        | jnp.where(hi, jnp.uint32(bits << 16), jnp.uint32(0)))
            kvar = [(2 * v + 1, (2 * v + 2) % RM) for v in range(7)] + [(None, 0), (191 % RM, None)]
            qvar = [(2 * v, 2 * v + 1) for v in range(7)] + [(3, 3), (188 % RM, 188 % RM)]
            for v in range(9):
                augx_ref[m, v] = words(kaug(kvar[v][0]), kaug(kvar[v][1]), ONE)
                augq_ref[m, v] = words(qaug(qvar[v][0]), qaug(qvar[v][1]), NBIG)
        pad_plane = jnp.where(_iota((XR, 128), 1) == L_PAD, jnp.uint32(ONE2), jnp.uint32(0))
        for pr in range(2):
            for sl in range(NR):
                for p in range(4):
                    x2_ref[sl, pr, p, 0:8] = pad_word
                    x2_ref[sl, pr, p, XR - 8:XR] = pad_word
                    if sl == 0 and p < 2:
                        x2_ref[sl, pr, p] = pad_plane
                        xs_ref[sl, pr, p] = pad_word
        xbuf_ref[0, 0:2] = jnp.zeros((2, C, W), bf16)

    colpatch_lane = (lane8 >= L_COL) & (lane8 < L_ONE)
    klabel = jnp.where(lane8 - L_COL == 7 + sub8, jnp.uint32(ONE2), jnp.uint32(0))
    qlabel = jnp.where(lane8 - L_COL < 8, jnp.uint32(NBIG * 0x10001), jnp.uint32(0))

    def key_words(xa, xb, aug, tile, pr, p, m, dup=None):
        slot = tile % NR
        w = jnp.concatenate([_packi(_unpack(xa, 0), _unpack(xb, 0)), _packi(_unpack(xa, 1), _unpack(xb, 1)), aug],
                            axis=0)
        wt = w.T
        for sl_, p_ in [(slot, p)] + ([dup] if dup else []):
            x2_ref[sl_, pr, p_, 8 + 128 * m:8 + 128 * (m + 1)] = wt
            if m == 2:
                xs_ref[sl_, pr, p_] = jnp.where(colpatch_lane, klabel, x2_ref[sl_, pr, p_, _s2(8 + 369)])

    def pre_unit(xsrc, r0, blk, tile, pr, k, m, dup=None, part=3):
        rows = [xsrc[r0 + 2 * il + pr, :, m * 128:(m + 1) * 128] for il in (2 * k - 1, 2 * k, 2 * k + 1)]
        ra = 8 * blk + 2 * k
        vx = jnp.where(ra < 1, 7, ((ra + RM - 1) % RM) // 2)
        vq = jnp.where(ra < 3, 7, jnp.where(ra >= 188, 8, (ra % RM) // 2))
        if part & 1:
            key_words(_u(rows[0]), _u(rows[1]), augx_ref[m, vx], tile + k // 2, pr, (k + 2) % 4, m, dup)
        if not part & 2:
            return
        at = _b(at_ref[...])
        qw = jnp.concatenate([_packi(_nn(at, rows[1]), _nn(at, rows[2])), augq_ref[m, vq]], axis=0)
        slot = tile % NR
        q2_ref[slot, pr, k, 128 * m:128 * (m + 1)] = qw.T
        if m == 2:
            qs_ref[slot, pr, k] = jnp.where(lo4, q2_ref[slot, pr, k, _s2(1)],
                                            jnp.where(colpatch_lane, qlabel, q2_ref[slot, pr, k, _s2(368)]))

    def keytile(tiles_pairs, pr, vi):
        pc, j = VSTRIPS[vi]
        vs = []
        for tile, p in tiles_pairs:
            if j == NS:
                vs += [x2_ref[tile % NR, pr, p, _s2(8)], xs_ref[tile % NR, pr, p]]
            else:
                vs += [x2_ref[tile % NR, pr, p, _s2(16 * j + pc)], x2_ref[tile % NR, pr, p, _s2(16 * j + 16 + pc)]]
        return _b(jnp.concatenate(vs, axis=0))

    def qrows(tiles_pairs, pr, vi):
        pc, j = VSTRIPS[vi]
        return [qs_ref[tile % NR, pr, k] if j == NS else q2_ref[tile % NR, pr, k, _s2(16 * j + pc)]
                for tile, k in tiles_pairs]

    sib_inv = {}

    sib_inv = {}

    def out_unit(dst, r0, h, m, size):
        pr = h % 2
        i = h // 2

        def words(i_):
            return jnp.concatenate([ow_ref[pr, i_ // 2, 8 * m + v, _s2(i_ % 2), :] for v in range(8)], axis=0)
        if i % size == 0:
            lane = _iota((64, 128), 1)
            w = jnp.where(lane == L_ONE2, words(i + 1), words(i))
            if size == 4:
                w = jnp.where((lane >= C) & (lane < L_COL), words(i + 2), w)
                w = jnp.where((lane >= L_COL) & (lane < L_ONE), words(i + 3), w)
            r = _nt(_b(bt_ref[...]), _b(w))
            inv = 1.0 / r[C:C + 8]
            for n in range(1, size):
                sib_inv[h + 2 * n, m] = inv[n:n + 1]
            inv = inv[0:1]
        else:
            r = _nt(_b(bt_ref[0:C // 2]), _b(words(i)))
            inv = sib_inv.pop((h, m))
        dst[(r0 + h) // 2, h % 2, :, m * 128:(m + 1) * 128] = (r[0:C] * inv).astype(bf16)

    def in_copy(p):
        return pltpu.make_async_copy(x_hbm.at[pl.ds(32 * p - 2, 34)], xbuf_ref.at[p % 2], sem.at[p % 2])

    def in_part(i):
        b, r0, nr = IN_PARTS[i]
        return pltpu.make_async_copy(x_hbm.at[pl.ds(32 * b - 2 + r0, nr)], xbuf_ref.at[b, pl.ds(r0, nr)],
                                     sem.at[5 + i])

    def w_copy(i):
        return pltpu.make_async_copy((wqkv_hbm, wo_hbm)[i], (wqkv_ref, wo_ref)[i], sem.at[14 + i])

    def out_copy(p, half):
        return pltpu.make_async_copy(obuf_ref.at[p % 3, pl.ds(8 * half, 8)], out_ref.at[pl.ds(16 * p + 8 * half, 8)],
                                     sem.at[(2, 16)[half] + p % 3])

    def out_part(h, m):
        return pltpu.make_async_copy(obuf_ref.at[(NP - 1) % 3, 8 + h // 2, h % 2, :, pl.ds(128 * m, 128)],
                                     out_ref.at[16 * (NP - 1) + 8 + h // 2, h % 2, :, pl.ds(128 * m, 128)],
                                     sem.at[5 + m])

    def colidx(n):
        r = _iota((n, 128), 0)
        return 4 * ((r // 8) % 2) + (r % 8) // 2

    def store_pair(res, key0, key1, keysp, j, col):
        o0 = res.pop(key0)
        o1 = res.pop(key1)
        if j == 0:
            o1 = jnp.where(col < 3, res[keysp], o1)
        if j == NS - 1:
            o0 = jnp.where(col >= 5, res.pop(keysp), o0)
        return _packi(o0, o1)

    def attn_stage(base, blk0, nsub, with_pre, xsrc, o_prev, o_cur, o_prev_r0, o_cur_r0, top, calls=(), bot=False):
        nt = 2 * NV
        sch = FIRST if top else LAST if bot else MAIN
        la = sch['la']
        gtiles = []
        for d in range(nsub):
            if bot and d == nsub - 1:
                gtiles += [(d, pr, vi) for pr in (1, 0) for vi in [NV - 1] + list(range(NV - 1))]
            else:
                gtiles += [(d, pr, vi) for pr in range(2) for vi in [NV - 1] + list(range(NV - 1))]
        ntot = len(gtiles)
        col = colidx(64)
        sl = _iota((32, 128), 0)
        ln = _iota((32, 128), 1)
        mnew = (2 * (ln // 32) + ln % 2) <= (2 + 2 * (sl // 16) + sl % 2)
        odd16 = _iota((16, 128), 0) % 2 == 1
        svals = {}
        pvals = {}
        res = {}

        def tile_a(d, pr, vi):
            g = base + d
            return keytile([(g + 1, 0), (g, 1), (g, 2), (g, 3)], pr, vi)

        def tile_b(d, pr, vi):
            return keytile([(base + d + 1, p) for p in range(4)], pr, vi)

        def border(d):
            return 'top' if top and d == 0 else 'bot' if bot and d == nsub - 1 else None

        def pairs(d, pr):
            bd = border(d)
            pa, pb = [0, 1, 2], [1, 2, 3]
            if (bd, pr) == ('top', 1):
                pa = [1, 2]
            if (bd, pr) == ('bot', 0):
                pb = [1, 2]
            return pa, pb, (bd, pr) == ('top', 0), (bd, pr) == ('bot', 1)

        def qka(d, pr, vi):
            pa, _, xa, _ = pairs(d, pr)
            ql = qrows([(base + d, k) for k in pa], pr, vi)
            if xa:
                ql = ql + qrows([(base + d, 0), (base + d, 1)], 1, vi)
            svals[(d, pr, vi)] = _nt(_b(jnp.concatenate(ql, axis=0)), tile_a(d, pr, vi))

        def qkb(d, pr, vi):
            pa, pb, xa, xb = pairs(d, pr)
            ql = qrows([(base + d, k) for k in pb], pr, vi)
            if xb:
                ql = ql + qrows([(base + d, 2), (base + d, 3)], 0, vi)
            sb = _nt(_b(jnp.concatenate(ql, axis=0)), tile_b(d, pr, vi))
            sa = svals.pop((d, pr, vi))
            na = 16 * (len(pa) - 2)
            parts = [sa[0:na]] if na else []
            parts += [jnp.maximum(sa[na:na + 32], sb[0:32])]
            parts += [sb[32:]] if sb.shape[0] > 32 else []
            parts += [sa[48:80]] if xa else []
            comb = jnp.concatenate(parts, axis=0)
            m = jnp.max(comb, axis=1, keepdims=True)
            e = jnp.exp2(comb - m)
            nb = na + 32 + sb.shape[0] - 32
            mid = e[na:na + 32]
            pn = jnp.concatenate([jnp.where(mnew, mid, 0.0)] + ([e[na + 32:nb]] if sb.shape[0] > 32 else []), axis=0)
            po = jnp.concatenate(([e[0:na]] if na else []) + [jnp.where(mnew, 0.0, mid)]
                                 + ([e[nb:]] if xa else []), axis=0)
            pvals[(d, pr, vi)] = (pn.astype(bf16), po.astype(bf16))

        def pva(d, pr, vi):
            res[(pr, vi, 'a')] = _nn(pvals[(d, pr, vi)][1], tile_a(d, pr, vi))

        def pvb(d, pr, vi):
            pa, pb, xa, xb = pairs(d, pr)
            pn, po = pvals.pop((d, pr, vi))
            o = _nn(pn, tile_b(d, pr, vi))
            oa = res.pop((pr, vi, 'a'))
            na = 16 * (len(pa) - 2)
            res[(pr, vi)] = jnp.concatenate(([oa[0:na]] if na else []) + [oa[na:na + 32] + o[0:32]]
                                            + ([o[32:48]] if len(pb) == 3 else []), axis=0)
            if xa or xb:
                res[(pr, vi, 'x')] = oa[48:80] if xa else o[48:80]
            if vi < 2 * NS and vi % 2 == 1:
                j = vi // 2
                w = store_pair(res, (pr, vi - 1), (pr, vi), (pr, NV - 1), j, col[0:16 * (len(pa) + len(pb) - 2)])
                if (border(d), pr) == ('top', 1):
                    w = w[16 * (len(pa) - 2):]
                    ow_ref[pr, 1, j] = jnp.where(odd16, w[0:16], ow_ref[pr, 1, j])
                    ow_ref[pr, 2:4, j] = w[16:48].reshape(2, 16, 128)
                elif (border(d), pr) == ('bot', 0):
                    ow_ref[pr, 0:2, j] = w[0:32].reshape(2, 16, 128)
                    ow_ref[pr, 2, j] = jnp.where(odd16, ow_ref[pr, 2, j], w[32:48])
                else:
                    ow_ref[pr, :, j] = w.reshape(4, 16, 128)
                if xa or xb:
                    wx = store_pair(res, (pr, vi - 1, 'x'), (pr, vi, 'x'), (pr, NV - 1, 'x'), j, col[0:32])
                    p0 = 0 if xa else 2
                    ow_ref[1 - pr, p0:p0 + 2, j] = wx.reshape(2, 16, 128)

        extra = {}
        mark = {}
        done = {}
        for n, (d, pr, vi) in enumerate(gtiles):
            if vi < 2 * NS:
                done[d, pr, vi // 16] = n + la
        for d in range(nsub):
            off = d * nt
            dst_late = (o_prev, o_prev_r0) if d == 0 else (o_cur, o_cur_r0 + 16 * (d - 1))
            dst = (o_cur, o_cur_r0 + 16 * d)
            for n, (h, m) in enumerate([] if top and d == 0 else LATE_UNITS):
                pos_ = sch['late0'] + n if d == 0 else off + la + sch['late'] + 2 * n
                extra.setdefault(pos_, []).append(('o', dst_late, h, m, 4))
                mark['late', d] = pos_
            for h, m in (EARLY_UNITS + LATE_UNITS if border(d) == 'bot' else EARLY_UNITS):
                pr, i = h % 2, h // 2
                if border(d) == 'bot':
                    pr = 1 if i >= 6 else pr
                    pos_ = done[d, pr, m] + (sch['lag_end'] if (pr, m) == (0, 2) else sch['lag_b'] + i)
                elif with_pre and d == nsub - 1 and pr == 1 and m == 1 and i >= 8 - sch['nfill']:
                    pos_ = ntot + la + sch['fpos'] + (sch['fstep'] * (i - 8 + sch['nfill'])) // 2
                else:
                    pos_ = done[d, pr, m] + sch['lag'] + 2 * i
                size = 2 if border(d) == 'bot' and h % 2 == 0 and i >= 4 else 4
                if i % size:
                    pos_ = max(pos_, mark['unit', d, h - 2 * (i % size), m])
                extra.setdefault(pos_, []).append(('o', dst, h, m, size))
                mark['unit', d, h, m] = pos_
            if with_pre:
                span = nt + (sch['p1'] if d == nsub - 1 else 0) - (sch['p0'] if d == 0 else 0)
                start = off + (sch['p0'] if d == 0 else 0)
                for n, un in enumerate(PRE_UNITS):
                    pos_ = start + (n * span) // len(PRE_UNITS)
                    if top and (d, n) == (0, 12):
                        extra.setdefault(pos_, []).append(('c', lambda: in_part(7).wait()))
                        extra[pos_].append(('c', lambda: in_part(8).wait()))
                        extra[pos_].append(('c', lambda: in_copy(2).start()))
                    if sch['split'] is None:
                        extra.setdefault(pos_, []).append(('p', d) + un + (None, 3))
                    else:
                        extra.setdefault(pos_ + max(sch['split'], 0), []).append(('p', d) + un + (None, 2))
                        extra.setdefault(pos_ + max(-sch['split'], 0), []).append(('p', d) + un + (None, 1))
        mark['end'] = max(extra)
        for pos_, fn in calls:
            pos_ = min(mark[pos_] + sch['dma_lag'], mark['end']) if pos_ in mark else pos_
            extra.setdefault(pos_, []).append(('c', fn))
        nslot = max([ntot + la + 2] + [k + 1 for k in extra])
        for n in range(nslot):
            for op, k in ((qka, n), (pva, n - la), (qkb, n), (pvb, n - la)):
                if 0 <= k < ntot:
                    op(*gtiles[k])
            for e in extra.get(n, []):
                if e[0] == 'o':
                    out_unit(e[1][0], e[1][1], e[2], e[3], e[4])
                elif e[0] == 'c':
                    e[1]()
                else:
                    d = e[1]
                    pre_unit(xsrc, 2 + 16 * d, blk0 + 2 + d, base + 2 + d, *e[2:])

    def main_block(par):
        attn_stage(2 * par + 2, 2 * t - 2, 2, True, xbuf_ref.at[par], obuf_ref.at[(t + 1) % 3],
                   obuf_ref.at[(t + 2) % 3], 16, 0, False)

    def first_block():
        in_part(6).wait()
        attn_stage(0, 0, 2, True, xbuf_ref.at[1], None, obuf_ref.at[0], 0, 0, True)

    def last_block():
        last = obuf_ref.at[(NP - 1) % 3]
        prev = obuf_ref.at[(NP - 2) % 3]

        def tail_keys(pr, m):
            xa = _u(xbuf_ref[(NP - 1) % 2, 32 + pr, :, m * 128:(m + 1) * 128])
            key_words(xa, jnp.zeros_like(xa), augx_ref[m, 8], NB, pr, 2, m)

        def tail_fill():
            x2_ref[NB % NR, 0, 3] = jnp.where(_iota((XR, 128), 1) == L_PAD, jnp.uint32(ONE2), jnp.uint32(0))
            xs_ref[NB % NR, 0, 3] = pad_word
            x2_ref[NB % NR, 1, 3] = x2_ref[(NB - 1) % NR, 1, 3]
            xs_ref[NB % NR, 1, 3] = xs_ref[(NB - 1) % NR, 1, 3]

        calls = [(LAST['tail'] + 6 * n, lambda pr=n // 3, m=n % 3: tail_keys(pr, m)) for n in range(6)]
        calls += [(LAST['tail'] + 36, tail_fill),
                  (('late', 0), lambda: out_copy(NP - 2, 1).start()),
                  (('late', 1), lambda: out_copy(NP - 1, 0).start()),
                  ]
        calls += [(('unit', 1, h, m), lambda h=h, m=m: out_part(h, m).start()) for m in range(3) for h in range(16)]
        attn_stage(NB - 2, NB - 2, 2, False, None, prev, last, 16, 0, False, calls, True)
        for p, half in ((NP - 3, 0), (NP - 3, 1), (NP - 2, 0), (NP - 2, 1), (NP - 1, 0)):
            out_copy(p, half).wait()
        for m in range(3):
            for h in range(16):
                out_part(h, m).wait()

    @pl.when(t == 0)
    def _():
        w_copy(0).start()
        w_copy(1).start()
        for i in range(6):
            in_part(i).start()
        _setup_tables()
        w_copy(0).wait()
        w_copy(1).wait()
        _setup_at()
        _setup_bt()
        for k in range(4):
            in_part(k).wait()
            if k == 1:
                for i in range(6, 9):
                    in_part(i).start()
            for pr in range(2):
                for m in range(3):
                    pre_unit(xbuf_ref.at[0], 2, 0, 0, pr, k, m, (0, 1) if (pr, k) == (0, 3) else None)
        for k in range(4):
            if k % 2 == 0:
                in_part(4 + k // 2).wait()
            for pr in range(2):
                for m in range(3):
                    pre_unit(xbuf_ref.at[0], 18, 1, 1, pr, k, m)

    @pl.when(t >= 1)
    def _():
        @pl.when((t >= 2) & (t < NP))
        def _():
            in_copy(t).wait()

        @pl.when((t >= 2) & (t < NP - 1))
        def _():
            in_copy(t + 1).start()

        @pl.when(t >= 4)
        def _():
            out_copy(t - 4, 0).wait()
            out_copy(t - 4, 1).wait()

    @pl.when(t == 1)
    def _():
        first_block()

    for par in range(2):
        @pl.when((t >= 2) & (t < NP) & (t % 2 == par))
        def _():
            main_block(par)

    @pl.when((t >= 2) & (t < NP))
    def _():
        out_copy(t - 2, 1).start()

    @pl.when((t >= 1) & (t < NP))
    def _():
        out_copy(t - 1, 0).start()

    @pl.when(t == NP)
    def _():
        last_block()


@jax.jit
def pallas_standalone__neighborhood_nat__vision_kernel(x, wqkv, wo):
    xt = jnp.transpose(x.reshape(H, W, C), (0, 2, 1))
    out = pl.pallas_call(
        _kernel,
        grid=(NP + 1,),
        in_specs=[
            pl.BlockSpec(memory_space=pl.ANY),
            pl.BlockSpec(memory_space=pl.ANY),
            pl.BlockSpec(memory_space=pl.ANY),
        ],
        out_specs=pl.BlockSpec(memory_space=pl.ANY),
        out_shape=jax.ShapeDtypeStruct((H // 2, 2, C, W), bf16),
        scratch_shapes=[
            pltpu.VMEM((C, 3 * C), bf16),
            pltpu.VMEM((C, C), bf16),
            pltpu.VMEM((48, 96), u32),
            pltpu.VMEM((56, 128), u32),
            pltpu.VMEM((3, 9, 32, 128), u32),
            pltpu.VMEM((3, 9, 32, 128), u32),
            pltpu.VMEM((NR, 2, 4, XR, 128), u32),
            pltpu.VMEM((NR, 2, 4, 8, 128), u32),
            pltpu.VMEM((NR, 2, 4, W, 128), u32),
            pltpu.VMEM((NR, 2, 4, 8, 128), u32),
            pltpu.VMEM((2, 4, NS, 16, 128), u32),
            pltpu.VMEM((2, 34, C, W), bf16),
            pltpu.VMEM((3, 16, 2, C, W), bf16),
            pltpu.SemaphoreType.DMA((19,)),
        ],
        compiler_params=pltpu.CompilerParams(
            dimension_semantics=("arbitrary",), vmem_limit_bytes=64 * 1024 * 1024,
            disable_bounds_checks=True),
        name="nat_kernel",
    )(xt, wqkv, wo)
    return jnp.transpose(out.reshape(H, C, W), (0, 2, 1)).reshape(1, H, W, C)
```
